```python
import jax
import jax.numpy as jnp

def _softmax(x, axis=-1):
    return jax.nn.softmax(x, axis=axis)

def _gelu(x):
    return jax.nn.gelu(x, approximate=True)

def _silu(x):
    return jax.nn.silu(x)

def _sigmoid(x):
    return jax.nn.sigmoid(x)

def _layernorm(x, axis=-1, eps=1e-05):
    m = jnp.mean(x, axis=axis, keepdims=True)
    v = jnp.var(x, axis=axis, keepdims=True)
    return (x - m) / jnp.sqrt(v + eps)

def _scatter_add(tgt, idx, src, axis=0):
    return tgt.at[idx].add(src)

def _segment_sum(src, seg, n):
    return jax.ops.segment_sum(src, seg, n)

class _Rng:

    def __init__(self, key):
        self._k = key

    def _next(self):
        self._k, sub = jax.random.split(self._k)
        return sub

    def normal(self, shape):
        return jax.random.normal(self._next(), shape, dtype=jnp.bfloat16)

    def randint(self, lo, hi, shape):
        return jax.random.randint(self._next(), shape, lo, hi, dtype=jnp.int32)

    def uniform(self, shape, lo=0.0, hi=1.0):
        return jax.random.uniform(self._next(), shape, jnp.bfloat16, lo, hi)

    def permutation(self, n):
        return jax.random.permutation(self._next(), n)
kernel_name = 'adaLN_cond__memory_aug_recurrent_mem_tr__glu_gated_swiglu__prompt'

def setup_inputs():
    _rng = _Rng(jax.random.key(int.from_bytes(__import__("os").urandom(4), "little")))
    _w = lambda a: (lambda t: t.astype(jnp.bfloat16) if jnp.issubdtype(t.dtype, jnp.floating) else t)(jnp.asarray(a))

    def _A_setup():
        B, S, Dm = (1, 2048, 1024)
        H, Dh = (32, 128)
        M, seg = (8, 32)
        seg = min(seg, S)
        S = S // seg * seg
        return {'x': _w((lambda *s: _rng.normal(s) * 0.05)(B, S, Dm)), 'mem0': _w((lambda *s: _rng.normal(s) * 0.05)(B, M, Dm)), 'Wq': _w((lambda *s: _rng.normal(s) * 0.05)(Dm, H, Dh) * Dm ** (-0.5)), 'Wk': _w((lambda *s: _rng.normal(s) * 0.05)(Dm, H, Dh) * Dm ** (-0.5)), 'Wv': _w((lambda *s: _rng.normal(s) * 0.05)(Dm, H, Dh) * Dm ** (-0.5)), 'Wo': _w((lambda *s: _rng.normal(s) * 0.05)(H, Dh, Dm) * (H * Dh) ** (-0.5)), 'seg_len': seg}
    _A_in = _A_setup()

    def _B_setup():
        B, S, D, F = (1, 2048, 1024, 3584)
        return {'x': _w((lambda *s: _rng.normal(s) * 0.05)(B, S, D)), 'w1': _w((lambda *s: _rng.normal(s) * 0.05)(D, F) * (2.0 / D) ** 0.5), 'w3': _w((lambda *s: _rng.normal(s) * 0.05)(D, F) * (2.0 / D) ** 0.5), 'w2': _w((lambda *s: _rng.normal(s) * 0.05)(F, D) * (2.0 / F) ** 0.5)}
    _B_in = _B_setup()
    return {'A_x': _A_in['x'], 'A_mem0': _A_in['mem0'], 'A_Wq': _A_in['Wq'], 'A_Wk': _A_in['Wk'], 'A_Wv': _A_in['Wv'], 'A_Wo': _A_in['Wo'], 'A_seg_len': _A_in['seg_len'], 'B_x': _B_in['x'], 'B_w1': _B_in['w1'], 'B_w3': _B_in['w3'], 'B_w2': _B_in['w2'], 'c': _w((lambda *s: _rng.normal(s) * 0.05)(1, 1024)), 'w_mod': _w((lambda *s: _rng.normal(s) * 0.05)(1024, 6 * 1024) * 1024 ** (-0.5))}

def reference(A_x, A_mem0, A_Wq, A_Wk, A_Wv, A_Wo, A_seg_len, B_x, B_w1, B_w3, B_w2, c, w_mod):

    def _A_ref(x, mem0, Wq, Wk, Wv, Wo, seg_len):
        B, S, Dm = x.shape
        H, Dh = (Wq.shape[1], Wq.shape[2])
        M = mem0.shape[1]
        scale = Dh ** (-0.5)
        n_seg = S // seg_len
        L = M + seg_len
        idx = jnp.arange(L)
        mask = (idx[:, None] < M) | (idx[:, None] >= idx[None, :])
        mem = mem0
        outs = []
        for s in range(n_seg):
            xs = x[:, s * seg_len:(s + 1) * seg_len, :].copy()
            h = jnp.concatenate([mem, xs], axis=1)
            q = jnp.einsum('btd,dhe->bhte', h, Wq)
            k = jnp.einsum('btd,dhe->bhte', h, Wk)
            v = jnp.einsum('btd,dhe->bhte', h, Wv)
            scores = jnp.einsum('bhqe,bhke->bhqk', q, k) * scale
            scores = jnp.where(mask[None, None], scores, -1000000000.0)
            p = _softmax(scores, axis=-1)
            o = jnp.einsum('bhqk,bhke->bhqe', p, v)
            o = jnp.einsum('bhte,hed->btd', o, Wo)
            mem = o[:, :M, :].copy()
            outs.append(o[:, M:, :])
        return jnp.concatenate(outs, axis=1)

    def _B_ref(x, w1, w3, w2):
        gate = jnp.einsum('bsd,df->bsf', x, w1)
        up = jnp.einsum('bsd,df->bsf', x, w3)
        h = _silu(gate) * up
        out = jnp.einsum('bsf,fd->bsd', h, w2)
        return out
    x = A_x
    mod = (_silu(c) @ w_mod).reshape(c.shape[0], 6, 1, -1)
    sa, ca, ga, sb, cb, gb = (mod[:, 0].copy(), mod[:, 1].copy(), mod[:, 2].copy(), mod[:, 3].copy(), mod[:, 4].copy(), mod[:, 5].copy())
    h = _layernorm(x, axis=-1) * (1 + ca) + sa
    x = x + ga * _A_ref(h, A_mem0, A_Wq, A_Wk, A_Wv, A_Wo, A_seg_len)
    h = _layernorm(x, axis=-1) * (1 + cb) + sb
    x = x + gb * _B_ref(h, B_w1, B_w3, B_w2)
    return x
```

```python
import functools

import jax
import jax.numpy as jnp
import jax.experimental.pallas as pl
import jax.experimental.pallas.tpu as pltpu

F32 = jnp.float32
BF16 = jnp.bfloat16
U32 = jnp.uint32

HG = 4
FFN_TM = 512
FFN_TF = 512


def _dot(a, b):
    return jax.lax.dot_general(a, b, (((1,), (0,)), ((), ())), preferred_element_type=F32)


def _dot_nt(a, b):
    return jax.lax.dot_general(a, b, (((1,), (1,)), ((), ())), preferred_element_type=F32)


def _round_bf16(x):
    return x.astype(BF16).astype(F32)


def _layernorm(x):
    m = jnp.mean(x, axis=-1, keepdims=True)
    d = x - m
    v = jnp.mean(d * d, axis=-1, keepdims=True)
    return d * jax.lax.rsqrt(v + 1e-5)


def _kernel(x_hbm, mem0_ref, wq_hbm, wk_hbm, wv_hbm, wo_hbm, w1_hbm, w3_hbm, w2_hbm, c_ref, wmod_hbm,
            out_hbm,
            x_buf, wqkv, wo, w1, w3, w2, mod, h1, x1, h2, stage, wstage, obuf,
            sem_x, sem_stage, sem_wstage, sem_ffn, sem_out, *, seg, n_heads, dh):
    S, D = x_buf.shape
    M = mem0_ref.shape[0]
    L = M + seg
    n_seg = S // seg
    scale = dh ** -0.5
    F = w1.shape[1]

    x_cp = pltpu.make_async_copy(x_hbm, x_buf, sem_x)

    def wmod_cp(j):
        return pltpu.make_async_copy(wmod_hbm.at[:, pl.ds(j * D, D)], wstage.at[j % 2], sem_wstage.at[j % 2])

    def wo_cp(j):
        return pltpu.make_async_copy(wo_hbm.at[pl.ds(j * D, D), :], wstage.at[j % 2], sem_wstage.at[j % 2])

    n_slot, stage_rows, _ = stage.shape
    dch = stage_rows // n_heads
    n_ch = D // dch
    w_hbms = (wq_hbm, wk_hbm, wv_hbm)

    def wqkv_cp(i):
        return pltpu.make_async_copy(w_hbms[i // n_ch].at[pl.ds((i % n_ch) * stage_rows, stage_rows), :],
                                     stage.at[i % n_slot], sem_stage.at[i % n_slot])

    ffn_cps = [pltpu.make_async_copy(s_, d_, sem_ffn.at[i])
               for i, (s_, d_) in enumerate(((w1_hbm, w1), (w3_hbm, w3), (w2_hbm, w2)))]

    wmod_cp(0).start()
    wmod_cp(1).start()
    x_cp.start()
    for i in range(n_slot):
        wqkv_cp(i).start()

    cc = c_ref[...].astype(F32)
    sc = jnp.broadcast_to(_round_bf16(cc * jax.nn.sigmoid(cc)), (8, D))
    for j in range(6):
        wmod_cp(j).wait()
        mod[j] = _dot(sc, wstage[j % 2])
        if j + 2 < 6:
            wmod_cp(j + 2).start()
        else:
            wo_cp(j - 4).start()

    x_cp.wait()

    def ln1_body(i, _):
        r = pl.ds(pl.multiple_of(i * 128, 128), 128)
        h = _layernorm(x_buf[r, :].astype(F32)) * (1.0 + mod[1, 0:1, :]) + mod[0, 0:1, :]
        h1[r, :] = _round_bf16(h)
        return 0

    jax.lax.fori_loop(0, S // 128, ln1_body, 0)

    stage32 = stage.bitcast(U32)
    for i in range(3 * n_ch):
        wqkv_cp(i).wait()
        for hp in range(n_heads // 2):
            w = stage32[i % n_slot, pl.ds(hp, dch, stride=n_heads // 2), :]
            lo = pltpu.bitcast(w << 16, F32).astype(BF16)
            hi = pltpu.bitcast(w & jnp.uint32(0xFFFF0000), F32).astype(BF16)
            rows = pl.ds((i % n_ch) * (dch // 2), dch // 2)
            wqkv[i // n_ch, rows, pl.ds(2 * hp * dh, dh)] = pltpu.bitcast(lo, U32)
            wqkv[i // n_ch, rows, pl.ds((2 * hp + 1) * dh, dh)] = pltpu.bitcast(hi, U32)
        if i + n_slot < 3 * n_ch:
            wqkv_cp(i + n_slot).start()

    n_wo = n_heads * dh // D
    for j in range(n_wo):
        wo_cp(j).wait()
        wo[pl.ds(j * (D // 2), D // 2), :] = pltpu.bitcast(wstage[j % 2], U32)
        if j + 2 < n_wo:
            wo_cp(j + 2).start()
    for cp in ffn_cps:
        cp.start()

    def seg_body(s, mem):
        r = pl.ds(pl.multiple_of(s * seg, seg), seg)
        lhs = jnp.concatenate([mem, h1[r, :]], axis=0)
        qi = jax.lax.broadcasted_iota(jnp.int32, (L, L), 0)
        ki = jax.lax.broadcasted_iota(jnp.int32, (L, L), 1)
        mask = (qi < M) | (qi >= ki)
        acc = None
        for g in range(n_heads // HG):
            cols = pl.ds(g * HG * dh, HG * dh)
            q, k, v = (_dot(lhs, pltpu.bitcast(wqkv[t, :, cols], BF16)) for t in range(3))
            o = []
            for h in range(HG):
                hs = slice(h * dh, (h + 1) * dh)
                sc_ = _dot_nt(q[:, hs], k[:, hs].astype(BF16)) * scale
                sc_ = jnp.where(mask, sc_, -1e9)
                e = jnp.exp(sc_ - jnp.max(sc_, axis=-1, keepdims=True))
                den = jnp.sum(e, axis=-1, keepdims=True)
                o.append(_dot(e, v[:, hs].astype(BF16)) / den)
            o = jnp.concatenate(o, axis=1)
            y = _dot(o, pltpu.bitcast(wo[pl.ds(g * HG * dh // 2, HG * dh // 2), :], BF16))
            acc = y if acc is None else acc + y
        xn = x_buf[r, :].astype(F32) + mod[2, 0:1, :] * acc[M:]
        x1[r, :] = xn
        h2[r, :] = (_layernorm(xn) * (1.0 + mod[4, 0:1, :]) + mod[3, 0:1, :]).astype(BF16)
        return _round_bf16(acc[:M])

    jax.lax.fori_loop(0, n_seg, seg_body, mem0_ref[...].astype(F32))

    for cp in ffn_cps:
        cp.wait()

    def out_cp(i):
        return pltpu.make_async_copy(obuf.at[i % 2], out_hbm.at[pl.ds(i * FFN_TM, FFN_TM), :], sem_out.at[i % 2])

    n_blk = S // FFN_TM

    def ffn_body(i, _):
        r = pl.ds(pl.multiple_of(i * FFN_TM, FFN_TM), FFN_TM)
        h = h2[r, :]
        acc = None
        for j in range(F // FFN_TF):
            cols = pl.ds(j * FFN_TF, FFN_TF)
            gate = _dot(h, w1[:, cols])
            up = _dot(h, w3[:, cols])
            a = (gate * jax.nn.sigmoid(gate) * up).astype(BF16)
            y = _dot(a, w2[cols, :])
            acc = y if acc is None else acc + y

        @pl.when(i >= 2)
        def _():
            out_cp(i - 2).wait()

        obuf[i % 2] = (x1[r, :] + mod[5, 0:1, :] * acc).astype(obuf.dtype)
        out_cp(i).start()
        return 0

    jax.lax.fori_loop(0, n_blk, ffn_body, 0)
    for i in range(max(n_blk - 2, 0), n_blk):
        out_cp(i).wait()


@functools.partial(jax.jit, static_argnames=("A_seg_len",))
def pallas_adaLN_cond__memory_aug_recurrent_mem_tr__glu_gated_swiglu__prompt_kernel(
    A_x, A_mem0, A_Wq, A_Wk, A_Wv, A_Wo, A_seg_len, B_x, B_w1, B_w3, B_w2, c, w_mod,
):
    del B_x
    B, S, D = A_x.shape
    assert B == 1
    M = A_mem0.shape[1]
    _, H, Dh = A_Wq.shape
    F = B_w1.shape[1]
    any_spec = pl.BlockSpec(memory_space=pl.ANY)
    vmem_spec = pl.BlockSpec(memory_space=pltpu.VMEM)
    out = pl.pallas_call(
        functools.partial(_kernel, seg=int(A_seg_len), n_heads=H, dh=Dh),
        out_shape=jax.ShapeDtypeStruct((S, D), A_x.dtype),
        in_specs=[any_spec, vmem_spec] + [any_spec] * 7 + [vmem_spec, any_spec],
        out_specs=any_spec,
        scratch_shapes=[
            pltpu.VMEM((S, D), BF16),
            pltpu.VMEM((3, D // 2, H * Dh), U32),
            pltpu.VMEM((H * Dh // 2, D), U32),
            pltpu.VMEM((D, F), BF16),
            pltpu.VMEM((D, F), BF16),
            pltpu.VMEM((F, D), BF16),
            pltpu.VMEM((6, 8, D), F32),
            pltpu.VMEM((S, D), F32),
            pltpu.VMEM((S, D), F32),
            pltpu.VMEM((S, D), BF16),
            pltpu.VMEM((4, 256 * H, Dh), BF16),
            pltpu.VMEM((2, D, D), BF16),
            pltpu.VMEM((2, FFN_TM, D), A_x.dtype),
            pltpu.SemaphoreType.DMA(()),
            pltpu.SemaphoreType.DMA((4,)),
            pltpu.SemaphoreType.DMA((2,)),
            pltpu.SemaphoreType.DMA((3,)),
            pltpu.SemaphoreType.DMA((2,)),
        ],
        compiler_params=pltpu.CompilerParams(vmem_limit_bytes=124 * 1024 * 1024),
    )(
        A_x.reshape(S, D), A_mem0.reshape(M, D),
        A_Wq.reshape(D * H, Dh), A_Wk.reshape(D * H, Dh), A_Wv.reshape(D * H, Dh), A_Wo.reshape(H * Dh, D),
        B_w1, B_w3, B_w2, c, w_mod,
    )
    return out.reshape(B, S, D)
```

```python
import functools

import jax
import jax.numpy as jnp
import jax.experimental.pallas as pl
import jax.experimental.pallas.tpu as pltpu

F32 = jnp.float32
BF16 = jnp.bfloat16
U32 = jnp.uint32

PRE = 8
WG = 8
LAG = 3
UNROLL = 1
HG = 4
FFN_TM = 512
FFN_TF = 512


def _dot(a, b):
    return jax.lax.dot_general(a, b, (((1,), (0,)), ((), ())), preferred_element_type=F32)


def _dot_nt(a, b):
    return jax.lax.dot_general(a, b, (((1,), (1,)), ((), ())), preferred_element_type=F32)


def _round_bf16(x):
    return x.astype(BF16).astype(F32)


def _layernorm(x):
    m = jnp.mean(x, axis=-1, keepdims=True)
    d = x - m
    v = jnp.mean(d * d, axis=-1, keepdims=True)
    return d * jax.lax.rsqrt(v + 1e-5)


def _kernel(x_hbm, mem0_ref, wq_hbm, wk_hbm, wv_hbm, wo_hbm, w1_hbm, w3_hbm, w2_hbm, c_ref, wmod_hbm,
            out_hbm,
            x_buf, xp, hp, wq, wk, wv, wo, pre, w1, w3, w2, mod, hn, att, x1, h2, stage, mstage, ostage, obuf,
            sem_x, sem_stage, sem_m, sem_o, sem_ffn, sem_out, *, n_heads, dh):
    n_seg, seg, D = x_buf.shape
    S = n_seg * seg
    M = mem0_ref.shape[0]
    L = M + seg
    scale = dh ** -0.5
    F = w1.shape[1]
    n_grp = n_heads // WG
    w_hbms = (wq_hbm, wk_hbm, wv_hbm)
    w_bufs = (wq, wk, wv)

    xp_cp = pltpu.make_async_copy(x_hbm.at[:, pl.ds(0, PRE), :], xp, sem_x.at[0])
    x_cp = pltpu.make_async_copy(x_hbm, x_buf, sem_x.at[1])

    def wmod_cp(j, slot):
        return pltpu.make_async_copy(wmod_hbm.at[:, pl.ds(pl.multiple_of(j * D, D), D)], mstage.at[slot],
                                     sem_m.at[slot])

    def wo_cp(g):
        return pltpu.make_async_copy(wo_hbm.at[pl.ds(pl.multiple_of(g * WG * dh, WG * dh), WG * dh), :], ostage, sem_o)

    def w_cps(t, g):
        return [pltpu.make_async_copy(w_hbms[t].at[:, pl.ds(pl.multiple_of(p * n_heads + g * WG, WG), WG), :],
                                      stage.at[t, :, pl.ds(p * WG, WG), :], sem_stage.at[2 * t + p])
                for p in range(2)]

    def start(cps):
        for cp in cps:
            cp.start()

    def wait(cps):
        for cp in cps:
            cp.wait()

    ffn_cps = [pltpu.make_async_copy(s_, d_, sem_ffn.at[i])
               for i, (s_, d_) in enumerate(((w1_hbm, w1), (w3_hbm, w3), (w2_hbm, w2)))]

    def relayout(t, g):
        rb = 64
        for b in range(D // 2 // rb):
            rows = pl.ds(b * rb, rb)
            w = jnp.swapaxes(pltpu.bitcast(stage[t, rows], U32), 0, 1)
            for j in range(WG // 2):
                even, odd = w[j], w[WG // 2 + j]
                w_bufs[t][g, rows, pl.ds(2 * j * dh, dh)] = (even & jnp.uint32(0xFFFF)) | (odd << 16)
                w_bufs[t][g, rows, pl.ds((2 * j + 1) * dh, dh)] = (even >> 16) | (odd & jnp.uint32(0xFFFF0000))

    def ada_ln(x, j):
        return _layernorm(x) * (1.0 + mod[j + 1, 0:1, :]) + mod[j, 0:1, :]

    xp_cp.start()
    wmod_cp(0, 0).start()
    wmod_cp(1, 1).start()
    start(w_cps(0, 0))
    cc = c_ref[...].astype(F32)
    sc = jnp.broadcast_to(cc * jax.nn.sigmoid(cc), (16, D)).astype(BF16)
    att[...] = jnp.zeros_like(att)
    for j in range(2):
        wmod_cp(j, j).wait()
        start(w_cps(j + 1, 0))
        mod[j] = _dot(sc, mstage[j])[:8]
    xp_cp.wait()
    nb = 128 // PRE
    for i in range(n_seg // nb):
        xs = xp[pl.ds(i * nb, nb)].astype(F32).reshape(nb * PRE, D)
        hp[pl.ds(i * nb * PRE, nb * PRE), :] = ada_ln(xs, 0).astype(BF16)
    wait(w_cps(0, 0))
    relayout(0, 0)

    def pre_body(g, _):
        wmod_cp(g + 2, 0).start()
        wo_cp(g).start()
        for t in range(3):
            @pl.when(g + 1 < n_grp)
            def _():
                start(w_cps(t, g + 1))

            if t == 0:
                @pl.when(g + 1 == n_grp)
                def _():
                    x_cp.start()

            if t < 2:
                wait(w_cps(t + 1, g))
            else:
                @pl.when(g + 1 < n_grp)
                def _():
                    wait(w_cps(0, g + 1))

                wmod_cp(g + 2, 0).wait()
                wo_cp(g).wait()
            pre[t, g] = _dot(hp[...], pltpu.bitcast(w_bufs[t][g], BF16))
            if t < 2:
                relayout(t + 1, g)
            else:
                relayout(0, jnp.minimum(g + 1, n_grp - 1))
                wo[g] = pltpu.bitcast(ostage[...], U32)
                mod[g + 2] = _dot(sc, mstage[0])[:8]
        return 0

    jax.lax.fori_loop(0, n_grp, pre_body, 0)
    start(ffn_cps)
    x_cp.wait()

    def ln1(s):
        hn[...] = ada_ln(x_buf[s, pl.ds(PRE, seg - PRE), :].astype(F32), 0)

    def ln2(s):
        r = pl.ds(pl.multiple_of(s * seg, seg), seg)
        xn = x_buf[s].astype(F32) + mod[2, 0:1, :] * att[...]
        x1[r, :] = xn
        h2[r, :] = ada_ln(xn, 3).astype(BF16)

    ln1(0)
    n_hg = n_heads // HG

    def seg_body(s, mem):
        lhs = jnp.concatenate([mem, hn[...]], axis=0).astype(BF16)
        ln2(jnp.maximum(s - 1, 0))
        ln1(jnp.minimum(s + 1, n_seg - 1))
        qi = jax.lax.broadcasted_iota(jnp.int32, (L, L), 0)
        ki = jax.lax.broadcasted_iota(jnp.int32, (L, L), 1)
        mask = (qi < M) | (qi >= ki)
        pr = pl.ds(pl.multiple_of(s * PRE, PRE), PRE)

        def proj(t, g):
            gi, cols = g * HG // WG, pl.ds(g * HG % WG * dh, HG * dh)
            y = _dot(lhs, pltpu.bitcast(w_bufs[t][gi, :, cols], BF16))
            y = jnp.concatenate([y[:M], pre[t, gi, pr, cols], y[M:]], axis=0)
            return [y[:, h * dh:(h + 1) * dh] for h in range(HG)]

        def probs(q, k):
            sc_ = jnp.where(mask, _dot_nt(q, k.astype(BF16)) * scale, -1e9)
            e = jnp.exp(sc_ - jnp.max(sc_, axis=-1, keepdims=True))
            return e, 1.0 / jnp.sum(e, axis=-1, keepdims=True)

        def mix(p, v):
            return jnp.concatenate([_dot(e, vh.astype(BF16)) * r for (e, r), vh in zip(p, v)], axis=1)

        def out_proj(o, g):
            rows = pl.ds(g * HG % WG * dh // 2, HG * dh // 2)
            return _dot(o, pltpu.bitcast(wo[g * HG // WG, rows, :], BF16))

        o, acc, p, v = {}, None, None, None
        done = 0
        for g in range(n_hg):
            q = proj(0, g)
            k = proj(1, g)
            if g:
                o[g - 1] = mix(p, v)
            v = proj(2, g)
            p = [probs(qh, kh) for qh, kh in zip(q, k)]
            upto = g + 1 - LAG if g + 1 < n_hg else n_hg - 2
            while done < upto:
                y = out_proj(o.pop(done), done)
                acc = y if acc is None else acc + y
                done += 1
        o[n_hg - 1] = mix(p, v)
        for g in range(done, n_hg):
            acc = acc + out_proj(o.pop(g), g)
        att[...] = acc[M:]
        return acc[:M]

    jax.lax.fori_loop(0, n_seg, seg_body, mem0_ref[...].astype(F32), unroll=UNROLL)
    ln2(n_seg - 1)

    for cp in ffn_cps:
        cp.wait()

    def out_cp(i):
        return pltpu.make_async_copy(obuf.at[i % 2], out_hbm.at[pl.ds(i * FFN_TM, FFN_TM), :], sem_out.at[i % 2])

    n_blk = S // FFN_TM

    def ffn_body(i, _):
        r = pl.ds(pl.multiple_of(i * FFN_TM, FFN_TM), FFN_TM)
        h = h2[r, :]
        acc = None
        for j in range(F // FFN_TF):
            cols = pl.ds(j * FFN_TF, FFN_TF)
            gate = _dot(h, w1[:, cols])
            up = _dot(h, w3[:, cols])
            a = (gate * jax.nn.sigmoid(gate) * up).astype(BF16)
            y = _dot(a, w2[cols, :])
            acc = y if acc is None else acc + y

        @pl.when(i >= 2)
        def _():
            out_cp(i - 2).wait()

        obuf[i % 2] = (x1[r, :] + mod[5, 0:1, :] * acc).astype(obuf.dtype)
        out_cp(i).start()
        return 0

    jax.lax.fori_loop(0, n_blk, ffn_body, 0)
    for i in range(max(n_blk - 2, 0), n_blk):
        out_cp(i).wait()


@functools.partial(jax.jit, static_argnames=("A_seg_len",))
def pallas_adaLN_cond__memory_aug_recurrent_mem_tr__glu_gated_swiglu__prompt_kernel(
    A_x, A_mem0, A_Wq, A_Wk, A_Wv, A_Wo, A_seg_len, B_x, B_w1, B_w3, B_w2, c, w_mod,
):
    del B_x
    B, S, D = A_x.shape
    assert B == 1
    M = A_mem0.shape[1]
    _, H, Dh = A_Wq.shape
    F = B_w1.shape[1]
    seg = int(A_seg_len)
    n_seg, n_grp = S // seg, H // WG
    assert n_grp == 4
    any_spec = pl.BlockSpec(memory_space=pl.ANY)
    vmem_spec = pl.BlockSpec(memory_space=pltpu.VMEM)
    out = pl.pallas_call(
        functools.partial(_kernel, n_heads=H, dh=Dh),
        out_shape=jax.ShapeDtypeStruct((S, D), A_x.dtype),
        in_specs=[any_spec, vmem_spec] + [any_spec] * 7 + [vmem_spec, any_spec],
        out_specs=any_spec,
        scratch_shapes=[
            pltpu.VMEM((n_seg, seg, D), BF16),
            pltpu.VMEM((n_seg, PRE, D), BF16),
            pltpu.VMEM((n_seg * PRE, D), BF16),
            pltpu.VMEM((n_grp, D // 2, WG * Dh), U32),
            pltpu.VMEM((n_grp, D // 2, WG * Dh), U32),
            pltpu.VMEM((n_grp, D // 2, WG * Dh), U32),
            pltpu.VMEM((n_grp, WG * Dh // 2, D), U32),
            pltpu.VMEM((3, n_grp, n_seg * PRE, WG * Dh), F32),
            pltpu.VMEM((D, F), BF16),
            pltpu.VMEM((D, F), BF16),
            pltpu.VMEM((F, D), BF16),
            pltpu.VMEM((6, 8, D), F32),
            pltpu.VMEM((seg - PRE, D), F32),
            pltpu.VMEM((seg, D), F32),
            pltpu.VMEM((S, D), F32),
            pltpu.VMEM((S, D), BF16),
            pltpu.VMEM((3, D // 2, 2 * WG, Dh), BF16),
            pltpu.VMEM((2, D, D), BF16),
            pltpu.VMEM((WG * Dh, D), BF16),
            pltpu.VMEM((2, FFN_TM, D), A_x.dtype),
            pltpu.SemaphoreType.DMA((2,)),
            pltpu.SemaphoreType.DMA((6,)),
            pltpu.SemaphoreType.DMA((2,)),
            pltpu.SemaphoreType.DMA(()),
            pltpu.SemaphoreType.DMA((3,)),
            pltpu.SemaphoreType.DMA((2,)),
        ],
        compiler_params=pltpu.CompilerParams(vmem_limit_bytes=124 * 1024 * 1024),
    )(
        A_x.reshape(n_seg, seg, D), A_mem0.reshape(M, D),
        A_Wq.reshape(D // 2, 2 * H, Dh), A_Wk.reshape(D // 2, 2 * H, Dh), A_Wv.reshape(D // 2, 2 * H, Dh),
        A_Wo.reshape(H * Dh, D),
        B_w1, B_w3, B_w2, c, w_mod,
    )
    return out.reshape(B, S, D)
```

```python
import functools

import jax
import jax.numpy as jnp
import jax.experimental.pallas as pl
import jax.experimental.pallas.tpu as pltpu

F32 = jnp.float32
BF16 = jnp.bfloat16
U32 = jnp.uint32

PRE = 8
WG = 8
LAG = 3
LHS_AT = 2
LR = 16
PREP_G = 6
DMA_AT = 0
RB = 8
UNROLL = 1
HG = 4
FFN_TM = 256
FFN_TF = 128


def _dot(a, b):
    return jax.lax.dot_general(a, b, (((1,), (0,)), ((), ())), preferred_element_type=F32)


def _dot_nt(a, b):
    return jax.lax.dot_general(a, b, (((1,), (1,)), ((), ())), preferred_element_type=F32)


def _round_bf16(x):
    return x.astype(BF16).astype(F32)


def _layernorm(x):
    m = jnp.mean(x, axis=-1, keepdims=True)
    d = x - m
    v = jnp.mean(d * d, axis=-1, keepdims=True)
    return d * jax.lax.rsqrt(v + 1e-5)


def _pack(x):
    return pltpu.bitcast(x.astype(BF16), U32)


def _unpack(w):
    return pltpu.bitcast(w, BF16)


def _strassen_lhs(a11, a12, a21, a22):
    return (a11 + a22, a21 + a22, a11, a22, a11 + a12, a21 - a11, a12 - a22)


def _strassen_rhs(b11, b12, b21, b22):
    return (b11 + b22, b11, b12 - b22, b21 - b11, b22, b11 + b12, b21 + b22)


def _strassen_rhs_packed(blocks):
    words = [pltpu.bitcast(b, U32) for b in blocks]
    even = _strassen_rhs(*[pltpu.bitcast(w << 16, F32) for w in words])
    odd = _strassen_rhs(*[pltpu.bitcast(w & jnp.uint32(0xFFFF0000), F32) for w in words])
    out = [pltpu.pack_elementwise([e, o], packed_dtype=BF16) for e, o in zip(even, odd)]
    out[1], out[4] = words[0], words[3]
    return out


def _strassen_out(m):
    return (m[0] + m[3] - m[4] + m[6], m[2] + m[4], m[1] + m[3], m[0] - m[1] + m[2] + m[5])


def _kernel(x_hbm, mem0_ref, wq_hbm, wk_hbm, wv_hbm, wo_hbm, w1_hbm, w3_hbm, w2_hbm, c_ref, wmod_hbm,
            out_hbm,
            x_buf, wqkv, wo, pre, mod, mstage, sem_x, sem_stage, sem_m, sem_o, sem_ffn, sem_out, *, n_heads, dh):
    n_seg, seg, D = x_buf.shape
    S = n_seg * seg
    M = mem0_ref.shape[0]
    L = M + seg
    scale = dh ** -0.5
    F = w1_hbm.shape[2]
    n_grp = n_heads // WG
    w_hbms = (wq_hbm, wk_hbm, wv_hbm)

    x_cp = pltpu.make_async_copy(x_hbm, x_buf, sem_x.at[1])

    def wmod_cp(j, slot):
        return pltpu.make_async_copy(wmod_hbm.at[:, pl.ds(pl.multiple_of(j * D, D), D)], mstage.at[slot],
                                     sem_m.at[slot])

    def start(cps):
        for cp in cps:
            cp.start()

    def wait(cps):
        for cp in cps:
            cp.wait()

    def ada_ln(x, j):
        return _layernorm(x) * (1.0 + mod[j + 1, 0:1, :]) + mod[j, 0:1, :]

    cc = c_ref[...].astype(F32)
    sc = jnp.broadcast_to(cc * jax.nn.sigmoid(cc), (16, D)).astype(BF16)

    def load_phase(xp, hp, stage, ostage):
        xp_cp = pltpu.make_async_copy(x_hbm.at[:, pl.ds(0, PRE), :], xp, sem_x.at[0])

        def wo_cp(g):
            return pltpu.make_async_copy(wo_hbm.at[pl.ds(pl.multiple_of(g * WG * dh, WG * dh), WG * dh), :], ostage, sem_o)

        def w_cps(t, g):
            return [pltpu.make_async_copy(w_hbms[t].at[:, pl.ds(pl.multiple_of(p * n_heads + g * WG, WG), WG), :],
                                          stage.at[t, :, pl.ds(p * WG, WG), :], sem_stage.at[2 * t + p])
                    for p in range(2)]

        def relayout(t, c, part=0, n_part=1):
            nb_ = D // 2 // RB // n_part
            for b in range(part * nb_, (part + 1) * nb_):
                rows = pl.ds(b * RB, RB)
                w = jnp.swapaxes(pltpu.bitcast(stage[t, rows], U32), 0, 1)
                for j in range(WG // 2):
                    even, odd = w[j], w[WG // 2 + j]
                    wqkv[c, rows, pl.ds(2 * j * dh, dh)] = (even & jnp.uint32(0xFFFF)) | (odd << 16)
                    wqkv[c, rows, pl.ds((2 * j + 1) * dh, dh)] = (even >> 16) | (odd & jnp.uint32(0xFFFF0000))

        xp_cp.start()
        wmod_cp(0, 0).start()
        wmod_cp(1, 1).start()
        start(w_cps(0, 0))
        for j in range(2):
            wmod_cp(j, j).wait()
            start(w_cps(j + 1, 0))
            mod[j] = _dot(sc, mstage[j])[:8]
        xp_cp.wait()
        nb = 128 // PRE
        for i in range(n_seg // nb):
            xs = xp[pl.ds(i * nb, nb)].astype(F32).reshape(nb * PRE, D)
            hp[pl.ds(i * nb * PRE // 2, nb * PRE // 2), :] = _pack(ada_ln(xs, 0))
        wait(w_cps(0, 0))
        relayout(0, 0)

        n_chunk = 3 * n_grp

        def pre_body(c, _):
            g = c // 3
            for t in range(3):
                @pl.when(c % 3 == t)
                def _():
                    @pl.when(g + 1 < n_grp)
                    def _():
                        start(w_cps(t, g + 1))

                    if t == 0:
                        wo_cp(g).start()

                        @pl.when(g + 1 == n_grp)
                        def _():
                            x_cp.start()

                    if t < 2:
                        wait(w_cps(t + 1, g))
                    else:
                        @pl.when(g + 1 < n_grp)
                        def _():
                            wait(w_cps(0, g + 1))

                        wo_cp(g).wait()
                        wmod_cp(g + 2, g).start()
                        wo[g] = pltpu.bitcast(ostage[...], U32)

            nxt = jnp.minimum(c + 1, n_chunk - 1)
            for i in range(WG):
                cols = pl.ds(i * dh, dh)
                y = _dot(_unpack(hp[...]), _unpack(wqkv[c, :, cols]))
                relayout(nxt % 3, nxt, i, WG)
                pre[c, :, cols] = y
            return 0

        with jax.named_scope('ph_pre'):
            jax.lax.fori_loop(0, n_chunk, pre_body, 0)

    pl.run_scoped(load_phase,
                  pltpu.VMEM((n_seg, PRE, D), BF16),
                  pltpu.VMEM((n_seg * PRE // 2, D), U32),
                  pltpu.VMEM((3, D // 2, 2 * WG, dh), BF16),
                  pltpu.VMEM((WG * dh, D), BF16))

    def main_phase(hn, att, st13, st2, w13, w2, h2, abuf, obuf):
        x_cp.wait()

        Dh2, Fh = D // 2, F // 2
        r13, r2, Fq = st13.shape[3], st2.shape[2], F // 4
        n13, n2 = 2 * Dh2 // r13, Fh // r2
        assert n13 <= n_seg and n2 <= n_seg

        def ffn_w_cps(s):
            slot, s13, s2 = s % 2, jnp.minimum(s, n13 - 1), jnp.minimum(s, n2 - 1)
            rows = pl.ds(pl.multiple_of(s13 // 2 * r13, r13), r13)
            cps = [pltpu.make_async_copy(w_hbm.at[:, rows, pl.ds(pl.multiple_of(p * Fh + s13 % 2 * Fq, 128), Fq)],
                                         st13.at[slot, 2 * t + p], sem_ffn.at[slot * 5 + 2 * t + p])
                   for t, w_hbm in enumerate((w1_hbm, w3_hbm)) for p in range(2)]
            return cps + [pltpu.make_async_copy(w2_hbm.at[:, pl.ds(pl.multiple_of(s2 * r2, r2), r2), :],
                                                st2.at[slot], sem_ffn.at[slot * 5 + 4])]

        def ffn_w_prepare(s, part, anchor):
            slot, s13, s2 = s % 2, jnp.minimum(s, n13 - 1), jnp.minimum(s, n2 - 1)
            spare = 2 + s // n_seg
            nq = Fq // 128
            if part < 2 * nq:
                t, cols = part // nq, pl.ds(part % nq * 128, 128)
                st13[spare, 0, 0, :, pl.ds(0, 128)] = anchor
                b = [st13[slot, 2 * t + p, hf, :, cols] for hf in range(2) for p in range(2)]
                rows = pl.ds(pl.multiple_of(s13 // 2 * (r13 // 2), r13 // 2), r13 // 2)
                for i, w in enumerate(_strassen_rhs_packed(b)):
                    w13[t, i, s13 % 2, rows, cols] = w
            else:
                rb, cb = divmod(part - 2 * nq, Dh2 // 128)
                st2[spare, 0, pl.ds(0, r13), pl.ds(0, 128)] = anchor
                b = [st2[slot, hf, pl.ds(rb * r13, r13), pl.ds(p * Dh2 + cb * 128, 128)]
                     for hf in range(2) for p in range(2)]
                rows = pl.ds(pl.multiple_of(s2 * (r2 // 2) + rb * (r13 // 2), r13 // 2), r13 // 2)
                for i, w in enumerate(_strassen_rhs_packed(b)):
                    w2[i, rows, pl.ds(cb * 128, 128)] = w

        n_prep = 2 * (Fq // 128) + r2 // r13 * (Dh2 // 128)
        start(ffn_w_cps(jnp.int32(0)))

        def ln1(s):
            hn[...] = ada_ln(x_buf[s, pl.ds(PRE, seg - PRE), :].astype(F32), 0)

        ln1(0)
        n_hg = n_heads // HG

        def seg_body(s, mem):
            lhs = jnp.concatenate([mem, hn[...]], axis=0).astype(BF16)
            ln1(jnp.minimum(s + 1, n_seg - 1))
            qi = jax.lax.broadcasted_iota(jnp.int32, (L, L), 0)
            ki = jax.lax.broadcasted_iota(jnp.int32, (L, L), 1)
            mask = (qi < M) | (qi >= ki)
            pr = pl.ds(pl.multiple_of(s * PRE, PRE), PRE)

            def proj(t, g):
                gi, cols = g * HG // WG, pl.ds(g * HG % WG * dh, HG * dh)
                y = _dot(lhs, pltpu.bitcast(wqkv[3 * gi + t, :, cols], BF16))
                y = jnp.concatenate([y[:M], pre[3 * gi + t, pr, cols], y[M:]], axis=0)
                return [y[:, h * dh:(h + 1) * dh] for h in range(HG)]

            def probs(q, k):
                sc_ = jnp.where(mask, _dot_nt(q, k.astype(BF16)) * scale, -1e9)
                e = jnp.exp(sc_ - jnp.max(sc_, axis=-1, keepdims=True))
                return e, 1.0 / jnp.sum(e, axis=-1, keepdims=True)

            def mix(p, v):
                return jnp.concatenate([_dot(e, vh.astype(BF16)) * r for (e, r), vh in zip(p, v)], axis=1)

            def out_proj(o, g):
                rows = pl.ds(g * HG % WG * dh // 2, HG * dh // 2)
                y = _dot(o, pltpu.bitcast(wo[g * HG // WG, rows, :], BF16))
                per = -(-n_prep // PREP_G)
                for i in range(g * per, min((g + 1) * per, n_prep)):
                    n = (i - g * per) * (D // 128) // per
                    ffn_w_prepare(s, i, y[:r13, n * 128:(n + 1) * 128].astype(BF16))
                return y

            o, acc, p, v = {}, None, None, None
            done = 0
            for g in range(n_hg):
                q = proj(0, g)
                k = proj(1, g)
                if g == DMA_AT:
                    wait(ffn_w_cps(s))
                    start(ffn_w_cps(s + 1))
                if g:
                    o[g - 1] = mix(p, v)
                v = proj(2, g)
                p = [probs(qh, kh) for qh, kh in zip(q, k)]
                upto = g + 1 - LAG if g + 1 < n_hg else n_hg - 2
                while done < upto:
                    y = out_proj(o.pop(done), done)
                    acc = y if acc is None else acc + y
                    done += 1
            o[n_hg - 1] = mix(p, v)
            for g in range(done, n_hg):
                acc = acc + out_proj(o.pop(g), g)
            att[s] = acc[M:].astype(BF16)
            return acc[:M]

        with jax.named_scope('ph_seg'):
            jax.lax.fori_loop(0, n_seg, seg_body, mem0_ref[...].astype(F32), unroll=UNROLL)

        wait(ffn_w_cps(jnp.int32(n_seg)))
        for j in range(4):
            wmod_cp(j + 2, j).wait()
            mod[j + 2] = _dot(sc, mstage[j])[:8]
        sb = FFN_TM // seg

        def resid(sg, rows):
            return x_buf[sg, rows, :].astype(F32) + mod[2, 0:1, :] * att[sg, rows, :].astype(F32)

        hm = FFN_TM // 2

        def ffn_lhs(i, slot, part):
            top, bot = (ada_ln(resid(i * sb + hf * sb // 2 + part * LR // seg, pl.ds(part * LR % seg, LR)), 3)
                        for hf in range(2))
            for j, a in enumerate(_strassen_lhs(top[:, :Dh2], top[:, Dh2:], bot[:, :Dh2], bot[:, Dh2:])):
                h2[slot, j, pl.ds(part * LR // 2, LR // 2), :] = _pack(a)

        for part in range(hm // LR):
            ffn_lhs(0, 0, part)

        def out_cp(i):
            return pltpu.make_async_copy(obuf.at[i % 2], out_hbm.at[pl.ds(i * FFN_TM, FFN_TM), :], sem_out.at[i % 2])

        n_blk = S // FFN_TM

        def ffn_body(i, _):
            @pl.when(i >= 2)
            def _():
                out_cp(i - 2).wait()

            for j in range(Fh // FFN_TF):
                nq = Fq // FFN_TF
                cols, wcols = pl.ds(j * FFN_TF, FFN_TF), pl.ds(j % nq * FFN_TF, FFN_TF)
                gate, up = (_strassen_out([_dot(_unpack(h2[i % 2, k]), _unpack(w13[t, k, j // nq, :, wcols])) for k in range(7)])
                            for t in range(2))
                if 0 <= j - LHS_AT < hm // LR:
                    ffn_lhs(jnp.minimum(i + 1, n_blk - 1), (i + 1) % 2, j - LHS_AT)
                act = [g * jax.nn.sigmoid(g) * u for g, u in zip(gate, up)]
                for k, a in enumerate(_strassen_lhs(*act)):
                    abuf[k, :, cols] = _pack(a)
            y = _strassen_out([_dot(_unpack(abuf[k]), _unpack(w2[k])) for k in range(7)])
            y = jnp.concatenate([jnp.concatenate(y[:2], axis=1), jnp.concatenate(y[2:], axis=1)], axis=0)
            obuf[i % 2] = (resid(pl.ds(i * sb, sb), slice(None)).reshape(FFN_TM, D) + mod[5, 0:1, :] * y).astype(obuf.dtype)
            out_cp(i).start()
            return 0

        with jax.named_scope('ph_ffn'):
            jax.lax.fori_loop(0, n_blk, ffn_body, 0)
        for i in range(max(n_blk - 2, 0), n_blk):
            out_cp(i).wait()

    pl.run_scoped(main_phase,
                  pltpu.VMEM((seg - PRE, D), F32),
                  pltpu.VMEM((n_seg, seg, D), BF16),
                  pltpu.VMEM((3, 4, 2, 16, F // 4), BF16),
                  pltpu.VMEM((3, 2, 32, D), BF16),
                  pltpu.VMEM((2, 7, 2, D // 4, F // 4), U32),
                  pltpu.VMEM((7, F // 4, D // 2), U32),
                  pltpu.VMEM((2, 7, FFN_TM // 4, D // 2), U32),
                  pltpu.VMEM((7, FFN_TM // 4, F // 2), U32),
                  pltpu.VMEM((2, FFN_TM, D), out_hbm.dtype))


@functools.partial(jax.jit, static_argnames=("A_seg_len",))
def pallas_adaLN_cond__memory_aug_recurrent_mem_tr__glu_gated_swiglu__prompt_kernel(
    A_x, A_mem0, A_Wq, A_Wk, A_Wv, A_Wo, A_seg_len, B_x, B_w1, B_w3, B_w2, c, w_mod,
):
    del B_x
    B, S, D = A_x.shape
    assert B == 1
    M = A_mem0.shape[1]
    _, H, Dh = A_Wq.shape
    F = B_w1.shape[1]
    seg = int(A_seg_len)
    n_seg, n_grp = S // seg, H // WG
    any_spec = pl.BlockSpec(memory_space=pl.ANY)
    vmem_spec = pl.BlockSpec(memory_space=pltpu.VMEM)
    out = pl.pallas_call(
        functools.partial(_kernel, n_heads=H, dh=Dh),
        out_shape=jax.ShapeDtypeStruct((S, D), A_x.dtype),
        in_specs=[any_spec, vmem_spec] + [any_spec] * 7 + [vmem_spec, any_spec],
        out_specs=any_spec,
        scratch_shapes=[
            pltpu.VMEM((n_seg, seg, D), BF16),
            pltpu.VMEM((3 * n_grp, D // 2, WG * Dh), U32),
            pltpu.VMEM((n_grp, WG * Dh // 2, D), U32),
            pltpu.VMEM((3 * n_grp, n_seg * PRE, WG * Dh), F32),
            pltpu.VMEM((6, 8, D), F32),
            pltpu.VMEM((4, D, D), BF16),
            pltpu.SemaphoreType.DMA((2,)),
            pltpu.SemaphoreType.DMA((6,)),
            pltpu.SemaphoreType.DMA((4,)),
            pltpu.SemaphoreType.DMA(()),
            pltpu.SemaphoreType.DMA((10,)),
            pltpu.SemaphoreType.DMA((2,)),
        ],
        compiler_params=pltpu.CompilerParams(vmem_limit_bytes=124 * 1024 * 1024),
    )(
        A_x.reshape(n_seg, seg, D), A_mem0.reshape(M, D),
        A_Wq.reshape(D // 2, 2 * H, Dh), A_Wk.reshape(D // 2, 2 * H, Dh), A_Wv.reshape(D // 2, 2 * H, Dh),
        A_Wo.reshape(H * Dh, D),
        B_w1.reshape(2, D // 2, F), B_w3.reshape(2, D // 2, F), B_w2.reshape(2, F // 2, D), c, w_mod,
    )
    return out.reshape(B, S, D)
```

```python
import functools

import jax
import jax.numpy as jnp
import jax.experimental.pallas as pl
import jax.experimental.pallas.tpu as pltpu

F32 = jnp.float32
BF16 = jnp.bfloat16
U32 = jnp.uint32

PRE = 8
WG = 8
LAG = 3
LHS_K = 2
DN = 128
MODN = 256
NSUB = 4
LR = 8
PREP_G = 6
RB = 8
UNROLL = 2
HG = 4
FFN_TM = 256
FFN_TF = 128


def _dot(a, b):
    return jax.lax.dot_general(a, b, (((1,), (0,)), ((), ())), preferred_element_type=F32)


def _dot_nt(a, b):
    return jax.lax.dot_general(a, b, (((1,), (1,)), ((), ())), preferred_element_type=F32)


def _round_bf16(x):
    return x.astype(BF16).astype(F32)


def _layernorm(x):
    m = jnp.mean(x, axis=-1, keepdims=True)
    d = x - m
    v = jnp.mean(d * d, axis=-1, keepdims=True)
    return d * jax.lax.rsqrt(v + 1e-5)


def _pack(x):
    return pltpu.bitcast(x.astype(BF16), U32)


def _unpack(w):
    return pltpu.bitcast(w, BF16)


def _strassen_lhs(a11, a12, a21, a22):
    return (a11 + a22, a21 + a22, a11, a22, a11 + a12, a21 - a11, a12 - a22)


def _strassen_rhs(b11, b12, b21, b22):
    return (b11 + b22, b11, b12 - b22, b21 - b11, b22, b11 + b12, b21 + b22)


def _strassen_rhs_packed(blocks):
    words = [pltpu.bitcast(b, U32) for b in blocks]
    even = _strassen_rhs(*[pltpu.bitcast(w << 16, F32) for w in words])
    odd = _strassen_rhs(*[pltpu.bitcast(w & jnp.uint32(0xFFFF0000), F32) for w in words])
    out = [pltpu.pack_elementwise([e, o], packed_dtype=BF16) for e, o in zip(even, odd)]
    out[1], out[4] = words[0], words[3]
    return out


def _strassen_out(m):
    return (m[0] + m[3] - m[4] + m[6], m[2] + m[4], m[1] + m[3], m[0] - m[1] + m[2] + m[5])


def _kernel(x_hbm, mem0_ref, wq_hbm, wk_hbm, wv_hbm, wo_hbm, w1_hbm, w3_hbm, w2_hbm, c_ref, wmod_hbm,
            out_hbm,
            x_buf, wqkv, wo, pre, mod, mstage, sem_x, sem_stage, sem_m, sem_o, sem_ffn, sem_out, *, n_heads, dh):
    n_seg, seg, D = x_buf.shape
    S = n_seg * seg
    M = mem0_ref.shape[0]
    L = M + seg
    scale = dh ** -0.5
    F = w1_hbm.shape[2]
    n_grp = n_heads // WG
    w_hbms = (wq_hbm, wk_hbm, wv_hbm)

    x_cp = pltpu.make_async_copy(x_hbm, x_buf, sem_x.at[1])

    def wmod_cp(j, slot):
        return pltpu.make_async_copy(wmod_hbm.at[:, pl.ds(pl.multiple_of(j * D, D), D)], mstage.at[slot],
                                     sem_m.at[slot])

    def start(cps):
        for cp in cps:
            cp.start()

    def wait(cps):
        for cp in cps:
            cp.wait()

    def ada_ln(x, j):
        return _layernorm(x) * (1.0 + mod[j + 1, 0:1, :]) + mod[j, 0:1, :]

    cc = c_ref[...].astype(F32)
    sc = jnp.broadcast_to(cc * jax.nn.sigmoid(cc), (16, D)).astype(BF16)

    def modulation(j, slot):
        @pl.loop(0, D // MODN)
        def _(n):
            cols = pl.ds(pl.multiple_of(n * MODN, MODN), MODN)
            mod[j, :, cols] = _dot(sc, mstage[slot, :, cols])[:8]

    def load_phase(xp, hp, stage, ostage):
        xp_cp = pltpu.make_async_copy(x_hbm.at[:, pl.ds(0, PRE), :], xp, sem_x.at[0])

        n_wo, wo_rows = wo.shape[0], ostage.shape[1]

        def wo_cp(p):
            return pltpu.make_async_copy(wo_hbm.at[pl.ds(pl.multiple_of(p * wo_rows, wo_rows), wo_rows), :],
                                         ostage.at[p % 2], sem_o.at[p % 2])

        def w_cps(t, g):
            return [pltpu.make_async_copy(w_hbms[t].at[:, pl.ds(pl.multiple_of(p * n_heads + g * WG, WG), WG), :],
                                          stage.at[t, pl.ds(0, D // 2), pl.ds(p * WG, WG), :], sem_stage.at[2 * t + p])
                    for p in range(2)]

        def relayout(t, c, part=0, n_part=1):
            nb_ = D // 2 // RB // n_part
            for b in range(nb_):
                rows = pl.ds(pl.multiple_of((part * nb_ + b) * RB, RB), RB)
                w = jnp.swapaxes(pltpu.bitcast(stage[t, rows], U32), 0, 1)
                for j in range(WG // 2):
                    even, odd = w[j], w[WG // 2 + j]
                    wqkv[c, rows, pl.ds(2 * j * dh, dh)] = (even & jnp.uint32(0xFFFF)) | (odd << 16)
                    wqkv[c, rows, pl.ds((2 * j + 1) * dh, dh)] = (even >> 16) | (odd & jnp.uint32(0xFFFF0000))

        xp_cp.start()
        start(w_cps(0, 0))
        wmod_cp(1, 1).start()
        wmod_cp(0, 0).start()
        ostage[2] = jnp.zeros(ostage.shape[1:], BF16)
        xp_cp.wait()
        nb = 64 // PRE

        @pl.loop(0, n_seg // nb)
        def _(i):
            xs = xp[pl.ds(i * nb, nb)].astype(F32).reshape(nb * PRE, D)
            pre[0, pl.ds(pl.multiple_of(i * nb * PRE, nb * PRE), nb * PRE), :] = _layernorm(xs)

        wait(w_cps(0, 0))

        @pl.loop(0, 8)
        def _(i):
            relayout(0, 0, i, 8)

        @pl.loop(0, 2)
        def _(i):
            wmod_cp(1 - i, 1 - i).wait()

            @pl.when(i == 0)
            def _():
                start(w_cps(1, 0))

            modulation(1 - i, 1 - i)

        start(w_cps(2, 0))

        @pl.loop(0, n_seg // nb)
        def _(i):
            ln = pre[0, pl.ds(pl.multiple_of(i * nb * PRE, nb * PRE), nb * PRE), :]
            rows = pl.ds(pl.multiple_of(i * (nb * PRE // 2), nb * PRE // 2), nb * PRE // 2)
            hp[rows, :] = _pack(ln * (1.0 + mod[1, 0:1, :]) + mod[0, 0:1, :])

        n_chunk = 3 * n_grp

        def pre_body(c, _):
            g = c // 3
            p = c - (n_chunk - n_wo)

            @pl.when(jnp.logical_and(p + 1 >= 0, p + 1 < n_wo))
            def _():
                wo_cp(p + 1).start()

            for t in range(3):
                @pl.when(c % 3 == t)
                def _():
                    @pl.when(g + 1 < n_grp)
                    def _():
                        start(w_cps(t, g + 1))

                    if t == 0:
                        @pl.when(g + 1 == n_grp)
                        def _():
                            x_cp.start()

                    if t < 2:
                        wait(w_cps(t + 1, g))
                    else:
                        @pl.when(g + 1 < n_grp)
                        def _():
                            wait(w_cps(0, g + 1))

                        wmod_cp(g + 2, g).start()

            @pl.when(p >= 0)
            def _():
                wo_cp(p).wait()

            nxt = jnp.minimum(c + 1, n_chunk - 1)
            for i in range(WG):
                cols = pl.ds(i * dh, dh)
                y = _dot(_unpack(hp[...]), _unpack(wqkv[c, :, cols]))
                relayout(nxt % 3, nxt, i * NSUB, WG * NSUB)
                for u in range(1, NSUB + (i + 1 < WG)):
                    r0 = (u - 1) * (n_seg * PRE // NSUB)
                    stage[nxt % 3, D // 2 + c // n_chunk] = y[r0:r0 + 2 * WG].astype(BF16)
                    if u < NSUB:
                        relayout(nxt % 3, nxt, i * NSUB + u, WG * NSUB)
                pre[c, :, cols] = y
                wr = wo_rows // WG
                wo[jnp.maximum(p, 0), pl.ds(i * wr // 2, wr // 2), :] = pltpu.bitcast(
                    ostage[jnp.where(p >= 0, p % 2, 2), pl.ds(i * wr, wr), :], U32)
            return 0

        with jax.named_scope('ph_pre'):
            jax.lax.fori_loop(0, n_chunk, pre_body, 0)

    pl.run_scoped(load_phase,
                  pltpu.VMEM((n_seg, PRE, D), BF16),
                  pltpu.VMEM((n_seg * PRE // 2, D), U32),
                  pltpu.VMEM((3, D // 2 + 1, 2 * WG, dh), BF16),
                  pltpu.VMEM((3, HG * dh, D), BF16))

    def main_phase(hn, att, st13, st2, w13, w2, abuf, xres, obuf):
        x_cp.wait()

        Dh2, Fh = D // 2, F // 2
        n_trip = n_seg // UNROLL
        r13, r2 = st13.shape[3], st2.shape[2]
        n2 = Fh // r2
        assert n_trip * r13 == Dh2 and n2 * r2 == Fh and n2 <= n_trip

        def ffn_w_cps(i):
            slot, i13, i2 = i % 2, jnp.minimum(i, n_trip - 1), jnp.minimum(i, n2 - 1)
            cps = [pltpu.make_async_copy(w_hbm.at[:, pl.ds(pl.multiple_of(i13 * r13, r13), r13), :],
                                         st13.at[slot, t], sem_ffn.at[slot * 3 + t])
                   for t, w_hbm in enumerate((w1_hbm, w3_hbm))]
            return cps + [pltpu.make_async_copy(w2_hbm.at[:, pl.ds(pl.multiple_of(i2 * r2, r2), r2), :],
                                                st2.at[slot], sem_ffn.at[slot * 3 + 2])]

        prep = ([(t, rb, cb) for t in range(2) for rb in range(r13 // 16) for cb in range(Fh // 128)]
                + [(2, rb, cb) for rb in range(r2 // 16) for cb in range(Dh2 // 128)])

        def ffn_w_prepare(i, part, anchor):
            t, rb, cb = prep[part]
            slot, spare = i % 2, 2 + i // n_trip
            src, cols = pl.ds(rb * 16, 16), pl.ds(cb * 128, 128)
            if t < 2:
                st13[spare, 0, 0, pl.ds(0, 16), pl.ds(0, 128)] = anchor
                b = [st13[slot, t, hf, src, pl.ds(p * Fh + cb * 128, 128)] for hf in range(2) for p in range(2)]
                rows = pl.ds(pl.multiple_of(i * (r13 // 2) + rb * 8, 8), 8)
                for k, w in enumerate(_strassen_rhs_packed(b)):
                    w13[t, k, rows, cols] = w
            else:
                st2[spare, 0, pl.ds(0, 16), pl.ds(0, 128)] = anchor
                b = [st2[slot, hf, src, pl.ds(p * Dh2 + cb * 128, 128)] for hf in range(2) for p in range(2)]
                rows = pl.ds(pl.multiple_of(jnp.minimum(i, n2 - 1) * (r2 // 2) + rb * 8, 8), 8)
                for k, w in enumerate(_strassen_rhs_packed(b)):
                    w2[k, rows, cols] = w

        start(ffn_w_cps(jnp.int32(0)))

        def ln1(s):
            hn[...] = ada_ln(x_buf[s, pl.ds(PRE, seg - PRE), :].astype(F32), 0)

        ln1(0)
        n_hg = n_heads // HG

        def seg_step(trip, u, mem):
            s = trip * UNROLL + u
            lhs = jnp.concatenate([mem, hn[...]], axis=0).astype(BF16)
            ln1(jnp.minimum(s + 1, n_seg - 1))
            qi = jax.lax.broadcasted_iota(jnp.int32, (L, L), 0)
            ki = jax.lax.broadcasted_iota(jnp.int32, (L, L), 1)
            mask = (qi < M) | (qi >= ki)
            pr = pl.ds(pl.multiple_of(s * PRE, PRE), PRE)

            def proj(t, g):
                gi, cols = g * HG // WG, pl.ds(g * HG % WG * dh, HG * dh)
                y = _dot(lhs, pltpu.bitcast(wqkv[3 * gi + t, :, cols], BF16))
                y = jnp.concatenate([y[:M], pre[3 * gi + t, pr, cols], y[M:]], axis=0)
                return [y[:, h * dh:(h + 1) * dh] for h in range(HG)]

            def probs(q, k):
                sc_ = jnp.where(mask, _dot_nt(q, k.astype(BF16)) * scale, -1e9)
                e = jnp.exp(sc_ - jnp.max(sc_, axis=-1, keepdims=True))
                return e, 1.0 / jnp.sum(e, axis=-1, keepdims=True)

            def mix(p, v):
                return jnp.concatenate([_dot(e, vh.astype(BF16)) * r for (e, r), vh in zip(p, v)], axis=1)

            def out_proj(o, g):
                y = _dot(o, _unpack(wo[g]))
                per = -(-len(prep) // (PREP_G * UNROLL))
                first = (u * PREP_G + g) * per
                for i in range(first, min(first + per, len(prep)) if g < PREP_G else 0):
                    n = (i - first) * (D // 128) // per
                    ffn_w_prepare(trip, i, y[:16, n * 128:(n + 1) * 128].astype(BF16))
                return y

            o, acc, p, v = {}, None, None, None
            done = 0
            for g in range(n_hg):
                q = proj(0, g)
                k = proj(1, g)
                if g == 1 and u == 0:
                    start(ffn_w_cps(trip + 1))
                if g:
                    o[g - 1] = mix(p, v)
                v = proj(2, g)
                p = [probs(qh, kh) for qh, kh in zip(q, k)]
                upto = g + 1 - LAG if g + 1 < n_hg else n_hg - 2
                while done < upto:
                    y = out_proj(o.pop(done), done)
                    acc = y if acc is None else acc + y
                    done += 1
            o[n_hg - 1] = mix(p, v)
            for g in range(done, n_hg):
                acc = acc + out_proj(o.pop(g), g)
            att[s] = acc[M:].astype(BF16)
            return acc[:M]

        def seg_body(trip, mem):
            wait(ffn_w_cps(trip))
            for u in range(UNROLL):
                mem = seg_step(trip, u, mem)
            return mem

        with jax.named_scope('ph_seg'):
            jax.lax.fori_loop(0, n_trip, seg_body, mem0_ref[...].astype(F32))

        wait(ffn_w_cps(jnp.int32(n_trip)))

        @pl.loop(0, 4)
        def _(j):
            wmod_cp(j + 2, j).wait()
            modulation(j + 2, j)

        sb = FFN_TM // seg

        hm = FFN_TM // 2

        def ffn_lhs(i, row, n, zero=0):
            hs = []
            for hf in range(2):
                sg, rows = i * sb + hf * sb // 2 + row // seg, pl.ds(row % seg if n < seg else 0, n)
                xn = x_buf[sg, rows, :].astype(F32) + mod[2, 0:1, :] * att[sg, rows, :].astype(F32)
                xres[i % 2, pl.ds(hf * hm + row, n), :] = xn
                hs.append(ada_ln(xn, 3))
            top, bot = hs
            for j, a in enumerate(_strassen_lhs(top[:, :Dh2], top[:, Dh2:], bot[:, :Dh2], bot[:, Dh2:])):
                abuf[j + zero, pl.ds(row, n), pl.ds(Fh, Dh2)] = a

        @pl.loop(0, hm // seg)
        def _(j):
            ffn_lhs(0, pl.multiple_of(j * seg, seg), seg)

        def out_cp(i):
            return pltpu.make_async_copy(obuf.at[i % 2], out_hbm.at[pl.ds(i * FFN_TM, FFN_TM), :], sem_out.at[i % 2])

        n_blk = S // FFN_TM

        def ffn_body(i, _):
            @pl.when(i >= 2)
            def _():
                out_cp(i - 2).wait()

            for j in range(Fh // FFN_TF):
                cols = pl.ds(j * FFN_TF, FFN_TF)
                gu = []
                for t in range(2):
                    gu.append(_strassen_out([_dot(abuf[k, :, pl.ds(Fh, Dh2)], _unpack(w13[t, k, :, cols])) for k in range(7)]))
                gate, up = gu
                act = [g * jax.nn.sigmoid(g) * u for g, u in zip(gate, up)]
                for k, a in enumerate(_strassen_lhs(*act)):
                    abuf[k, :, cols] = a
            m, nn = [], Dh2 // DN
            for k in range(7):
                mk = []
                for n in range(nn):
                    mk.append(_dot(abuf[k, :, pl.ds(0, Fh)], _unpack(w2[k, :, pl.ds(n * DN, DN)])))
                    part = k * nn + n - LHS_K
                    if 0 <= part < hm // LR:
                        ffn_lhs(jnp.minimum(i + 1, n_blk - 1), part * LR, LR, i // n_blk)
                    if 0 <= part + 1 < hm // LR:
                        att[n_seg + i // n_blk, pl.ds(0, 16), pl.ds(0, 128)] = mk[n][:16, :128].astype(BF16)
                m.append(jnp.concatenate(mk, axis=1))
            y = _strassen_out(m)
            y = jnp.concatenate([jnp.concatenate(y[:2], axis=1), jnp.concatenate(y[2:], axis=1)], axis=0)
            obuf[i % 2] = (xres[i % 2] + mod[5, 0:1, :] * y).astype(obuf.dtype)
            out_cp(i).start()
            return 0

        with jax.named_scope('ph_ffn'):
            jax.lax.fori_loop(0, n_blk, ffn_body, 0)
        for i in range(max(n_blk - 2, 0), n_blk):
            out_cp(i).wait()

    pl.run_scoped(main_phase,
                  pltpu.VMEM((seg - PRE, D), F32),
                  pltpu.VMEM((n_seg + 1, seg, D), BF16),
                  pltpu.VMEM((3, 2, 2, 8 * UNROLL, F), BF16),
                  pltpu.VMEM((3, 2, 32 * UNROLL, D), BF16),
                  pltpu.VMEM((2, 7, D // 4, F // 2), U32),
                  pltpu.VMEM((7, F // 4, D // 2), U32),
                  pltpu.VMEM((7, FFN_TM // 2, F // 2 + D // 2), F32),
                  pltpu.VMEM((2, FFN_TM, D), F32),
                  pltpu.VMEM((2, FFN_TM, D), out_hbm.dtype))


@functools.partial(jax.jit, static_argnames=("A_seg_len",))
def pallas_adaLN_cond__memory_aug_recurrent_mem_tr__glu_gated_swiglu__prompt_kernel(
    A_x, A_mem0, A_Wq, A_Wk, A_Wv, A_Wo, A_seg_len, B_x, B_w1, B_w3, B_w2, c, w_mod,
):
    del B_x
    B, S, D = A_x.shape
    assert B == 1
    M = A_mem0.shape[1]
    _, H, Dh = A_Wq.shape
    F = B_w1.shape[1]
    seg = int(A_seg_len)
    n_seg, n_grp = S // seg, H // WG
    any_spec = pl.BlockSpec(memory_space=pl.ANY)
    vmem_spec = pl.BlockSpec(memory_space=pltpu.VMEM)
    out = pl.pallas_call(
        functools.partial(_kernel, n_heads=H, dh=Dh),
        out_shape=jax.ShapeDtypeStruct((S, D), A_x.dtype),
        in_specs=[any_spec, vmem_spec] + [any_spec] * 7 + [vmem_spec, any_spec],
        out_specs=any_spec,
        scratch_shapes=[
            pltpu.VMEM((n_seg, seg, D), BF16),
            pltpu.VMEM((3 * n_grp, D // 2, WG * Dh), U32),
            pltpu.VMEM((H // HG, HG * Dh // 2, D), U32),
            pltpu.VMEM((3 * n_grp, n_seg * PRE, WG * Dh), F32),
            pltpu.VMEM((6, 8, D), F32),
            pltpu.VMEM((4, D, D), BF16),
            pltpu.SemaphoreType.DMA((2,)),
            pltpu.SemaphoreType.DMA((6,)),
            pltpu.SemaphoreType.DMA((4,)),
            pltpu.SemaphoreType.DMA((2,)),
            pltpu.SemaphoreType.DMA((6,)),
            pltpu.SemaphoreType.DMA((2,)),
        ],
        compiler_params=pltpu.CompilerParams(vmem_limit_bytes=127 * 1024 * 1024),
    )(
        A_x.reshape(n_seg, seg, D), A_mem0.reshape(M, D),
        A_Wq.reshape(D // 2, 2 * H, Dh), A_Wk.reshape(D // 2, 2 * H, Dh), A_Wv.reshape(D // 2, 2 * H, Dh),
        A_Wo.reshape(H * Dh, D),
        B_w1.reshape(2, D // 2, F), B_w3.reshape(2, D // 2, F), B_w2.reshape(2, F // 2, D), c, w_mod,
    )
    return out.reshape(B, S, D)
```

```python
import functools

import jax
import jax.numpy as jnp
import jax.experimental.pallas as pl
import jax.experimental.pallas.tpu as pltpu

F32 = jnp.float32
BF16 = jnp.bfloat16
U32 = jnp.uint32
LOG2E = 1.4426950408889634

PRE = 8
WG = 8
LAG = 3
LHS_K = 2
DN = 128
MOD_AT = 4
NSUB = 4
LR = 8
PREP_G = 6
RB = 8
UNROLL = 2
HG = 4
FFN_TM = 256
FFN_TF = 128


def _dot(a, b):
    return jax.lax.dot_general(a, b, (((1,), (0,)), ((), ())), preferred_element_type=F32)


def _dot_nt(a, b):
    return jax.lax.dot_general(a, b, (((1,), (1,)), ((), ())), preferred_element_type=F32)


def _round_bf16(x):
    return x.astype(BF16).astype(F32)


def _layernorm(x):
    m = jnp.mean(x, axis=-1, keepdims=True)
    d = x - m
    v = jnp.mean(d * d, axis=-1, keepdims=True)
    return d * jax.lax.rsqrt(v + 1e-5)


def _pack(x):
    return pltpu.bitcast(x.astype(BF16), U32)


def _unpack(w):
    return pltpu.bitcast(w, BF16)


def _strassen_lhs(a11, a12, a21, a22):
    return (a11 + a22, a21 + a22, a11, a22, a11 + a12, a21 - a11, a12 - a22)


def _strassen_rhs(b11, b12, b21, b22):
    return (b11 + b22, b11, b12 - b22, b21 - b11, b22, b11 + b12, b21 + b22)


def _strassen_rhs_packed(blocks):
    words = [pltpu.bitcast(b, U32) for b in blocks]
    even = _strassen_rhs(*[pltpu.bitcast(w << 16, F32) for w in words])
    odd = _strassen_rhs(*[pltpu.bitcast(w & jnp.uint32(0xFFFF0000), F32) for w in words])
    out = [pltpu.pack_elementwise([e, o], packed_dtype=BF16) for e, o in zip(even, odd)]
    out[1], out[4] = words[0], words[3]
    return out


def _strassen_out(m):
    return (m[0] + m[3] - m[4] + m[6], m[2] + m[4], m[1] + m[3], m[0] - m[1] + m[2] + m[5])


def _kernel(x_hbm, mem0_ref, wq_hbm, wk_hbm, wv_hbm, wo_hbm, w1_hbm, w3_hbm, w2_hbm, c_ref, wmod_hbm,
            out_hbm,
            x_buf, wqkv, wo, pre, mod, sem_x, sem_stage, sem_m, sem_o, sem_ffn, sem_out, *, n_heads, dh):
    n_seg, seg, D = x_buf.shape
    S = n_seg * seg
    M = mem0_ref.shape[0]
    L = M + seg
    scale = dh ** -0.5
    F = w1_hbm.shape[2]
    n_grp = n_heads // WG
    w_hbms = (wq_hbm, wk_hbm, wv_hbm)

    x_cp = pltpu.make_async_copy(x_hbm, x_buf, sem_x.at[1])

    def start(cps):
        for cp in cps:
            cp.start()

    def wait(cps):
        for cp in cps:
            cp.wait()

    def mod_row(j):
        return jnp.concatenate([mod[j * (D // 128) + n, 0:1, :] for n in range(D // 128)], axis=1)

    def ada_ln(x, j):
        return _layernorm(x) * (1.0 + mod_row(j + 1)) + mod_row(j)

    cc = c_ref[...].astype(F32)
    sc = jnp.broadcast_to(cc * jax.nn.sigmoid(cc), (16, D)).astype(BF16)

    def load_phase(xp, hp, stage, ostage, mstage):
        xp_cp = pltpu.make_async_copy(x_hbm.at[:, pl.ds(0, PRE), :], xp, sem_x.at[0])

        n_mod, _, mod_cols = mstage.shape

        def wmod_cp(j):
            return pltpu.make_async_copy(wmod_hbm.at[:, pl.ds(pl.multiple_of(j * mod_cols, mod_cols), mod_cols)],
                                         mstage.at[j], sem_m.at[j])

        n_wo, wo_rows = wo.shape[0], ostage.shape[1]

        def wo_cp(p):
            return pltpu.make_async_copy(wo_hbm.at[pl.ds(pl.multiple_of(p * wo_rows, wo_rows), wo_rows), :],
                                         ostage.at[p % 2], sem_o.at[p % 2])

        def w_cps(t, g):
            return [pltpu.make_async_copy(w_hbms[t].at[:, pl.ds(pl.multiple_of(p * n_heads + g * WG, WG), WG), :],
                                          stage.at[t, pl.ds(0, D // 2), pl.ds(p * WG, WG), :], sem_stage.at[2 * t + p])
                    for p in range(2)]

        def relayout(t, c, part=0, n_part=1):
            nb_ = D // 2 // RB // n_part
            for b in range(nb_):
                rows = pl.ds(pl.multiple_of((part * nb_ + b) * RB, RB), RB)
                w = jnp.swapaxes(pltpu.bitcast(stage[t, rows], U32), 0, 1)
                for j in range(WG // 2):
                    even, odd = w[j], w[WG // 2 + j]
                    wqkv[c, rows, pl.ds(2 * j * dh, dh)] = (even & jnp.uint32(0xFFFF)) | (odd << 16)
                    wqkv[c, rows, pl.ds((2 * j + 1) * dh, dh)] = (even >> 16) | (odd & jnp.uint32(0xFFFF0000))

        xp_cp.start()
        start(w_cps(0, 0))
        wmod_cp(0).start()
        ostage[2] = jnp.zeros(ostage.shape[1:], BF16)
        xp_cp.wait()
        for j in range(1, n_mod):
            wmod_cp(j).start()
        nb = 64 // PRE

        @pl.loop(0, n_seg // nb)
        def _(i):
            xs = xp[pl.ds(i * nb, nb)].astype(F32).reshape(nb * PRE, D)
            pre[0, pl.ds(pl.multiple_of(i * nb * PRE, nb * PRE), nb * PRE), :] = _layernorm(xs)

        wait(w_cps(0, 0))

        @pl.loop(0, 8)
        def _(i):
            relayout(0, 0, i, 8)

        start(w_cps(1, 0))

        @pl.loop(0, n_mod)
        def _(j):
            wmod_cp(j).wait()
            y = _dot(sc, mstage[j])
            for n in range(mod_cols // 128):
                mod[j * (mod_cols // 128) + n] = y[:8, n * 128:(n + 1) * 128]

        start(w_cps(2, 0))

        @pl.loop(0, n_seg // nb)
        def _(i):
            ln = pre[0, pl.ds(pl.multiple_of(i * nb * PRE, nb * PRE), nb * PRE), :]
            rows = pl.ds(pl.multiple_of(i * (nb * PRE // 2), nb * PRE // 2), nb * PRE // 2)
            hp[rows, :] = _pack(ln * (1.0 + mod_row(1)) + mod_row(0))

        n_chunk = 3 * n_grp

        def pre_body(c, _):
            g = c // 3
            p = c - (n_chunk - n_wo)

            @pl.when(jnp.logical_and(p + 1 >= 0, p + 1 < n_wo))
            def _():
                wo_cp(p + 1).start()

            for t in range(3):
                @pl.when(c % 3 == t)
                def _():
                    @pl.when(g + 1 < n_grp)
                    def _():
                        start(w_cps(t, g + 1))

                    if t == 0:
                        @pl.when(g + 1 == n_grp)
                        def _():
                            x_cp.start()

                    if t < 2:
                        wait(w_cps(t + 1, g))
                    else:
                        @pl.when(g + 1 < n_grp)
                        def _():
                            wait(w_cps(0, g + 1))


            @pl.when(p >= 0)
            def _():
                wo_cp(p).wait()

            nxt = jnp.minimum(c + 1, n_chunk - 1)
            for i in range(WG):
                cols = pl.ds(i * dh, dh)
                y = _dot(_unpack(hp[...]), _unpack(wqkv[c, :, cols]))
                relayout(nxt % 3, nxt, i * NSUB, WG * NSUB)
                for u in range(1, NSUB + (i + 1 < WG)):
                    r0 = (u - 1) * (n_seg * PRE // NSUB)
                    stage[nxt % 3, D // 2 + c // n_chunk] = y[r0:r0 + 2 * WG].astype(BF16)
                    if u < NSUB:
                        relayout(nxt % 3, nxt, i * NSUB + u, WG * NSUB)
                pre[c, :, cols] = y
                wr = wo_rows // WG
                wo[jnp.maximum(p, 0), pl.ds(i * wr // 2, wr // 2), :] = pltpu.bitcast(
                    ostage[jnp.where(p >= 0, p % 2, 2), pl.ds(i * wr, wr), :], U32)
            return 0

        with jax.named_scope('ph_pre'):
            jax.lax.fori_loop(0, n_chunk, pre_body, 0)

    pl.run_scoped(load_phase,
                  pltpu.VMEM((n_seg, PRE, D), BF16),
                  pltpu.VMEM((n_seg * PRE // 2, D), U32),
                  pltpu.VMEM((3, D // 2 + 1, 2 * WG, dh), BF16),
                  pltpu.VMEM((3, HG * dh, D), BF16),
                  pltpu.VMEM((4, D, 2 * D // 4), BF16))

    def main_phase(hn, att, st13, st2, stm, w13, w2, abuf, xres, obuf):
        x_cp.wait()

        Dh2, Fh = D // 2, F // 2
        n_trip = n_seg // UNROLL
        r13, r2 = st13.shape[3], st2.shape[2]
        n2 = Fh // r2
        assert n_trip * r13 == Dh2 and n2 * r2 == Fh and n2 <= n_trip and n_trip * 128 == 4 * D

        def ffn_w_cps(i):
            slot, i13, i2 = i % 2, jnp.minimum(i, n_trip - 1), jnp.minimum(i, n2 - 1)
            cps = [pltpu.make_async_copy(w_hbm.at[:, pl.ds(pl.multiple_of(i13 * r13, r13), r13), :],
                                         st13.at[slot, t], sem_ffn.at[slot * 4 + t])
                   for t, w_hbm in enumerate((w1_hbm, w3_hbm))]
            return cps + [pltpu.make_async_copy(w2_hbm.at[:, pl.ds(pl.multiple_of(i2 * r2, r2), r2), :],
                                                st2.at[slot], sem_ffn.at[slot * 4 + 2]),
                          pltpu.make_async_copy(wmod_hbm.at[:, pl.ds(pl.multiple_of(2 * D + i13 * 128, 128), 128)],
                                                stm.at[slot], sem_ffn.at[slot * 4 + 3])]

        prep = ([(t, rb, cb) for t in range(2) for rb in range(r13 // 16) for cb in range(Fh // 128)]
                + [(2, rb, cb) for rb in range(r2 // 16) for cb in range(Dh2 // 128)])

        def ffn_w_prepare(i, part, anchor):
            t, rb, cb = prep[part]
            slot, spare = i % 2, 2 + i // n_trip
            src, cols = pl.ds(rb * 16, 16), pl.ds(cb * 128, 128)
            if t < 2:
                st13[spare, 0, 0, pl.ds(0, 16), pl.ds(0, 128)] = anchor
                b = [st13[slot, t, hf, src, pl.ds(p * Fh + cb * 128, 128)] for hf in range(2) for p in range(2)]
                rows = pl.ds(pl.multiple_of(i * (r13 // 2) + rb * 8, 8), 8)
                for k, w in enumerate(_strassen_rhs_packed(b)):
                    w13[t, k, rows, cols] = w
            else:
                st2[spare, 0, pl.ds(0, 16), pl.ds(0, 128)] = anchor
                b = [st2[slot, hf, src, pl.ds(p * Dh2 + cb * 128, 128)] for hf in range(2) for p in range(2)]
                rows = pl.ds(pl.multiple_of(jnp.minimum(i, n2 - 1) * (r2 // 2) + rb * 8, 8), 8)
                for k, w in enumerate(_strassen_rhs_packed(b)):
                    w2[k, rows, cols] = w

        start(ffn_w_cps(jnp.int32(0)))

        def ln1(s):
            hn[...] = ada_ln(x_buf[s, pl.ds(PRE, seg - PRE), :].astype(F32), 0)

        ln1(0)
        n_hg = n_heads // HG

        def seg_step(trip, u, mem):
            s = trip * UNROLL + u
            lhs = jnp.concatenate([mem, hn[...]], axis=0).astype(BF16)
            ln1(jnp.minimum(s + 1, n_seg - 1))
            qi = jax.lax.broadcasted_iota(jnp.int32, (L, L), 0)
            ki = jax.lax.broadcasted_iota(jnp.int32, (L, L), 1)
            mask = (qi < M) | (qi >= ki)
            pr = pl.ds(pl.multiple_of(s * PRE, PRE), PRE)

            def proj(t, g):
                gi, cols = g * HG // WG, pl.ds(g * HG % WG * dh, HG * dh)
                y = _dot(lhs, pltpu.bitcast(wqkv[3 * gi + t, :, cols], BF16))
                y = jnp.concatenate([y[:M], pre[3 * gi + t, pr, cols], y[M:]], axis=0)
                return [y[:, h * dh:(h + 1) * dh] for h in range(HG)]

            def probs(q, k):
                sc_ = jnp.where(mask, _dot_nt(q, k.astype(BF16)) * (scale * LOG2E), -1e9 * LOG2E)
                e = jnp.exp2(sc_ - jnp.max(sc_, axis=-1, keepdims=True))
                den = jnp.sum(e, axis=-1, keepdims=True)
                r = pl.reciprocal(den, approx=True)
                return e, r * (2.0 - den * r)

            def mix(p, v):
                return jnp.concatenate([_dot(e, vh.astype(BF16)) * r for (e, r), vh in zip(p, v)], axis=1)

            def out_proj(o, g):
                y = _dot(o, _unpack(wo[g]))
                per = -(-len(prep) // (PREP_G * UNROLL))
                first = (u * PREP_G + g) * per
                for i in range(first, min(first + per, len(prep)) if g < PREP_G else 0):
                    n = (i - first) * (D // 128) // per
                    ffn_w_prepare(trip, i, y[:16, n * 128:(n + 1) * 128].astype(BF16))
                return y

            o, acc, p, v = {}, None, None, None
            done = 0
            for g in range(n_hg):
                q = proj(0, g)
                k = proj(1, g)
                if g == 1 and u == 0:
                    start(ffn_w_cps(trip + 1))
                if g:
                    o[g - 1] = mix(p, v)
                v = proj(2, g)
                p = [probs(qh, kh) for qh, kh in zip(q, k)]
                upto = g + 1 - LAG if g + 1 < n_hg else n_hg - 2
                while done < upto:
                    y = out_proj(o.pop(done), done)
                    acc = y if acc is None else acc + y
                    if done == MOD_AT and u == UNROLL - 1:
                        mod[2 * D // 128 + trip] = _dot(sc, stm[trip % 2])[:8]
                    done += 1
            o[n_hg - 1] = mix(p, v)
            for g in range(done, n_hg):
                acc = acc + out_proj(o.pop(g), g)
            att[s] = acc[M:].astype(BF16)
            return acc[:M]

        def seg_body(trip, mem):
            wait(ffn_w_cps(trip))
            for u in range(UNROLL):
                mem = seg_step(trip, u, mem)
            return mem

        with jax.named_scope('ph_seg'):
            jax.lax.fori_loop(0, n_trip, seg_body, mem0_ref[...].astype(F32))

        wait(ffn_w_cps(jnp.int32(n_trip)))

        sb = FFN_TM // seg

        hm = FFN_TM // 2

        def ffn_lhs(i, row, n, zero=0):
            hs = []
            for hf in range(2):
                sg, rows = i * sb + hf * sb // 2 + row // seg, pl.ds(row % seg if n < seg else 0, n)
                xn = x_buf[sg, rows, :].astype(F32) + mod_row(2) * att[sg, rows, :].astype(F32)
                xres[i % 2, pl.ds(hf * hm + row, n), :] = xn
                hs.append(ada_ln(xn, 3))
            top, bot = hs
            for j, a in enumerate(_strassen_lhs(top[:, :Dh2], top[:, Dh2:], bot[:, :Dh2], bot[:, Dh2:])):
                abuf[j + zero, pl.ds(row, n), pl.ds(Fh, Dh2)] = a

        @pl.loop(0, hm // seg)
        def _(j):
            ffn_lhs(0, pl.multiple_of(j * seg, seg), seg)

        def out_cp(i):
            return pltpu.make_async_copy(obuf.at[i % 2], out_hbm.at[pl.ds(i * FFN_TM, FFN_TM), :], sem_out.at[i % 2])

        n_blk = S // FFN_TM

        def ffn_body(i, _):
            @pl.when(i >= 2)
            def _():
                out_cp(i - 2).wait()

            for j in range(Fh // FFN_TF):
                cols = pl.ds(j * FFN_TF, FFN_TF)
                gu = []
                for t in range(2):
                    gu.append(_strassen_out([_dot(abuf[k, :, pl.ds(Fh, Dh2)], _unpack(w13[t, k, :, cols])) for k in range(7)]))
                gate, up = gu
                act = [g * jax.nn.sigmoid(g) * u for g, u in zip(gate, up)]
                for k, a in enumerate(_strassen_lhs(*act)):
                    abuf[k, :, cols] = a
            m, nn = [], Dh2 // DN
            for k in range(7):
                mk = []
                for n in range(nn):
                    mk.append(_dot(abuf[k, :, pl.ds(0, Fh)], _unpack(w2[k, :, pl.ds(n * DN, DN)])))
                    part = k * nn + n - LHS_K
                    if 0 <= part < hm // LR:
                        ffn_lhs(jnp.minimum(i + 1, n_blk - 1), part * LR, LR, i // n_blk)
                    if 0 <= part + 1 < hm // LR:
                        att[n_seg + i // n_blk, pl.ds(0, 16), pl.ds(0, 128)] = mk[n][:16, :128].astype(BF16)
                m.append(jnp.concatenate(mk, axis=1))
            y = _strassen_out(m)
            y = jnp.concatenate([jnp.concatenate(y[:2], axis=1), jnp.concatenate(y[2:], axis=1)], axis=0)
            obuf[i % 2] = (xres[i % 2] + mod_row(5) * y).astype(obuf.dtype)
            out_cp(i).start()
            return 0

        with jax.named_scope('ph_ffn'):
            jax.lax.fori_loop(0, n_blk, ffn_body, 0)
        for i in range(max(n_blk - 2, 0), n_blk):
            out_cp(i).wait()

    pl.run_scoped(main_phase,
                  pltpu.VMEM((seg - PRE, D), F32),
                  pltpu.VMEM((n_seg + 1, seg, D), BF16),
                  pltpu.VMEM((3, 2, 2, 8 * UNROLL, F), BF16),
                  pltpu.VMEM((3, 2, 32 * UNROLL, D), BF16),
                  pltpu.VMEM((2, D, 128), BF16),
                  pltpu.VMEM((2, 7, D // 4, F // 2), U32),
                  pltpu.VMEM((7, F // 4, D // 2), U32),
                  pltpu.VMEM((7, FFN_TM // 2, F // 2 + D // 2), F32),
                  pltpu.VMEM((2, FFN_TM, D), F32),
                  pltpu.VMEM((2, FFN_TM, D), out_hbm.dtype))


@functools.partial(jax.jit, static_argnames=("A_seg_len",))
def pallas_adaLN_cond__memory_aug_recurrent_mem_tr__glu_gated_swiglu__prompt_kernel(
    A_x, A_mem0, A_Wq, A_Wk, A_Wv, A_Wo, A_seg_len, B_x, B_w1, B_w3, B_w2, c, w_mod,
):
    del B_x
    B, S, D = A_x.shape
    assert B == 1
    M = A_mem0.shape[1]
    _, H, Dh = A_Wq.shape
    F = B_w1.shape[1]
    seg = int(A_seg_len)
    n_seg, n_grp = S // seg, H // WG
    any_spec = pl.BlockSpec(memory_space=pl.ANY)
    vmem_spec = pl.BlockSpec(memory_space=pltpu.VMEM)
    out = pl.pallas_call(
        functools.partial(_kernel, n_heads=H, dh=Dh),
        out_shape=jax.ShapeDtypeStruct((S, D), A_x.dtype),
        in_specs=[any_spec, vmem_spec] + [any_spec] * 7 + [vmem_spec, any_spec],
        out_specs=any_spec,
        scratch_shapes=[
            pltpu.VMEM((n_seg, seg, D), BF16),
            pltpu.VMEM((3 * n_grp, D // 2, WG * Dh), U32),
            pltpu.VMEM((H // HG, HG * Dh // 2, D), U32),
            pltpu.VMEM((3 * n_grp, n_seg * PRE, WG * Dh), F32),
            pltpu.VMEM((6 * D // 128, 8, 128), F32),
            pltpu.SemaphoreType.DMA((2,)),
            pltpu.SemaphoreType.DMA((6,)),
            pltpu.SemaphoreType.DMA((4,)),
            pltpu.SemaphoreType.DMA((2,)),
            pltpu.SemaphoreType.DMA((8,)),
            pltpu.SemaphoreType.DMA((2,)),
        ],
        compiler_params=pltpu.CompilerParams(vmem_limit_bytes=127 * 1024 * 1024),
    )(
        A_x.reshape(n_seg, seg, D), A_mem0.reshape(M, D),
        A_Wq.reshape(D // 2, 2 * H, Dh), A_Wk.reshape(D // 2, 2 * H, Dh), A_Wv.reshape(D // 2, 2 * H, Dh),
        A_Wo.reshape(H * Dh, D),
        B_w1.reshape(2, D // 2, F), B_w3.reshape(2, D // 2, F), B_w2.reshape(2, F // 2, D), c, w_mod,
    )
    return out.reshape(B, S, D)
```

```python
import functools

import jax
import jax.numpy as jnp
import jax.experimental.pallas as pl
import jax.experimental.pallas.tpu as pltpu

F32 = jnp.float32
BF16 = jnp.bfloat16
U32 = jnp.uint32
LOG2E = 1.4426950408889634

PRE = 8
WG = 8
LAG = 4
EVERY = 1
FIRST = 4
SPLIT = 1
MOD_AT = 4
NSUB = 4
PREP_G = 7
RB = 8
UNROLL = 2
HG = 4
FFN_TM = 256
FFN_TF = 128


def _dot(a, b):
    return jax.lax.dot_general(a, b, (((1,), (0,)), ((), ())), preferred_element_type=F32)


def _dot_nt(a, b):
    return jax.lax.dot_general(a, b, (((1,), (1,)), ((), ())), preferred_element_type=F32)


def _round_bf16(x):
    return x.astype(BF16).astype(F32)


def _silu(x):
    t = 0.5 * x
    return t * jnp.tanh(t) + t


def _layernorm(x):
    m = jnp.mean(x, axis=-1, keepdims=True)
    d = x - m
    v = jnp.mean(d * d, axis=-1, keepdims=True)
    return d * jax.lax.rsqrt(v + 1e-5)


def _pack(x):
    return pltpu.bitcast(x.astype(BF16), U32)


def _unpack(w):
    return pltpu.bitcast(w, BF16)


def _low_half(w):
    return pltpu.bitcast(w << 16, F32)


def _high_half(w):
    return pltpu.bitcast(w & jnp.uint32(0xFFFF0000), F32)


def _strassen_lhs(a11, a12, a21, a22):
    return (a11 + a22, a21 + a22, a11, a22, a11 + a12, a21 - a11, a12 - a22)


def _strassen_rhs(b11, b12, b21, b22):
    return (b11 + b22, b11, b12 - b22, b21 - b11, b22, b11 + b12, b21 + b22)


def _strassen_out(m):
    return (m[0] + m[3] - m[4] + m[6], m[2] + m[4], m[1] + m[3], m[0] - m[1] + m[2] + m[5])


def _operands(level, x):
    outer = [level(x[r][c], x[r][c + 2], x[r + 2][c], x[r + 2][c + 2]) for r in range(2) for c in range(2)]
    return [y for i in range(7) for y in level(*[o[i] for o in outer])]


def _results(product):
    inner = [_strassen_out([product(7 * i + j) for j in range(7)]) for i in range(7)]
    outer = [_strassen_out([m[rc] for m in inner]) for rc in range(4)]
    return [[outer[r % 2 * 2 + c % 2][r // 2 * 2 + c // 2] for c in range(4)] for r in range(4)]


def _weight_operands(blocks):
    words = [[pltpu.bitcast(b, U32) for b in row] for row in blocks]
    even = _operands(_strassen_rhs, [[_low_half(w) for w in row] for row in words])
    odd = _operands(_strassen_rhs, [[_high_half(w) for w in row] for row in words])
    return [pltpu.pack_elementwise([e, o], packed_dtype=BF16) for e, o in zip(even, odd)]


def _kernel(x_hbm, mem0_ref, wq_hbm, wk_hbm, wv_hbm, wo_hbm, w1_hbm, w3_hbm, w2_hbm, c_ref, wmod_hbm,
            out_hbm,
            x_buf, wqkv, wo, pre, mod, sem_x, sem_stage, sem_m, sem_o, sem_ffn, sem_out, *, n_heads, dh):
    n_trip, _, seg, D = x_buf.shape
    n_seg = 2 * n_trip
    S = n_seg * seg
    M = mem0_ref.shape[0]
    L = M + seg
    scale = dh ** -0.5
    F = w1_hbm.shape[2]
    n_grp = n_heads // WG
    w_hbms = (wq_hbm, wk_hbm, wv_hbm)

    x_cp = pltpu.make_async_copy(x_hbm, x_buf, sem_x.at[2])

    def start(cps):
        for cp in cps:
            cp.start()

    def wait(cps):
        for cp in cps:
            cp.wait()

    def mod_row(j):
        return jnp.concatenate([mod[j * (D // 128) + n, 0:1, :] for n in range(D // 128)], axis=1)

    def ada_ln(x, j):
        return _layernorm(x) * (1.0 + mod_row(j + 1)) + mod_row(j)

    cc = c_ref[...].astype(F32)
    sc = jnp.broadcast_to(cc * jax.nn.sigmoid(cc), (16, D)).astype(BF16)

    def load_phase(xp, lnp, hp, stage, ostage, mstage):
        xp_cps = [pltpu.make_async_copy(x_hbm.at[:, u, pl.ds(0, PRE), :], xp.at[pl.ds(u * n_trip, n_trip)],
                                        sem_x.at[u]) for u in range(2)]

        n_mod, _, mod_cols = mstage.shape

        def wmod_cp(j):
            return pltpu.make_async_copy(wmod_hbm.at[:, pl.ds(pl.multiple_of(j * mod_cols, mod_cols), mod_cols)],
                                         mstage.at[j], sem_m.at[j])

        n_wo, wo_rows = wo.shape[0], ostage.shape[1]

        def wo_cp(p):
            return pltpu.make_async_copy(wo_hbm.at[pl.ds(pl.multiple_of(p * wo_rows, wo_rows), wo_rows), :],
                                         ostage.at[p % 2], sem_o.at[p % 2])

        def w_cps(t, g):
            return [pltpu.make_async_copy(w_hbms[t].at[:, pl.ds(pl.multiple_of(p * n_heads + g * WG, WG), WG), :],
                                          stage.at[t, pl.ds(0, D // 2), pl.ds(p * WG, WG), :], sem_stage.at[2 * t + p])
                    for p in range(2)]

        def relayout(t, c, part=0, n_part=1):
            nb_ = D // 2 // RB // n_part
            for b in range(nb_):
                rows = pl.ds(pl.multiple_of((part * nb_ + b) * RB, RB), RB)
                w = jnp.swapaxes(pltpu.bitcast(stage[t, rows], U32), 0, 1)
                for j in range(WG // 2):
                    even, odd = w[j], w[WG // 2 + j]
                    wqkv[c, rows, pl.ds(2 * j * dh, dh)] = (even & jnp.uint32(0xFFFF)) | (odd << 16)
                    wqkv[c, rows, pl.ds((2 * j + 1) * dh, dh)] = (even >> 16) | (odd & jnp.uint32(0xFFFF0000))

        start(xp_cps)
        start(w_cps(0, 0))
        wmod_cp(0).start()
        ostage[2] = jnp.zeros(ostage.shape[1:], BF16)
        wait(xp_cps)
        for j in range(1, n_mod):
            wmod_cp(j).start()
        nb = 64 // PRE

        @pl.loop(0, n_seg // nb)
        def _(i):
            xs = xp[pl.ds(i * nb, nb)].astype(F32).reshape(nb * PRE, D)
            lnp[pl.ds(pl.multiple_of(i * nb * PRE, nb * PRE), nb * PRE), :] = _layernorm(xs)

        wait(w_cps(0, 0))

        @pl.loop(0, 8)
        def _(i):
            relayout(0, 0, i, 8)

        start(w_cps(1, 0))

        @pl.loop(0, n_mod)
        def _(j):
            wmod_cp(j).wait()
            y = _dot(sc, mstage[j])
            for n in range(mod_cols // 128):
                mod[j * (mod_cols // 128) + n] = y[:8, n * 128:(n + 1) * 128]

        start(w_cps(2, 0))

        @pl.loop(0, n_seg // nb)
        def _(i):
            ln = lnp[pl.ds(pl.multiple_of(i * nb * PRE, nb * PRE), nb * PRE), :]
            rows = pl.ds(pl.multiple_of(i * (nb * PRE // 2), nb * PRE // 2), nb * PRE // 2)
            hp[rows, :] = _pack(ln * (1.0 + mod_row(1)) + mod_row(0))

        n_chunk = 3 * n_grp

        def pre_body(c, _):
            g = c // 3
            p = c - (n_chunk - n_wo)

            @pl.when(jnp.logical_and(p + 1 >= 0, p + 1 < n_wo))
            def _():
                wo_cp(p + 1).start()

            for t in range(3):
                @pl.when(c % 3 == t)
                def _():
                    @pl.when(g + 1 < n_grp)
                    def _():
                        start(w_cps(t, g + 1))

                    if t == 0:
                        @pl.when(g + 1 == n_grp)
                        def _():
                            x_cp.start()

                    if t < 2:
                        wait(w_cps(t + 1, g))
                    else:
                        @pl.when(g + 1 < n_grp)
                        def _():
                            wait(w_cps(0, g + 1))


            @pl.when(p >= 0)
            def _():
                wo_cp(p).wait()

            nxt = jnp.minimum(c + 1, n_chunk - 1)
            for i in range(WG):
                cols = pl.ds(i * dh, dh)
                y = _dot(_unpack(hp[...]), _unpack(wqkv[c, :, cols]))
                relayout(nxt % 3, nxt, i * NSUB, WG * NSUB)
                for u in range(1, NSUB + (i + 1 < WG)):
                    r0 = (u - 1) * (n_seg * PRE // NSUB)
                    stage[nxt % 3, D // 2 + c // n_chunk] = y[r0:r0 + 2 * WG].astype(BF16)
                    if u < NSUB:
                        relayout(nxt % 3, nxt, i * NSUB + u, WG * NSUB)
                pre[c, :, cols] = pltpu.pack_elementwise([y[:n_trip * PRE], y[n_trip * PRE:]], packed_dtype=BF16)
                wr = wo_rows // WG
                wo[jnp.maximum(p, 0), pl.ds(i * wr // 2, wr // 2), :] = pltpu.bitcast(
                    ostage[jnp.where(p >= 0, p % 2, 2), pl.ds(i * wr, wr), :], U32)
            return 0

        with jax.named_scope('ph_pre'):
            jax.lax.fori_loop(0, n_chunk, pre_body, 0)

    pl.run_scoped(load_phase,
                  pltpu.VMEM((n_seg, PRE, D), BF16),
                  pltpu.VMEM((n_seg * PRE, D), F32),
                  pltpu.VMEM((n_seg * PRE // 2, D), U32),
                  pltpu.VMEM((3, D // 2 + 1, 2 * WG, dh), BF16),
                  pltpu.VMEM((3, HG * dh, D), BF16),
                  pltpu.VMEM((4, D, 2 * D // 4), BF16))

    def main_phase(hn, att, st13, st2, stm, w13, w2, obuf):
        x_cp.wait()

        Dq, Fq = D // 4, F // 4
        r2 = st2.shape[2]
        n2 = Fq // r2
        assert n_trip * 8 == Dq and n2 * r2 == Fq and n2 <= n_trip and n_trip * 128 == 4 * D

        def ffn_w_cps(i):
            slot, i13, i2 = i % 2, jnp.minimum(i, n_trip - 1), jnp.minimum(i, n2 - 1)
            srcs = [w_hbm.at[:, pl.ds(pl.multiple_of(i13 // 2 * 16, 16), 16), :] for w_hbm in (w1_hbm, w3_hbm)]
            srcs += [w2_hbm.at[:, pl.ds(pl.multiple_of(i2 * r2, r2), r2), :],
                     wmod_hbm.at[:, pl.ds(pl.multiple_of(2 * D + i13 * 128, 128), 128)]]
            dsts = [st13.at[2 * slot], st13.at[2 * slot + 1], st2.at[slot], stm.at[slot]]
            return [pltpu.make_async_copy(a, b, sem_ffn.at[slot * 4 + n]) for n, (a, b) in enumerate(zip(srcs, dsts))]

        prep = ([(0, 0, cb) for cb in range(Fq // 128)]
                + [(1, rb, cb) for rb in range(r2 // 16) for cb in range(Dq // 128)])
        prep = [p + (ks,) for p in prep for ks in ([range(7 * i, 7 * i + 7) for i in range(7)] if SPLIT else [range(49)])]

        def ffn_w_prepare(i, part, anchor):
            down, rb, cb, ks = prep[part]
            cols = pl.ds(cb * 128, 128)
            if down:
                st2[2 + i // n_trip, 0, pl.ds(0, 16), pl.ds(0, 128)] = anchor
                w = _weight_operands([[st2[i % 2, r, pl.ds(rb * 16, 16), pl.ds(c * Dq + cb * 128, 128)]
                                       for c in range(4)] for r in range(4)])
                rows = pl.ds(pl.multiple_of(jnp.minimum(i, n2 - 1) * (r2 // 2) + rb * 8, 8), 8)
                for k in ks:
                    w2[k, rows, cols] = w[k]
            else:
                st13[4 + i // n_trip, 0, :, pl.ds(0, 128)] = anchor
                w = _weight_operands([[st13[i % 2 * 3, r, :, pl.ds(c * Fq + cb * 128, 128)]
                                       for c in range(4)] for r in range(4)])
                for k in ks:
                    w13[i % 2, k, pl.ds(pl.multiple_of(i // 2 * 8, 8), 8), cols] = w[k]

        start(ffn_w_cps(jnp.int32(0)))

        def ln1(trip, u):
            hn[...] = ada_ln(x_buf[trip, u, pl.ds(PRE, seg - PRE), :].astype(F32), 0)

        ln1(0, 0)
        n_hg = n_heads // HG

        def seg_step(trip, u, mem):
            s = trip * UNROLL + u
            lhs = jnp.concatenate([mem, hn[...]], axis=0).astype(BF16)
            ln1(jnp.minimum(trip + u, n_trip - 1), 1 - u)
            qi = jax.lax.broadcasted_iota(jnp.int32, (L, L), 0)
            ki = jax.lax.broadcasted_iota(jnp.int32, (L, L), 1)
            mask = (qi < M) | (qi >= ki)
            pr = pl.ds(pl.multiple_of(trip * PRE, PRE), PRE)

            def proj(t, g):
                gi, cols = g * HG // WG, pl.ds(g * HG % WG * dh, HG * dh)
                y = _dot(lhs, pltpu.bitcast(wqkv[3 * gi + t, :, cols], BF16))
                y = jnp.concatenate([y[:M], (_low_half, _high_half)[u](pre[3 * gi + t, pr, cols]), y[M:]], axis=0)
                return [y[:, h * dh:(h + 1) * dh] for h in range(HG)]

            def probs(q, k):
                sc_ = jnp.where(mask, _dot_nt(q, k.astype(BF16)) * (scale * LOG2E), -1e9 * LOG2E)
                e = jnp.exp2(sc_ - jnp.max(sc_, axis=-1, keepdims=True))
                den = jnp.sum(e, axis=-1, keepdims=True)
                r = pl.reciprocal(den, approx=True)
                return e, r * (2.0 - den * r)

            def mix(p, v):
                return jnp.concatenate([_dot(e, vh.astype(BF16)) * r for (e, r), vh in zip(p, v)], axis=1)

            def out_proj(o, g):
                y = _dot(o, _unpack(wo[g]))
                per = -(-len(prep) // (PREP_G * UNROLL))
                first = (u * PREP_G + g) * per
                for i in range(first, min(first + per, len(prep)) if g < PREP_G else 0):
                    n = (i - first) * (D // 128) // per
                    ffn_w_prepare(trip, i, y[:16, n * 128:(n + 1) * 128].astype(BF16))
                return y

            o, acc, p, v = {}, None, None, None
            done = 0
            for g in range(n_hg):
                q = proj(0, g)
                k = proj(1, g)
                if g == 1 and u == 0:
                    start(ffn_w_cps(trip + 1))
                if g:
                    o[g - 1] = mix(p, v)
                v = proj(2, g)
                p = [probs(qh, kh) for qh, kh in zip(q, k)]
                upto = g + 1 - LAG if g + 1 < n_hg else n_hg - 2
                while done < upto:
                    y = out_proj(o.pop(done), done)
                    acc = y if acc is None else acc + y
                    if done == MOD_AT and u == UNROLL - 1:
                        mod[2 * D // 128 + trip] = _dot(sc, stm[trip % 2])[:8]
                    done += 1
            o[n_hg - 1] = mix(p, v)
            for g in range(done, n_hg):
                acc = acc + out_proj(o.pop(g), g)
            att[s] = acc[M:].astype(BF16)
            return acc[:M]

        def seg_body(trip, mem):
            wait(ffn_w_cps(trip))
            for u in range(UNROLL):
                mem = seg_step(trip, u, mem)
            return mem

        with jax.named_scope('ph_seg'):
            jax.lax.fori_loop(0, n_trip, seg_body, mem0_ref[...].astype(F32))

        wait(ffn_w_cps(jnp.int32(n_trip)))

        sb = FFN_TM // seg

        qm = FFN_TM // 4

        a_per, h_per = D // 2 // qm, D // Dq
        h_base = -(-49 // a_per)

        def a_operand(k, cols):
            return (k // a_per, pl.ds(k % a_per * qm, qm // 2), cols)

        def h_operand(k, row, n, col=0, width=Dq):
            return (h_base + k // (a_per * h_per), pl.ds(k // h_per % a_per * qm + row, n),
                    pl.ds(k % h_per * Dq + col, width))

        def ffn_norm(i, row, odd):
            sg, rows = i * sb + row // seg, pl.ds(pl.multiple_of(row % seg, 16), 16)
            xw, aw = x_buf[sg // 2, sg % 2, rows, :], att[sg, rows, :]
            half = (_low_half, _high_half)[odd]
            h = ada_ln(half(pltpu.bitcast(xw, U32)) + mod_row(2) * half(pltpu.bitcast(aw, U32)), 3)
            xn = (xw.astype(F32) + mod_row(2) * aw.astype(F32))[8 * odd:8 * odd + 8]
            wo[2, pl.ds(row + 8 * odd, 8), :] = pltpu.bitcast(h, U32)
            wo[i % 2, pl.ds(row + 8 * odd, 8), :] = pltpu.bitcast(xn, U32)

        def ffn_lhs(row, col):
            hs = [[pltpu.bitcast(wo[2, pl.ds(r * qm + row, 8), pl.ds(c * Dq + col, 128)], F32)
                   for c in range(4)] for r in range(4)]
            for k, a in enumerate(_operands(_strassen_lhs, hs)):
                wqkv[h_operand(k, row, 8, col, 128)] = pltpu.bitcast(a, U32)

        @pl.loop(0, FFN_TM // seg)
        def _(j):
            for r in range(0, seg, 16):
                row = pl.multiple_of(j * seg + r, 16)
                for odd in range(2):
                    ffn_norm(0, row, odd)

        @pl.loop(0, qm // 8)
        def _(j):
            for col in range(0, Dq, 128):
                ffn_lhs(pl.multiple_of(j * 8, 8), col)

        def out_cp(i):
            return pltpu.make_async_copy(obuf.at[i % 2], out_hbm.at[pl.ds(i * FFN_TM, FFN_TM), :], sem_out.at[i % 2])

        n_blk = S // FFN_TM

        def ffn_body(i, _):
            @pl.when(i >= 2)
            def _():
                out_cp(i - 2).wait()

            zero, nxt = i // n_blk, jnp.minimum(i + 1, n_blk - 1)
            for j in range(Fq // 128):
                cols = pl.ds(j * 128, 128)
                gate, up = (_results(lambda k: _dot(pltpu.bitcast(wqkv[h_operand(k, 0, qm)], F32),
                                                    _unpack(w13[t, k, :, cols]))) for t in range(2))
                act = [[_silu(g) * u for g, u in zip(gr, ur)] for gr, ur in zip(gate, up)]
                for k, a in enumerate(_operands(_strassen_lhs, act)):
                    even, odd = (jnp.concatenate([a[r:r + 8] for r in range(p, qm, 16)], axis=0) for p in (0, 8))
                    wqkv[a_operand(k, cols)] = pltpu.pack_elementwise([even, odd], packed_dtype=BF16)

            def down_tile(k, n):
                m = _dot(_unpack(wqkv[a_operand(k, pl.ds(0, Fq))]), _unpack(w2[k, :, pl.ds(n * 128, 128)]))
                slot, n_norm = k * (Dq // 128) + n - FIRST, FFN_TM // 8
                if 0 <= slot < n_norm:
                    att[n_seg + zero, pl.ds(0, 16), pl.ds(0, 128)] = m[:16].astype(BF16)
                    ffn_norm(nxt, slot // 2 * 16, slot % 2)
                piece, phase = divmod(slot - n_norm, EVERY)
                if 0 <= piece < qm // 8 * (Dq // 128) and phase == 0:
                    wo[3 + zero, pl.ds(0, 8), pl.ds(0, 128)] = pltpu.bitcast(m[:8], U32)
                    ffn_lhs(piece // (Dq // 128) * 8, piece % (Dq // 128) * 128)
                return m

            def down(k):
                return jnp.concatenate([down_tile(k, n) for n in range(Dq // 128)], axis=1)

            y = jnp.concatenate([jnp.concatenate(row, axis=1) for row in _results(down)], axis=0)
            xn = pltpu.bitcast(wo[i % 2, pl.ds(0, FFN_TM), :], F32)
            obuf[i % 2] = (xn + mod_row(5) * y).astype(obuf.dtype)
            out_cp(i).start()
            return 0

        with jax.named_scope('ph_ffn'):
            jax.lax.fori_loop(0, n_blk, ffn_body, 0)
        for i in range(max(n_blk - 2, 0), n_blk):
            out_cp(i).wait()

    pl.run_scoped(main_phase,
                  pltpu.VMEM((seg - PRE, D), F32),
                  pltpu.VMEM((n_seg + 1, seg, D), BF16),
                  pltpu.VMEM((5, 4, 16, F), BF16),
                  pltpu.VMEM((3, 4, 32, D), BF16),
                  pltpu.VMEM((2, D, 128), BF16),
                  pltpu.VMEM((2, 49, D // 8, F // 4), U32),
                  pltpu.VMEM((49, F // 8, D // 4), U32),
                  pltpu.VMEM((2, FFN_TM, D), out_hbm.dtype))


@functools.partial(jax.jit, static_argnames=("A_seg_len",))
def pallas_adaLN_cond__memory_aug_recurrent_mem_tr__glu_gated_swiglu__prompt_kernel(
    A_x, A_mem0, A_Wq, A_Wk, A_Wv, A_Wo, A_seg_len, B_x, B_w1, B_w3, B_w2, c, w_mod,
):
    del B_x
    B, S, D = A_x.shape
    assert B == 1
    M = A_mem0.shape[1]
    _, H, Dh = A_Wq.shape
    F = B_w1.shape[1]
    seg = int(A_seg_len)
    n_seg, n_grp = S // seg, H // WG
    any_spec = pl.BlockSpec(memory_space=pl.ANY)
    vmem_spec = pl.BlockSpec(memory_space=pltpu.VMEM)
    out = pl.pallas_call(
        functools.partial(_kernel, n_heads=H, dh=Dh),
        out_shape=jax.ShapeDtypeStruct((S, D), A_x.dtype),
        in_specs=[any_spec, vmem_spec] + [any_spec] * 7 + [vmem_spec, any_spec],
        out_specs=any_spec,
        scratch_shapes=[
            pltpu.VMEM((n_seg // 2, 2, seg, D), BF16),
            pltpu.VMEM((3 * n_grp, D // 2, WG * Dh), U32),
            pltpu.VMEM((H // HG, HG * Dh // 2, D), U32),
            pltpu.VMEM((3 * n_grp, n_seg // 2 * PRE, WG * Dh), U32),
            pltpu.VMEM((6 * D // 128, 8, 128), F32),
            pltpu.SemaphoreType.DMA((3,)),
            pltpu.SemaphoreType.DMA((6,)),
            pltpu.SemaphoreType.DMA((4,)),
            pltpu.SemaphoreType.DMA((2,)),
            pltpu.SemaphoreType.DMA((8,)),
            pltpu.SemaphoreType.DMA((2,)),
        ],
        compiler_params=pltpu.CompilerParams(vmem_limit_bytes=127 * 1024 * 1024),
    )(
        A_x.reshape(n_seg // 2, 2, seg, D), A_mem0.reshape(M, D),
        A_Wq.reshape(D // 2, 2 * H, Dh), A_Wk.reshape(D // 2, 2 * H, Dh), A_Wv.reshape(D // 2, 2 * H, Dh),
        A_Wo.reshape(H * Dh, D),
        B_w1.reshape(4, D // 4, F), B_w3.reshape(4, D // 4, F), B_w2.reshape(4, F // 4, D), c, w_mod,
    )
    return out.reshape(B, S, D)
```

```python
import functools

import jax
import jax.numpy as jnp
import jax.experimental.pallas as pl
import jax.experimental.pallas.tpu as pltpu

F32 = jnp.float32
BF16 = jnp.bfloat16
U32 = jnp.uint32
LOG2E = 1.4426950408889634

PRE = 8
WG = 8
LAG = 6
EVERY = 4
LN2_AT = (1, 2)
DMA_AT = 1
LN1_AT = 0
FIRST = 0
SPLIT = 1
NSUB = 4
PREP_G = 8
RB = 8
UNROLL = 2
HG = 4
FFN_TM = 256
FFN_TF = 128


def _dot(a, b):
    return jax.lax.dot_general(a, b, (((1,), (0,)), ((), ())), preferred_element_type=F32)


def _dot_nt(a, b):
    return jax.lax.dot_general(a, b, (((1,), (1,)), ((), ())), preferred_element_type=F32)


def _round_bf16(x):
    return x.astype(BF16).astype(F32)


def _silu(x):
    t = 0.5 * x
    return t * jnp.tanh(t) + t


def _layernorm(x):
    m = jnp.mean(x, axis=-1, keepdims=True)
    d = x - m
    v = jnp.mean(d * d, axis=-1, keepdims=True)
    return d * jax.lax.rsqrt(v + 1e-5)


def _pack(x):
    return pltpu.bitcast(x.astype(BF16), U32)


def _unpack(w):
    return pltpu.bitcast(w, BF16)


def _low_half(w):
    return pltpu.bitcast(w << 16, F32)


def _high_half(w):
    return pltpu.bitcast(w & jnp.uint32(0xFFFF0000), F32)


def _strassen_lhs(a11, a12, a21, a22):
    return (a11 + a22, a21 + a22, a11, a22, a11 + a12, a21 - a11, a12 - a22)


def _strassen_rhs(b11, b12, b21, b22):
    return (b11 + b22, b11, b12 - b22, b21 - b11, b22, b11 + b12, b21 + b22)


def _strassen_out(m):
    return (m[0] + m[3] - m[4] + m[6], m[2] + m[4], m[1] + m[3], m[0] - m[1] + m[2] + m[5])


def _operands(level, x):
    outer = [level(x[r][c], x[r][c + 2], x[r + 2][c], x[r + 2][c + 2]) for r in range(2) for c in range(2)]
    return [y for i in range(7) for y in level(*[o[i] for o in outer])]


def _results(product):
    inner = [_strassen_out([product(7 * i + j) for j in range(7)]) for i in range(7)]
    outer = [_strassen_out([m[rc] for m in inner]) for rc in range(4)]
    return [[outer[r % 2 * 2 + c % 2][r // 2 * 2 + c // 2] for c in range(4)] for r in range(4)]


def _weight_operands(blocks):
    words = [[pltpu.bitcast(b, U32) for b in row] for row in blocks]
    even = _operands(_strassen_rhs, [[_low_half(w) for w in row] for row in words])
    odd = _operands(_strassen_rhs, [[_high_half(w) for w in row] for row in words])
    return [pltpu.pack_elementwise([e, o], packed_dtype=BF16) for e, o in zip(even, odd)]


def _kernel(x_hbm, mem0_ref, wq_hbm, wk_hbm, wv_hbm, wo_hbm, w1_hbm, w3_hbm, w2_hbm, c_ref, wmod_hbm,
            out_hbm,
            x_buf, wqkv, wo, pre, mod, st13, st2, sem_x, sem_stage, sem_m, sem_o, sem_ffn, sem_out, *, n_heads, dh):
    n_trip, _, seg, D = x_buf.shape
    n_seg = 2 * n_trip
    S = n_seg * seg
    M = mem0_ref.shape[0]
    L = M + seg
    scale = dh ** -0.5
    F = w1_hbm.shape[2]
    n_grp = n_heads // WG
    w_hbms = (wq_hbm, wk_hbm, wv_hbm)

    x_cp = pltpu.make_async_copy(x_hbm, x_buf, sem_x.at[2])

    Dq, Fq = D // 4, F // 4
    r2 = st2.shape[2]
    n2 = Fq // r2
    assert n_trip * 8 == Dq and n2 * r2 == Fq and n2 <= n_trip

    def ffn_w_cps(i):
        slot, i13, i2 = i % 2, jnp.minimum(i, n_trip - 1), jnp.minimum(i, n2 - 1)
        srcs = [w_hbm.at[:, pl.ds(pl.multiple_of(i13 // 2 * 16, 16), 16), :] for w_hbm in (w1_hbm, w3_hbm)]
        srcs += [w2_hbm.at[:, pl.ds(pl.multiple_of(i2 * r2, r2), r2), :]]
        dsts = [st13.at[2 * slot], st13.at[2 * slot + 1], st2.at[slot]]
        return [pltpu.make_async_copy(a, b, sem_ffn.at[slot * 3 + n]) for n, (a, b) in enumerate(zip(srcs, dsts))]

    def start(cps):
        for cp in cps:
            cp.start()

    def wait(cps):
        for cp in cps:
            cp.wait()

    def mod_rows(j, rows):
        tile = jnp.concatenate([mod[j * (D // 128) + n] for n in range(D // 128)], axis=1)
        return jnp.concatenate([tile] * (rows // 8), axis=0)

    def ada_ln(x, j):
        return _layernorm(x) * (1.0 + mod_rows(j + 1, x.shape[0])) + mod_rows(j, x.shape[0])

    cc = c_ref[...].astype(F32)
    sc = jnp.broadcast_to(cc * jax.nn.sigmoid(cc), (16, D)).astype(BF16)

    def load_phase(xp, lnp, hp, stage, ostage, mstage, lstage):
        xp_cps = [pltpu.make_async_copy(x_hbm.at[:, u, pl.ds(0, PRE), :], xp.at[pl.ds(u * n_trip, n_trip)],
                                        sem_x.at[u]) for u in range(2)]

        n_mod, _, mod_cols = mstage.shape

        def wmod_cp(j):
            return pltpu.make_async_copy(wmod_hbm.at[:, pl.ds(pl.multiple_of(j * mod_cols, mod_cols), mod_cols)],
                                         mstage.at[j], sem_m.at[j])

        lt = lstage.shape[2] // 128

        def late_tile(c):
            return jnp.minimum(2 * D // 128 + (c - 1) * lt, 6 * D // 128 - lt)

        def late_cp(c):
            return pltpu.make_async_copy(wmod_hbm.at[:, pl.ds(pl.multiple_of(late_tile(c) * 128, 128), lt * 128)],
                                         lstage.at[c % 2], sem_m.at[n_mod + c % 2])

        n_wo, wo_rows = wo.shape[0], ostage.shape[1]

        def wo_cp(p):
            return pltpu.make_async_copy(wo_hbm.at[pl.ds(pl.multiple_of(p * wo_rows, wo_rows), wo_rows), :],
                                         ostage.at[p % 2], sem_o.at[p % 2])

        def w_cps(t, g):
            return [pltpu.make_async_copy(w_hbms[t].at[:, pl.ds(pl.multiple_of(p * n_heads + g * WG, WG), WG), :],
                                          stage.at[t, pl.ds(0, D // 2), pl.ds(p * WG, WG), :], sem_stage.at[2 * t + p])
                    for p in range(2)]

        def relayout(t, c, part=0, n_part=1):
            nb_ = D // 2 // RB // n_part
            for b in range(nb_):
                rows = pl.ds(pl.multiple_of((part * nb_ + b) * RB, RB), RB)
                w = jnp.swapaxes(pltpu.bitcast(stage[t, rows], U32), 0, 1)
                for j in range(WG // 2):
                    even, odd = w[j], w[WG // 2 + j]
                    wqkv[c, rows, pl.ds(2 * j * dh, dh)] = (even & jnp.uint32(0xFFFF)) | (odd << 16)
                    wqkv[c, rows, pl.ds((2 * j + 1) * dh, dh)] = (even >> 16) | (odd & jnp.uint32(0xFFFF0000))

        start(xp_cps)
        start(w_cps(0, 0))
        wmod_cp(0).start()
        ostage[2] = jnp.zeros(ostage.shape[1:], BF16)
        lstage[0] = jnp.zeros(lstage.shape[1:], BF16)
        wait(xp_cps)
        for j in range(1, n_mod):
            wmod_cp(j).start()
        nb = 64 // PRE

        @pl.loop(0, n_seg // nb)
        def _(i):
            xs = xp[pl.ds(i * nb, nb)].astype(F32).reshape(nb * PRE, D)
            lnp[pl.ds(pl.multiple_of(i * nb * PRE, nb * PRE), nb * PRE), :] = _layernorm(xs)

        wait(w_cps(0, 0))
        start(w_cps(1, 0))

        @pl.loop(0, 8)
        def _(i):
            relayout(0, 0, i, 8)

        @pl.loop(0, n_mod)
        def _(j):
            wmod_cp(j).wait()
            y = _dot(sc, mstage[j])
            for n in range(mod_cols // 128):
                mod[j * (mod_cols // 128) + n] = y[:8, n * 128:(n + 1) * 128]

        start(w_cps(2, 0))

        @pl.loop(0, n_seg // nb)
        def _(i):
            ln = lnp[pl.ds(pl.multiple_of(i * nb * PRE, nb * PRE), nb * PRE), :]
            rows = pl.ds(pl.multiple_of(i * (nb * PRE // 2), nb * PRE // 2), nb * PRE // 2)
            hp[rows, :] = _pack(ln * (1.0 + mod_rows(1, nb * PRE)) + mod_rows(0, nb * PRE))

        n_chunk = 3 * n_grp
        assert (n_chunk - 1) * lt * 128 >= 4 * D

        def pre_body(c, _):
            g = c // 3
            p = c - (n_chunk - n_wo)

            @pl.when(jnp.logical_and(p + 1 >= 0, p + 1 < n_wo))
            def _():
                wo_cp(p + 1).start()

            @pl.when(c + 1 < n_chunk)
            def _():
                late_cp(c + 1).start()

            for t in range(3):
                @pl.when(c % 3 == t)
                def _():
                    @pl.when(g + 1 < n_grp)
                    def _():
                        start(w_cps(t, g + 1))

                    if t == 0:
                        @pl.when(g + 1 == n_grp)
                        def _():
                            x_cp.start()

                    if t < 2:
                        wait(w_cps(t + 1, g))
                    else:
                        @pl.when(g + 1 < n_grp)
                        def _():
                            wait(w_cps(0, g + 1))


            @pl.when(p >= 0)
            def _():
                wo_cp(p).wait()

            @pl.when(c + 1 == n_chunk)
            def _():
                start(ffn_w_cps(jnp.int32(0)))

            @pl.when(c > 0)
            def _():
                late_cp(c).wait()

            nxt = jnp.minimum(c + 1, n_chunk - 1)
            for i in range(WG):
                cols = pl.ds(i * dh, dh)
                y = _dot(_unpack(hp[...]), _unpack(wqkv[c, :, cols]))
                relayout(nxt % 3, nxt, i * NSUB, WG * NSUB)
                for u in range(1, NSUB + (i + 1 < WG)):
                    r0 = (u - 1) * (n_seg * PRE // NSUB)
                    stage[nxt % 3, D // 2 + c // n_chunk] = y[r0:r0 + 2 * WG].astype(BF16)
                    if u < NSUB:
                        relayout(nxt % 3, nxt, i * NSUB + u, WG * NSUB)
                pre[c, :, cols] = pltpu.pack_elementwise([y[:n_trip * PRE], y[n_trip * PRE:]], packed_dtype=BF16)
                if 1 <= i <= lt:
                    mod[late_tile(jnp.maximum(c, 1)) + i - 1] = _dot(sc, lstage[c % 2, :, pl.ds((i - 1) * 128, 128)])[:8]
                wr = wo_rows // WG
                wo[jnp.maximum(p, 0), pl.ds(i * wr // 2, wr // 2), :] = pltpu.bitcast(
                    ostage[jnp.where(p >= 0, p % 2, 2), pl.ds(i * wr, wr), :], U32)
            return 0

        with jax.named_scope('ph_pre'):
            jax.lax.fori_loop(0, n_chunk, pre_body, 0)

    pl.run_scoped(load_phase,
                  pltpu.VMEM((n_seg, PRE, D), BF16),
                  pltpu.VMEM((n_seg * PRE, D), F32),
                  pltpu.VMEM((n_seg * PRE // 2, D), U32),
                  pltpu.VMEM((3, D // 2 + 1, 2 * WG, dh), BF16),
                  pltpu.VMEM((3, HG * dh, D), BF16),
                  pltpu.VMEM((4, D, 2 * D // 4), BF16),
                  pltpu.VMEM((2, D, 3 * 128), BF16))

    def main_phase(hn, att, x1, h2, w13, w2, obuf):
        x_cp.wait()

        prep = ([(0, 0, cb) for cb in range(Fq // 128)]
                + [(1, rb, cb) for rb in range(r2 // 16) for cb in range(Dq // 128)])
        prep = [p + (ks,) for p in prep for ks in ([range(7 * i, 7 * i + 7) for i in range(7)] if SPLIT else [range(49)])]

        def ffn_w_prepare(i, part, anchor):
            down, rb, cb, ks = prep[part]
            cols = pl.ds(cb * 128, 128)
            if down:
                st2[2 + i // n_trip, 0, pl.ds(0, 16), pl.ds(0, 128)] = anchor
                w = _weight_operands([[st2[i % 2, r, pl.ds(rb * 16, 16), pl.ds(c * Dq + cb * 128, 128)]
                                       for c in range(4)] for r in range(4)])
                rows = pl.ds(pl.multiple_of(jnp.minimum(i, n2 - 1) * (r2 // 2) + rb * 8, 8), 8)
                for k in ks:
                    w2[k, rows, cols] = w[k]
            else:
                st13[4 + i // n_trip, 0, :, pl.ds(0, 128)] = anchor
                w = _weight_operands([[st13[i % 2 * 3, r, :, pl.ds(c * Fq + cb * 128, 128)]
                                       for c in range(4)] for r in range(4)])
                for k in ks:
                    w13[i % 2, k, pl.ds(pl.multiple_of(i // 2 * 8, 8), 8), cols] = w[k]

        def ln1(trip, u):
            hn[...] = ada_ln(x_buf[trip, u, pl.ds(PRE, seg - PRE), :].astype(F32), 0)

        def ln2(trip, u, r):
            rows = pl.ds(r, 16)
            xn = x_buf[trip, u, rows, :].astype(F32) + mod_rows(2, 16) * att[0, rows, :]
            x1[2 * trip + u, rows, :] = xn.astype(BF16)
            h2[2 * trip + u, rows, :] = ada_ln(xn, 3).astype(BF16)

        att[0] = jnp.zeros(att.shape[1:], F32)
        ln1(0, 0)
        n_hg = n_heads // HG

        def seg_step(trip, u, mem):
            lhs = jnp.concatenate([mem, hn[...]], axis=0).astype(BF16)
            qi = jax.lax.broadcasted_iota(jnp.int32, (L, L), 0)
            ki = jax.lax.broadcasted_iota(jnp.int32, (L, L), 1)
            mask = (qi < M) | (qi >= ki)
            pr = pl.ds(pl.multiple_of(trip * PRE, PRE), PRE)

            def proj(t, g):
                gi, cols = g * HG // WG, pl.ds(g * HG % WG * dh, HG * dh)
                y = _dot(lhs, pltpu.bitcast(wqkv[3 * gi + t, :, cols], BF16))
                y = jnp.concatenate([y[:M], (_low_half, _high_half)[u](pre[3 * gi + t, pr, cols]), y[M:]], axis=0)
                return [y[:, h * dh:(h + 1) * dh] for h in range(HG)]

            def probs(q, k):
                sc_ = jnp.where(mask, _dot_nt(q, k.astype(BF16)) * (scale * LOG2E), -1e9 * LOG2E)
                e = jnp.exp2(sc_ - jnp.max(sc_, axis=-1, keepdims=True))
                den = jnp.sum(e, axis=-1, keepdims=True)
                r = pl.reciprocal(den, approx=True)
                return e, r * (2.0 - den * r)

            def mix(p, v):
                return jnp.concatenate([_dot(e, vh.astype(BF16)) * r for (e, r), vh in zip(p, v)], axis=1)

            def out_proj(o, g):
                y = _dot(o, _unpack(wo[g]))
                per = -(-len(prep) // (PREP_G * UNROLL))
                first = (u * PREP_G + g) * per
                for i in range(first, min(first + per, len(prep)) if g < PREP_G else 0):
                    n = (i - first) * (D // 128) // per
                    ffn_w_prepare(trip, i, y[:16, n * 128:(n + 1) * 128].astype(BF16))
                return y

            o, acc, p, v = {}, None, None, None
            done = 0
            for g in range(n_hg):
                q = proj(0, g)
                k = proj(1, g)
                if g in LN2_AT:
                    att[1 + trip // n_trip, pl.ds(0, 8), pl.ds(0, dh)] = q[0][:8]
                    ln2(jnp.maximum(trip + u - 1, 0), 1 - u, LN2_AT.index(g) * 16)
                if g == LN1_AT:
                    ln1(jnp.minimum(trip + u, n_trip - 1), 1 - u)
                if g == DMA_AT and u == 0:
                    start(ffn_w_cps(trip + 1))
                if g:
                    o[g - 1] = mix(p, v)
                v = proj(2, g)
                p = [probs(qh, kh) for qh, kh in zip(q, k)]
                upto = g + 1 - LAG if g + 1 < n_hg else n_hg - 2
                while done < upto:
                    y = out_proj(o.pop(done), done)
                    acc = y if acc is None else acc + y
                    done += 1
            o[n_hg - 1] = mix(p, v)
            for g in range(done, n_hg):
                acc = acc + out_proj(o.pop(g), g)
            att[0] = acc[M:]
            return acc[:M]

        def seg_body(trip, mem):
            wait(ffn_w_cps(trip))
            for u in range(UNROLL):
                mem = seg_step(trip, u, mem)
            return mem

        with jax.named_scope('ph_seg'):
            jax.lax.fori_loop(0, n_trip, seg_body, mem0_ref[...].astype(F32))

        wait(ffn_w_cps(jnp.int32(n_trip)))
        for r in range(0, seg, 16):
            ln2(n_trip - 1, 1, r)

        sb = FFN_TM // seg

        qm = FFN_TM // 4

        a_per, h_per = D // 2 // qm, D // Dq
        h_base = -(-49 // a_per)

        def a_operand(k, cols):
            return (k // a_per, pl.ds(k % a_per * qm, qm // 2), cols)

        def h_operand(k, row, n, col=0, width=Dq):
            return (h_base + k // (a_per * h_per), pl.ds(k // h_per % a_per * qm + row, n),
                    pl.ds(k % h_per * Dq + col, width))

        def ffn_lhs(i, row, odd, col):
            rows = pl.ds(pl.multiple_of(row % seg, 16), 16)
            hs = [[(_low_half, _high_half)[odd](pltpu.bitcast(
                h2[i * sb + r * qm // seg + row // seg, rows, pl.ds(c * Dq + col, 128)], U32))
                for c in range(4)] for r in range(4)]
            for k, a in enumerate(_operands(_strassen_lhs, hs)):
                wqkv[h_operand(k, row + 8 * odd, 8, col, 128)] = pltpu.bitcast(a, U32)

        lhs_parts = [(odd, col) for odd in range(2) for col in range(0, Dq, 128)]

        @pl.loop(0, qm // 16)
        def _(j):
            for odd, col in lhs_parts:
                ffn_lhs(0, pl.multiple_of(j * 16, 16), odd, col)

        def out_cp(i):
            return pltpu.make_async_copy(obuf.at[i % 2], out_hbm.at[pl.ds(i * FFN_TM, FFN_TM), :], sem_out.at[i % 2])

        n_blk = S // FFN_TM

        def ffn_body(i, _):
            @pl.when(i >= 2)
            def _():
                out_cp(i - 2).wait()

            zero, nxt = i // n_blk, jnp.minimum(i + 1, n_blk - 1)
            for j in range(Fq // 128):
                cols = pl.ds(j * 128, 128)
                gate, up = (_results(lambda k: _dot(pltpu.bitcast(wqkv[h_operand(k, 0, qm)], F32),
                                                    _unpack(w13[t, k, :, cols]))) for t in range(2))
                act = [[_silu(g) * u for g, u in zip(gr, ur)] for gr, ur in zip(gate, up)]
                for k, a in enumerate(_operands(_strassen_lhs, act)):
                    even, odd = (jnp.concatenate([a[r:r + 8] for r in range(p, qm, 16)], axis=0) for p in (0, 8))
                    wqkv[a_operand(k, cols)] = pltpu.pack_elementwise([even, odd], packed_dtype=BF16)

            def down_tile(k, n):
                m = _dot(_unpack(wqkv[a_operand(k, pl.ds(0, Fq))]), _unpack(w2[k, :, pl.ds(n * 128, 128)]))
                piece, phase = divmod(k * (Dq // 128) + n - FIRST, EVERY)
                if 0 <= piece < qm // 16 * len(lhs_parts) and phase == 0:
                    h2[n_seg + zero, pl.ds(0, 16), pl.ds(0, 128)] = m[:16].astype(BF16)
                    ffn_lhs(nxt, piece // len(lhs_parts) * 16, *lhs_parts[piece % len(lhs_parts)])
                return m

            def down(k):
                return jnp.concatenate([down_tile(k, n) for n in range(Dq // 128)], axis=1)

            y = jnp.concatenate([jnp.concatenate(row, axis=1) for row in _results(down)], axis=0)
            xn = x1[pl.ds(i * sb, sb)].astype(F32).reshape(FFN_TM, D)
            obuf[i % 2] = (xn + mod_rows(5, FFN_TM) * y).astype(obuf.dtype)
            out_cp(i).start()
            return 0

        with jax.named_scope('ph_ffn'):
            jax.lax.fori_loop(0, n_blk, ffn_body, 0)
        for i in range(max(n_blk - 2, 0), n_blk):
            out_cp(i).wait()

    pl.run_scoped(main_phase,
                  pltpu.VMEM((seg - PRE, D), F32),
                  pltpu.VMEM((2, seg, D), F32),
                  pltpu.VMEM((n_seg, seg, D), BF16),
                  pltpu.VMEM((n_seg + 1, seg, D), BF16),
                  pltpu.VMEM((2, 49, D // 8, F // 4), U32),
                  pltpu.VMEM((49, F // 8, D // 4), U32),
                  pltpu.VMEM((2, FFN_TM, D), out_hbm.dtype))


@functools.partial(jax.jit, static_argnames=("A_seg_len",))
def pallas_adaLN_cond__memory_aug_recurrent_mem_tr__glu_gated_swiglu__prompt_kernel(
    A_x, A_mem0, A_Wq, A_Wk, A_Wv, A_Wo, A_seg_len, B_x, B_w1, B_w3, B_w2, c, w_mod,
):
    del B_x
    B, S, D = A_x.shape
    assert B == 1
    M = A_mem0.shape[1]
    _, H, Dh = A_Wq.shape
    F = B_w1.shape[1]
    seg = int(A_seg_len)
    n_seg, n_grp = S // seg, H // WG
    any_spec = pl.BlockSpec(memory_space=pl.ANY)
    vmem_spec = pl.BlockSpec(memory_space=pltpu.VMEM)
    out = pl.pallas_call(
        functools.partial(_kernel, n_heads=H, dh=Dh),
        out_shape=jax.ShapeDtypeStruct((S, D), A_x.dtype),
        in_specs=[any_spec, vmem_spec] + [any_spec] * 7 + [vmem_spec, any_spec],
        out_specs=any_spec,
        scratch_shapes=[
            pltpu.VMEM((n_seg // 2, 2, seg, D), BF16),
            pltpu.VMEM((3 * n_grp, D // 2, WG * Dh), U32),
            pltpu.VMEM((H // HG, HG * Dh // 2, D), U32),
            pltpu.VMEM((3 * n_grp, n_seg // 2 * PRE, WG * Dh), U32),
            pltpu.VMEM((6 * D // 128, 8, 128), F32),
            pltpu.VMEM((5, 4, 16, F), BF16),
            pltpu.VMEM((3, 4, 32, D), BF16),
            pltpu.SemaphoreType.DMA((3,)),
            pltpu.SemaphoreType.DMA((6,)),
            pltpu.SemaphoreType.DMA((6,)),
            pltpu.SemaphoreType.DMA((2,)),
            pltpu.SemaphoreType.DMA((6,)),
            pltpu.SemaphoreType.DMA((2,)),
        ],
        compiler_params=pltpu.CompilerParams(vmem_limit_bytes=127 * 1024 * 1024),
    )(
        A_x.reshape(n_seg // 2, 2, seg, D), A_mem0.reshape(M, D),
        A_Wq.reshape(D // 2, 2 * H, Dh), A_Wk.reshape(D // 2, 2 * H, Dh), A_Wv.reshape(D // 2, 2 * H, Dh),
        A_Wo.reshape(H * Dh, D),
        B_w1.reshape(4, D // 4, F), B_w3.reshape(4, D // 4, F), B_w2.reshape(4, F // 4, D), c, w_mod,
    )
    return out.reshape(B, S, D)
```

```python
import functools

import jax
import jax.numpy as jnp
import jax.experimental.pallas as pl
import jax.experimental.pallas.tpu as pltpu

F32 = jnp.float32
BF16 = jnp.bfloat16
U32 = jnp.uint32
LOG2E = 1.4426950408889634

PRE = 8
WG = 8
NSUB = 4
HG = 4
LAG = 7
FFN_TM = 256
PARKED = 2
EVERY = 4


def _dot(a, b):
    return jax.lax.dot_general(a, b, (((1,), (0,)), ((), ())), preferred_element_type=F32)


def _dot_nt(a, b):
    return jax.lax.dot_general(a, b, (((1,), (1,)), ((), ())), preferred_element_type=F32)


def _silu(x):
    t = 0.5 * x
    return t * jnp.tanh(t) + t


def _layernorm(x):
    m = jnp.mean(x, axis=-1, keepdims=True)
    d = x - m
    v = jnp.mean(d * d, axis=-1, keepdims=True)
    return d * jax.lax.rsqrt(v + 1e-5)


def _pack(x):
    return pltpu.bitcast(x.astype(BF16), U32)


def _unpack(w):
    return pltpu.bitcast(w, BF16)


def _strassen_lhs(a11, a12, a21, a22):
    return (a11 + a22, a21 + a22, a11, a22, a11 + a12, a21 - a11, a12 - a22)


def _strassen_rhs(b11, b12, b21, b22):
    return (b11 + b22, b11, b12 - b22, b21 - b11, b22, b11 + b12, b21 + b22)


def _strassen_out(m):
    return (m[0] + m[3] - m[4] + m[6], m[2] + m[4], m[1] + m[3], m[0] - m[1] + m[2] + m[5])


def _operands(level, x):
    outer = [level(x[r][c], x[r][c + 2], x[r + 2][c], x[r + 2][c + 2]) for r in range(2) for c in range(2)]
    return [y for i in range(7) for y in level(*[o[i] for o in outer])]


def _results(product):
    inner = [_strassen_out([product(7 * i + j) for j in range(7)]) for i in range(7)]
    outer = [_strassen_out([m[rc] for m in inner]) for rc in range(4)]
    return [[outer[r % 2 * 2 + c % 2][r // 2 * 2 + c // 2] for c in range(4)] for r in range(4)]


def _kernel(x_hbm, mem0_hbm, wq_hbm, wk_hbm, wv_hbm, wo_hbm, w1_hbm, w3_hbm, w2_hbm, c_hbm, wmod_hbm,
            out_hbm,
            x_buf, mem0, c_buf, wqkv, wo, pre, mod, st13, st2,
            sem_x, sem_stage, sem_m, sem_o, sem_ffn, sem_out, *, n_heads, dh):
    n_seg, seg, D = x_buf.shape
    n_trip = n_seg // 2
    S = n_seg * seg
    M = mem0.shape[0]
    L = M + seg
    scale = dh ** -0.5
    F = w1_hbm.shape[2]
    n_grp = n_heads // WG
    w_hbms = (wq_hbm, wk_hbm, wv_hbm)

    x_cp = pltpu.make_async_copy(x_hbm, x_buf, sem_x.at[0])

    Dq, Fq = D // 4, F // 4
    r2 = st2.shape[2]
    n2 = Fq // r2
    assert n_trip * 8 == Dq and n2 * r2 == Fq and n2 <= n_trip

    def ffn_w_cps(i):
        slot, i13, i2 = i % 2, jnp.minimum(i, n_trip - 1), jnp.minimum(i, n2 - 1)
        srcs = [w_hbm.at[:, pl.ds(pl.multiple_of(i13 // 2 * 16, 16), 16), :] for w_hbm in (w1_hbm, w3_hbm)]
        srcs += [w2_hbm.at[:, pl.ds(pl.multiple_of(i2 * r2, r2), r2), :]]
        dsts = [st13.at[2 * slot], st13.at[2 * slot + 1], st2.at[slot]]
        return [pltpu.make_async_copy(a, b, sem_ffn.at[slot * 3 + n]) for n, (a, b) in enumerate(zip(srcs, dsts))]

    def start(cps):
        for cp in cps:
            cp.start()

    def wait(cps):
        for cp in cps:
            cp.wait()

    def mod_rows(j, rows):
        tile = jnp.concatenate([mod[j * (D // 128) + n] for n in range(D // 128)], axis=1)
        return jnp.concatenate([tile] * (rows // 8), axis=0)

    def ada_ln(x, j):
        return _layernorm(x) * (1.0 + mod_rows(j + 1, x.shape[0])) + mod_rows(j, x.shape[0])

    def load_phase(xp, lnp, hp, stage, ostage, mstage, lstage):
        xp_cps = [pltpu.make_async_copy(x_hbm.at[:, pl.ds(0, PRE), :], xp, sem_x.at[1]),
                  pltpu.make_async_copy(c_hbm, c_buf, sem_x.at[2]),
                  pltpu.make_async_copy(mem0_hbm, mem0, sem_x.at[3])]
        n_mod, _, mod_cols = mstage.shape

        def wmod_cp(j):
            return pltpu.make_async_copy(wmod_hbm.at[:, pl.ds(pl.multiple_of(j * mod_cols, mod_cols), mod_cols)],
                                         mstage.at[j], sem_m.at[j])

        lt = lstage.shape[2] // 128

        def late_tile(c):
            return jnp.minimum(2 * D // 128 + (c - 1) * lt, 6 * D // 128 - lt)

        def late_cp(c):
            return pltpu.make_async_copy(wmod_hbm.at[:, pl.ds(pl.multiple_of(late_tile(c) * 128, 128), lt * 128)],
                                         lstage.at[c % 2], sem_m.at[n_mod + c % 2])

        n_wo, wo_rows = wo.shape[0], ostage.shape[1]

        def wo_cp(p):
            return pltpu.make_async_copy(wo_hbm.at[pl.ds(pl.multiple_of(p * wo_rows, wo_rows), wo_rows), :],
                                         ostage.at[p % 2], sem_o.at[p % 2])

        def w_cps(t, g):
            return [pltpu.make_async_copy(w_hbms[t].at[:, pl.ds(pl.multiple_of(p * n_heads + g * WG, WG), WG), :],
                                          stage.at[t, pl.ds(0, D // 2), pl.ds(p * WG, WG), :], sem_stage.at[2 * t + p])
                    for p in range(2)]

        def relayout(t, c, part, n_part):
            per = D // 2 // 8 // n_part
            for b in range(per):
                rows = pl.ds(pl.multiple_of((part * per + b) * 8, 8), 8)
                w = jnp.swapaxes(pltpu.bitcast(stage[t, rows], U32), 0, 1)
                for j in range(WG // 2):
                    even, odd = w[j], w[WG // 2 + j]
                    wqkv[c, rows, pl.ds(2 * j * dh, dh)] = (even & jnp.uint32(0xFFFF)) | (odd << 16)
                    wqkv[c, rows, pl.ds((2 * j + 1) * dh, dh)] = (even >> 16) | (odd & jnp.uint32(0xFFFF0000))

        start(xp_cps)
        start(w_cps(0, 0))
        wmod_cp(0).start()
        ostage[2] = jnp.zeros(ostage.shape[1:], BF16)
        lstage[0] = jnp.zeros(lstage.shape[1:], BF16)
        wait(xp_cps)
        for j in range(1, n_mod):
            wmod_cp(j).start()
        sc = jnp.broadcast_to(_silu(c_buf[...].astype(F32)), (16, D)).astype(BF16)
        nb = 64 // PRE

        @pl.loop(0, n_seg // nb)
        def _(i):
            xs = xp[pl.ds(i * nb, nb)].astype(F32).reshape(nb * PRE, D)
            lnp[pl.ds(pl.multiple_of(i * nb * PRE, nb * PRE), nb * PRE), :] = _layernorm(xs)

        wait(w_cps(0, 0))
        start(w_cps(1, 0))

        @pl.loop(0, 8)
        def _(i):
            relayout(0, 0, i, 8)

        @pl.loop(0, n_mod)
        def _(j):
            wmod_cp(j).wait()
            y = _dot(sc, mstage[j])
            for n in range(mod_cols // 128):
                mod[j * (mod_cols // 128) + n] = y[:8, n * 128:(n + 1) * 128]

        start(w_cps(2, 0))

        @pl.loop(0, n_seg // nb)
        def _(i):
            ln = lnp[pl.ds(pl.multiple_of(i * nb * PRE, nb * PRE), nb * PRE), :]
            rows = pl.ds(pl.multiple_of(i * (nb * PRE // 2), nb * PRE // 2), nb * PRE // 2)
            hp[rows, :] = _pack(ln * (1.0 + mod_rows(1, nb * PRE)) + mod_rows(0, nb * PRE))

        n_chunk = 3 * n_grp
        assert (n_chunk - 1) * lt * 128 >= 4 * D

        def pre_body(c, _):
            g = c // 3
            p = c - (n_chunk - n_wo)

            @pl.when(jnp.logical_and(p + 1 >= 0, p + 1 < n_wo))
            def _():
                wo_cp(p + 1).start()

            @pl.when(c + 1 < n_chunk)
            def _():
                late_cp(c + 1).start()

            for t in range(3):
                @pl.when(c % 3 == t)
                def _():
                    @pl.when(g + 1 < n_grp)
                    def _():
                        start(w_cps(t, g + 1))

                    if t == 0:
                        @pl.when(g + 1 == n_grp)
                        def _():
                            x_cp.start()

                    if t < 2:
                        wait(w_cps(t + 1, g))
                    else:
                        @pl.when(g + 1 < n_grp)
                        def _():
                            wait(w_cps(0, g + 1))

            @pl.when(p >= 0)
            def _():
                wo_cp(p).wait()

            @pl.when(c + 1 == n_chunk)
            def _():
                start(ffn_w_cps(jnp.int32(0)))

            @pl.when(c > 0)
            def _():
                late_cp(c).wait()

            nxt = jnp.minimum(c + 1, n_chunk - 1)
            for i in range(WG):
                cols = pl.ds(i * dh, dh)
                y = _dot(_unpack(hp[...]), _unpack(wqkv[c, :, cols]))
                relayout(nxt % 3, nxt, i * NSUB, WG * NSUB)
                for u in range(1, NSUB + (i + 1 < WG)):
                    r0 = (u - 1) * (n_seg * PRE // NSUB)
                    stage[nxt % 3, D // 2 + c // n_chunk] = y[r0:r0 + 2 * WG].astype(BF16)
                    if u < NSUB:
                        relayout(nxt % 3, nxt, i * NSUB + u, WG * NSUB)
                pre[c, :, cols] = y.astype(BF16)
                if 1 <= i <= lt:
                    mod[late_tile(jnp.maximum(c, 1)) + i - 1] = _dot(sc, lstage[c % 2, :, pl.ds((i - 1) * 128, 128)])[:8]
                wr = wo_rows // WG
                wo[jnp.maximum(p, 0), pl.ds(i * wr // 2, wr // 2), :] = pltpu.bitcast(
                    ostage[jnp.where(p >= 0, p % 2, 2), pl.ds(i * wr, wr), :], U32)
            return 0

        jax.lax.fori_loop(0, n_chunk, pre_body, 0)

    pl.run_scoped(load_phase,
                  pltpu.VMEM((n_seg, PRE, D), BF16),
                  pltpu.VMEM((n_seg * PRE, D), F32),
                  pltpu.VMEM((n_seg * PRE // 2, D), U32),
                  pltpu.VMEM((3, D // 2 + 1, 2 * WG, dh), BF16),
                  pltpu.VMEM((3, HG * dh, D), BF16),
                  pltpu.VMEM((4, D, 2 * D // 4), BF16),
                  pltpu.VMEM((2, D, 3 * 128), BF16))

    def main_phase(hn, att, h2, w13, w2):
        x_cp.wait()

        prep = ([(0, 0, cb) for cb in range(Fq // 128)]
                + [(1, rb, cb) for rb in range(r2 // 16) for cb in range(Dq // 128)])
        prep = [p + (range(7 * i, 7 * i + 7),) for p in prep for i in range(7)]

        def ffn_w_prepare(i, part, anchor):
            down, rb, cb, ks = prep[part]
            cols = pl.ds(cb * 128, 128)
            if down:
                st2[2 + i // n_trip, 0, pl.ds(0, 16), pl.ds(0, 128)] = anchor
                w = _operands(_strassen_rhs, [[st2[i % 2, r, pl.ds(rb * 16, 16), pl.ds(c * Dq + cb * 128, 128)]
                                               .astype(F32) for c in range(4)] for r in range(4)])
                rows = pl.ds(pl.multiple_of(jnp.minimum(i, n2 - 1) * (r2 // 2) + rb * 8, 8), 8)
                for k in ks:
                    w2[k, rows, cols] = _pack(w[k])
            else:
                st13[4 + i // n_trip, 0, :, pl.ds(0, 128)] = anchor
                w = _operands(_strassen_rhs, [[st13[i % 2 * 3, r, :, pl.ds(c * Fq + cb * 128, 128)]
                                               .astype(F32) for c in range(4)] for r in range(4)])
                for k in ks:
                    w13[i % 2, k, pl.ds(pl.multiple_of(i // 2 * 8, 8), 8), cols] = _pack(w[k])

        def ln1(s):
            hn[...] = ada_ln(x_buf[s, pl.ds(PRE, seg - PRE), :].astype(F32), 0)

        def ln2(s, r):
            rows = pl.ds(r, 16)
            xn = x_buf[s, rows, :].astype(F32) + mod_rows(2, 16) * att[0, rows, :]
            x_buf[s, rows, :] = xn.astype(BF16)
            h2[s, rows, :] = ada_ln(xn, 3).astype(BF16)

        att[0] = jnp.zeros(att.shape[1:], F32)
        ln1(0)
        n_hg = n_heads // HG

        def seg_step(trip, u, mem):
            lhs = jnp.concatenate([mem, hn[...]], axis=0).astype(BF16)
            qi = jax.lax.broadcasted_iota(jnp.int32, (L, L), 0)
            ki = jax.lax.broadcasted_iota(jnp.int32, (L, L), 1)
            mask = (qi < M) | (qi >= ki)
            pr = pl.ds(pl.multiple_of(trip * 2 * PRE, 2 * PRE), 2 * PRE)

            def proj(t, g):
                gi, cols = g * HG // WG, pl.ds(g * HG % WG * dh, HG * dh)
                y = _dot(lhs, _unpack(wqkv[3 * gi + t, :, cols]))
                y = jnp.concatenate([y[:M], pre[3 * gi + t, pr, cols].astype(F32)[u * PRE:(u + 1) * PRE], y[M:]], axis=0)
                return [y[:, h * dh:(h + 1) * dh] for h in range(HG)]

            def probs(q, k):
                sc_ = jnp.where(mask, _dot_nt(q, k.astype(BF16)) * (scale * LOG2E), -1e9 * LOG2E)
                e = jnp.exp2(sc_ - jnp.max(sc_, axis=-1, keepdims=True))
                den = jnp.sum(e, axis=-1, keepdims=True)
                r = pl.reciprocal(den, approx=True)
                return e, r * (2.0 - den * r)

            def mix(p, v):
                return jnp.concatenate([_dot(e, vh.astype(BF16)) * r for (e, r), vh in zip(p, v)], axis=1)

            def out_proj(o, g):
                y = _dot(o, _unpack(wo[g]))
                per = -(-len(prep) // (2 * n_hg))
                first = (u * n_hg + g) * per
                for i in range(first, min(first + per, len(prep))):
                    n = (i - first) * (D // 128) // per
                    ffn_w_prepare(trip, i, y[:16, n * 128:(n + 1) * 128].astype(BF16))
                return y

            o, acc, p, v = {}, None, None, None
            done = 0
            for g in range(n_hg):
                q = proj(0, g)
                k = proj(1, g)
                if 1 <= g <= seg // 16:
                    att[1 + trip // n_trip, pl.ds(0, 8), pl.ds(0, dh)] = q[0][:8]
                    ln2(jnp.maximum(2 * trip + u - 1, 0), (g - 1) * 16)
                if g == 0:
                    ln1(jnp.minimum(2 * trip + u + 1, n_seg - 1))
                if g == 1 and u == 0:
                    start(ffn_w_cps(trip + 1))
                if g:
                    o[g - 1] = mix(p, v)
                v = proj(2, g)
                p = [probs(qh, kh) for qh, kh in zip(q, k)]
                upto = g + 1 - LAG if g + 1 < n_hg else n_hg - 2
                while done < upto:
                    y = out_proj(o.pop(done), done)
                    acc = y if acc is None else acc + y
                    done += 1
            o[n_hg - 1] = mix(p, v)
            for g in range(done, n_hg):
                acc = acc + out_proj(o.pop(g), g)
            att[0] = acc[M:]
            return acc[:M]

        def seg_body(trip, mem):
            wait(ffn_w_cps(trip))
            for u in range(2):
                mem = seg_step(trip, u, mem)
            return mem

        jax.lax.fori_loop(0, n_trip, seg_body, mem0[...].astype(F32))

        wait(ffn_w_cps(jnp.int32(n_trip)))
        for r in range(0, seg, 16):
            ln2(n_seg - 1, r)

        sb = FFN_TM // seg

        qm = FFN_TM // 4

        def h_operand(k, row, n, col=0, width=Dq):
            per_row, per_chunk = WG * dh // Dq, D // 2 // qm
            return (k // (per_row * per_chunk), pl.ds(k // per_row % per_chunk * qm + row, n),
                    pl.ds(k % per_row * Dq + col, width))

        def a_operand(k, cols):
            per_chunk = D // 2 // qm
            return (2 + k // per_chunk, pl.ds(k % per_chunk * qm, qm // 2), cols)

        def ffn_lhs(i, row, half, col):
            rows = pl.ds(pl.multiple_of(row % seg, 16), 16)
            hs = [[h2[i * sb + r * qm // seg + row // seg, rows, pl.ds(c * Dq + col, 128)]
                   .astype(F32)[8 * half:8 * half + 8] for c in range(4)] for r in range(4)]
            for k, a in enumerate(_operands(_strassen_lhs, hs)):
                wqkv[h_operand(k, row + 8 * half, 8, col, 128)] = pltpu.bitcast(a, U32)

        lhs_parts = [(half, col) for half in range(2) for col in range(0, Dq, 128)]

        @pl.loop(0, qm // 16)
        def _(j):
            for half, col in lhs_parts:
                ffn_lhs(0, pl.multiple_of(j * 16, 16), half, col)

        def out_cp(i):
            return pltpu.make_async_copy(x_buf.at[pl.ds(i * sb, sb)], out_hbm.at[pl.ds(i * sb, sb)], sem_out.at[i % 2])

        n_blk = S // FFN_TM

        def ffn_body(i, _):
            @pl.when(i >= 2)
            def _():
                out_cp(i - 2).wait()

            zero, nxt = i // n_blk, jnp.minimum(i + 1, n_blk - 1)
            acts = [[] for _ in range(49)]
            for j in range(Fq // 128):
                cols = pl.ds(j * 128, 128)
                gate, up = (_results(lambda k: _dot(pltpu.bitcast(wqkv[h_operand(k, 0, qm)], F32),
                                                    _unpack(w13[t, k, :, cols]))) for t in range(2))
                act = [[_silu(g) * u for g, u in zip(gr, ur)] for gr, ur in zip(gate, up)]
                for k, a in enumerate(_operands(_strassen_lhs, act)):
                    if j < PARKED:
                        wqkv[a_operand(k, cols)] = _pack(a)
                    else:
                        acts[k].append(a.astype(BF16))

            def down_tile(k, n):
                m = _dot(jnp.concatenate([_unpack(wqkv[a_operand(k, pl.ds(0, PARKED * 128))])] + acts[k], axis=1),
                         _unpack(w2[k, :, pl.ds(n * 128, 128)]))
                piece, phase = divmod(k * (Dq // 128) + n, EVERY)
                if 0 <= piece < qm // 16 * len(lhs_parts) and phase == 0:
                    h2[n_seg + zero, pl.ds(0, 16), pl.ds(0, 128)] = m[:16].astype(BF16)
                    ffn_lhs(nxt, piece // len(lhs_parts) * 16, *lhs_parts[piece % len(lhs_parts)])
                return m

            def down(k):
                return jnp.concatenate([down_tile(k, n) for n in range(Dq // 128)], axis=1)

            y = jnp.concatenate([jnp.concatenate(row, axis=1) for row in _results(down)], axis=0)
            xn = x_buf[pl.ds(i * sb, sb)].astype(F32).reshape(FFN_TM, D)
            x_buf[pl.ds(i * sb, sb)] = (xn + mod_rows(5, FFN_TM) * y).reshape(sb, seg, D).astype(BF16)
            out_cp(i).start()
            return 0

        jax.lax.fori_loop(0, n_blk, ffn_body, 0)
        for i in range(max(n_blk - 2, 0), n_blk):
            out_cp(i).wait()

    pl.run_scoped(main_phase,
                  pltpu.VMEM((seg - PRE, D), F32),
                  pltpu.VMEM((2, seg, D), F32),
                  pltpu.VMEM((n_seg + 1, seg, D), BF16),
                  pltpu.VMEM((2, 49, D // 8, F // 4), U32),
                  pltpu.VMEM((49, F // 8, D // 4), U32))


@functools.partial(jax.jit, static_argnames=("A_seg_len",))
def pallas_adaLN_cond__memory_aug_recurrent_mem_tr__glu_gated_swiglu__prompt_kernel(
    A_x, A_mem0, A_Wq, A_Wk, A_Wv, A_Wo, A_seg_len, B_x, B_w1, B_w3, B_w2, c, w_mod,
):
    del B_x
    B, S, D = A_x.shape
    assert B == 1
    M = A_mem0.shape[1]
    _, H, Dh = A_Wq.shape
    F = B_w1.shape[1]
    seg = int(A_seg_len)
    n_seg, n_grp = S // seg, H // WG
    any_spec = pl.BlockSpec(memory_space=pl.ANY)
    out = pl.pallas_call(
        functools.partial(_kernel, n_heads=H, dh=Dh),
        out_shape=jax.ShapeDtypeStruct((n_seg, seg, D), A_x.dtype),
        in_specs=[any_spec] * 11,
        out_specs=any_spec,
        scratch_shapes=[
            pltpu.VMEM((n_seg, seg, D), BF16),
            pltpu.VMEM((M, D), BF16),
            pltpu.VMEM((1, D), BF16),
            pltpu.VMEM((3 * n_grp, D // 2, WG * Dh), U32),
            pltpu.VMEM((H // HG, HG * Dh // 2, D), U32),
            pltpu.VMEM((3 * n_grp, n_seg * PRE, WG * Dh), BF16),
            pltpu.VMEM((6 * D // 128, 8, 128), F32),
            pltpu.VMEM((5, 4, 16, F), BF16),
            pltpu.VMEM((3, 4, 32, D), BF16),
            pltpu.SemaphoreType.DMA((4,)),
            pltpu.SemaphoreType.DMA((6,)),
            pltpu.SemaphoreType.DMA((6,)),
            pltpu.SemaphoreType.DMA((2,)),
            pltpu.SemaphoreType.DMA((6,)),
            pltpu.SemaphoreType.DMA((2,)),
        ],
        compiler_params=pltpu.CompilerParams(vmem_limit_bytes=127 * 1024 * 1024),
    )(
        A_x.reshape(n_seg, seg, D), A_mem0.reshape(M, D),
        A_Wq.reshape(D // 2, 2 * H, Dh), A_Wk.reshape(D // 2, 2 * H, Dh), A_Wv.reshape(D // 2, 2 * H, Dh),
        A_Wo.reshape(H * Dh, D),
        B_w1.reshape(4, D // 4, F), B_w3.reshape(4, D // 4, F), B_w2.reshape(4, F // 4, D), c, w_mod,
    )
    return out.reshape(B, S, D)
```

```python
import functools

import jax
import jax.numpy as jnp
import jax.experimental.pallas as pl
import jax.experimental.pallas.tpu as pltpu

F32 = jnp.float32
BF16 = jnp.bfloat16
U32 = jnp.uint32
LOG2E = 1.4426950408889634

PRE = 8
WG = 8
NSUB = 4
HG = 4
LAG = 7
FFN_TM = 256
PARKED = 2
EVERY = 3


def _dot(a, b):
    return jax.lax.dot_general(a, b, (((1,), (0,)), ((), ())), preferred_element_type=F32)


def _dot_nt(a, b):
    return jax.lax.dot_general(a, b, (((1,), (1,)), ((), ())), preferred_element_type=F32)


def _silu(x):
    t = 0.5 * x
    return t * jnp.tanh(t) + t


def _layernorm(x):
    m = jnp.mean(x, axis=-1, keepdims=True)
    d = x - m
    v = jnp.mean(d * d, axis=-1, keepdims=True)
    return d * jax.lax.rsqrt(v + 1e-5)


def _pack(x):
    return pltpu.bitcast(x.astype(BF16), U32)


def _unpack(w):
    return pltpu.bitcast(w, BF16)


def _strassen_lhs(a11, a12, a21, a22):
    return (a11 + a22, a21 + a22, a11, a22, a11 + a12, a21 - a11, a12 - a22)


def _strassen_rhs(b11, b12, b21, b22):
    return (b11 + b22, b11, b12 - b22, b21 - b11, b22, b11 + b12, b21 + b22)


def _strassen_out(m):
    return (m[0] + m[3] - m[4] + m[6], m[2] + m[4], m[1] + m[3], m[0] - m[1] + m[2] + m[5])


def _operands(level, x):
    outer = [level(x[r][c], x[r][c + 2], x[r + 2][c], x[r + 2][c + 2]) for r in range(2) for c in range(2)]
    return [y for i in range(7) for y in level(*[o[i] for o in outer])]


def _results(product):
    inner = [_strassen_out([product(7 * i + j) for j in range(7)]) for i in range(7)]
    outer = [_strassen_out([m[rc] for m in inner]) for rc in range(4)]
    return [[outer[r % 2 * 2 + c % 2][r // 2 * 2 + c // 2] for c in range(4)] for r in range(4)]


def _kernel(x_hbm, mem0_hbm, wq_hbm, wk_hbm, wv_hbm, wo_hbm, w1_hbm, w3_hbm, w2_hbm, c_hbm, wmod_hbm,
            out_hbm,
            x_buf, mem0, c_buf, wqkv, wo, pre, mod, st13, st2,
            sem_x, sem_stage, sem_m, sem_o, sem_ffn, sem_out, *, n_heads, dh):
    n_seg, seg, D = x_buf.shape
    n_trip = n_seg // 2
    S = n_seg * seg
    M = mem0.shape[0]
    L = M + seg
    scale = dh ** -0.5
    F = w1_hbm.shape[2]
    n_grp = n_heads // WG
    w_hbms = (wq_hbm, wk_hbm, wv_hbm)

    x_cp = pltpu.make_async_copy(x_hbm, x_buf, sem_x.at[0])

    Dq, Fq = D // 4, F // 4
    r2 = st2.shape[2]
    n2 = Fq // r2
    assert n_trip * 8 == Dq and n2 * r2 == Fq and n2 <= n_trip

    def ffn_w_cps(i):
        slot, i13, i2 = i & 1, jnp.minimum(i, n_trip - 1), jnp.minimum(i, n2 - 1)
        srcs = [w_hbm.at[:, pl.ds(pl.multiple_of((i13 >> 1) * 16, 16), 16), :] for w_hbm in (w1_hbm, w3_hbm)]
        srcs += [w2_hbm.at[:, pl.ds(pl.multiple_of(i2 * r2, r2), r2), :]]
        dsts = [st13.at[2 * slot], st13.at[2 * slot + 1], st2.at[slot]]
        return [pltpu.make_async_copy(a, b, sem_ffn.at[slot * 3 + n]) for n, (a, b) in enumerate(zip(srcs, dsts))]

    def start(cps):
        for cp in cps:
            cp.start()

    def wait(cps):
        for cp in cps:
            cp.wait()

    def mod_rows(j, rows):
        tile = jnp.concatenate([mod[j * (D // 128) + n] for n in range(D // 128)], axis=1)
        return jnp.concatenate([tile] * (rows // 8), axis=0)

    def ada_ln(x, j):
        return _layernorm(x) * (1.0 + mod_rows(j + 1, x.shape[0])) + mod_rows(j, x.shape[0])

    def load_phase(xp, lnp, hp, stage, ostage, mstage, lstage):
        xp_cps = [pltpu.make_async_copy(x_hbm.at[:, pl.ds(0, PRE), :], xp, sem_x.at[1]),
                  pltpu.make_async_copy(c_hbm, c_buf, sem_x.at[2]),
                  pltpu.make_async_copy(mem0_hbm, mem0, sem_x.at[3])]
        n_mod, _, mod_cols = mstage.shape

        def wmod_cp(j):
            return pltpu.make_async_copy(wmod_hbm.at[:, pl.ds(pl.multiple_of(j * mod_cols, mod_cols), mod_cols)],
                                         mstage.at[j], sem_m.at[j])

        lt = lstage.shape[2] // 128

        def late_tile(c):
            return jnp.minimum(2 * D // 128 + (c - 1) * lt, 6 * D // 128 - lt)

        def late_cp(c):
            return pltpu.make_async_copy(wmod_hbm.at[:, pl.ds(pl.multiple_of(late_tile(c) * 128, 128), lt * 128)],
                                         lstage.at[c & 1], sem_m.at[n_mod + (c & 1)])

        n_wo, wo_rows = wo.shape[0], ostage.shape[1]

        def wo_cp(p):
            return pltpu.make_async_copy(wo_hbm.at[pl.ds(pl.multiple_of(p * wo_rows, wo_rows), wo_rows), :],
                                         ostage.at[p & 1], sem_o.at[p & 1])

        def w_cps(t, g):
            return [pltpu.make_async_copy(w_hbms[t].at[:, pl.ds(pl.multiple_of(p * n_heads + g * WG, WG), WG), :],
                                          stage.at[t, pl.ds(0, D // 2), pl.ds(p * WG, WG), :], sem_stage.at[2 * t + p])
                    for p in range(2)]

        def relayout(t, c, part, n_part):
            per = D // 2 // 8 // n_part
            for b in range(per):
                rows = pl.ds(pl.multiple_of((part * per + b) * 8, 8), 8)
                w = jnp.swapaxes(pltpu.bitcast(stage[t, rows], U32), 0, 1)
                for j in range(WG // 2):
                    even, odd = w[j], w[WG // 2 + j]
                    wqkv[c, rows, pl.ds(2 * j * dh, dh)] = (even & jnp.uint32(0xFFFF)) | (odd << 16)
                    wqkv[c, rows, pl.ds((2 * j + 1) * dh, dh)] = (even >> 16) | (odd & jnp.uint32(0xFFFF0000))

        start(xp_cps)
        start(w_cps(0, 0))
        wmod_cp(0).start()
        ostage[2] = jnp.zeros(ostage.shape[1:], BF16)
        lstage[0] = jnp.zeros(lstage.shape[1:], BF16)
        wait(xp_cps)
        for j in range(1, n_mod):
            wmod_cp(j).start()
        sc = jnp.broadcast_to(_silu(c_buf[...].astype(F32)), (16, D)).astype(BF16)
        nb = 64 // PRE

        @pl.loop(0, n_seg // nb)
        def _(i):
            xs = xp[pl.ds(i * nb, nb)].astype(F32).reshape(nb * PRE, D)
            lnp[pl.ds(pl.multiple_of(i * nb * PRE, nb * PRE), nb * PRE), :] = _layernorm(xs)

        wait(w_cps(0, 0))
        start(w_cps(1, 0))

        @pl.loop(0, 8)
        def _(i):
            relayout(0, 0, i, 8)

        @pl.loop(0, n_mod)
        def _(j):
            wmod_cp(j).wait()
            y = _dot(sc, mstage[j])
            for n in range(mod_cols // 128):
                mod[j * (mod_cols // 128) + n] = y[:8, n * 128:(n + 1) * 128]

        start(w_cps(2, 0))

        @pl.loop(0, n_seg // nb)
        def _(i):
            ln = lnp[pl.ds(pl.multiple_of(i * nb * PRE, nb * PRE), nb * PRE), :]
            rows = pl.ds(pl.multiple_of(i * (nb * PRE // 2), nb * PRE // 2), nb * PRE // 2)
            hp[rows, :] = _pack(ln * (1.0 + mod_rows(1, nb * PRE)) + mod_rows(0, nb * PRE))

        n_chunk = 3 * n_grp
        assert (n_chunk - 1) * lt * 128 >= 4 * D

        def pre_body(c, carry):
            g, t_now = carry
            p = c - (n_chunk - n_wo)
            last = c + 1 == n_chunk
            pl.when(jnp.logical_and(p + 1 >= 0, p + 1 < n_wo))(lambda: wo_cp(p + 1).start())
            pl.when(c + 1 < n_chunk)(lambda: late_cp(c + 1).start())
            pl.when(c == n_chunk - 3)(x_cp.start)
            pl.when(last)(lambda: start(ffn_w_cps(jnp.int32(0))))
            for t in range(3):
                @pl.when(t_now == t)
                def _():
                    pl.when(g + 1 < n_grp)(lambda: start(w_cps(t, g + 1)))
                    if t < 2:
                        wait(w_cps(t + 1, g))
                    else:
                        pl.when(g + 1 < n_grp)(lambda: wait(w_cps(0, g + 1)))

            pl.when(p >= 0)(lambda: wo_cp(p).wait())
            pl.when(c > 0)(lambda: late_cp(c).wait())
            t_next = jnp.where(t_now == 2, 0, t_now + 1)
            nxt, slot = jnp.where(last, c, c + 1), jnp.where(last, t_now, t_next)
            for i in range(WG):
                cols = pl.ds(i * dh, dh)
                y = _dot(_unpack(hp[...]), _unpack(wqkv[c, :, cols]))
                relayout(slot, nxt, i * NSUB, WG * NSUB)
                for u in range(1, NSUB + (i + 1 < WG)):
                    r0 = (u - 1) * (n_seg * PRE // NSUB)
                    stage[slot, D // 2 + (c >> 16)] = y[r0:r0 + 2 * WG].astype(BF16)
                    if u < NSUB:
                        relayout(slot, nxt, i * NSUB + u, WG * NSUB)
                pre[c, :, cols] = y.astype(BF16)
                if 1 <= i <= lt:
                    mod[late_tile(jnp.maximum(c, 1)) + i - 1] = _dot(sc, lstage[c & 1, :, pl.ds((i - 1) * 128, 128)])[:8]
                wr = wo_rows // WG
                wo[jnp.maximum(p, 0), pl.ds(i * wr // 2, wr // 2), :] = pltpu.bitcast(
                    ostage[jnp.where(p >= 0, p & 1, 2), pl.ds(i * wr, wr), :], U32)
            return jnp.where(t_now == 2, g + 1, g), t_next

        jax.lax.fori_loop(0, n_chunk, pre_body, (jnp.int32(0), jnp.int32(0)))

    pl.run_scoped(load_phase,
                  pltpu.VMEM((n_seg, PRE, D), BF16),
                  pltpu.VMEM((n_seg * PRE, D), F32),
                  pltpu.VMEM((n_seg * PRE // 2, D), U32),
                  pltpu.VMEM((3, D // 2 + 1, 2 * WG, dh), BF16),
                  pltpu.VMEM((3, HG * dh, D), BF16),
                  pltpu.VMEM((4, D, 2 * D // 4), BF16),
                  pltpu.VMEM((2, D, 3 * 128), BF16))

    def main_phase(hn, att, h2, w13, w2):
        x_cp.wait()

        prep = ([(0, 0, cb) for cb in range(Fq // 128)]
                + [(1, rb, cb) for rb in range(r2 // 16) for cb in range(Dq // 128)])
        prep = [p + (range(7 * i, 7 * i + 7),) for p in prep for i in range(7)]

        def ffn_w_prepare(i, part, anchor):
            down, rb, cb, ks = prep[part]
            cols = pl.ds(cb * 128, 128)
            if down:
                st2[2 + (i >> 16), 0, pl.ds(0, 16), pl.ds(0, 128)] = anchor
                w = _operands(_strassen_rhs, [[st2[i & 1, r, pl.ds(rb * 16, 16), pl.ds(c * Dq + cb * 128, 128)]
                                               .astype(F32) for c in range(4)] for r in range(4)])
                rows = pl.ds(pl.multiple_of(jnp.minimum(i, n2 - 1) * (r2 // 2) + rb * 8, 8), 8)
                for k in ks:
                    w2[k, rows, cols] = _pack(w[k])
            else:
                st13[4 + (i >> 16), 0, :, pl.ds(0, 128)] = anchor
                w = _operands(_strassen_rhs, [[st13[(i & 1) * 3, r, :, pl.ds(c * Fq + cb * 128, 128)]
                                               .astype(F32) for c in range(4)] for r in range(4)])
                for k in ks:
                    w13[i & 1, k, pl.ds(pl.multiple_of((i >> 1) * 8, 8), 8), cols] = _pack(w[k])

        def ln1(s):
            hn[...] = ada_ln(x_buf[s, pl.ds(PRE, seg - PRE), :].astype(F32), 0)

        def ln2(s, r):
            rows = pl.ds(r, 16)
            xn = x_buf[s, rows, :].astype(F32) + mod_rows(2, 16) * att[0, rows, :]
            x_buf[s, rows, :] = xn.astype(BF16)
            h2[s, rows, :] = ada_ln(xn, 3).astype(BF16)

        att[0] = jnp.zeros(att.shape[1:], F32)
        ln1(0)
        n_hg = n_heads // HG

        def seg_step(trip, u, mem):
            lhs = jnp.concatenate([mem, hn[...]], axis=0).astype(BF16)
            qi = jax.lax.broadcasted_iota(jnp.int32, (L, L), 0)
            ki = jax.lax.broadcasted_iota(jnp.int32, (L, L), 1)
            mask = (qi < M) | (qi >= ki)
            pr = pl.ds(pl.multiple_of(trip * 2 * PRE, 2 * PRE), 2 * PRE)

            def proj(t, g):
                gi, cols = g * HG // WG, pl.ds(g * HG % WG * dh, HG * dh)
                y = _dot(lhs, _unpack(wqkv[3 * gi + t, :, cols]))
                y = jnp.concatenate([y[:M], pre[3 * gi + t, pr, cols].astype(F32)[u * PRE:(u + 1) * PRE], y[M:]], axis=0)
                return [y[:, h * dh:(h + 1) * dh] for h in range(HG)]

            def probs(q, k):
                sc_ = jnp.where(mask, _dot_nt(q, k.astype(BF16)) * (scale * LOG2E), -1e9 * LOG2E)
                e = jnp.exp2(sc_ - jnp.max(sc_, axis=-1, keepdims=True))
                den = jnp.sum(e, axis=-1, keepdims=True)
                r = pl.reciprocal(den, approx=True)
                return e, r * (2.0 - den * r)

            def mix(p, v):
                return jnp.concatenate([_dot(e, vh.astype(BF16)) * r for (e, r), vh in zip(p, v)], axis=1)

            def out_proj(o, g):
                y = _dot(o, _unpack(wo[g]))
                per = -(-len(prep) // (2 * n_hg))
                first = (u * n_hg + g) * per
                for i in range(first, min(first + per, len(prep))):
                    n = (i - first) * (D // 128) // per
                    ffn_w_prepare(trip, i, y[:16, n * 128:(n + 1) * 128].astype(BF16))
                return y

            o, acc, p, v = {}, None, None, None
            done = 0
            for g in range(n_hg):
                q = proj(0, g)
                k = proj(1, g)
                if 1 <= g <= seg // 16:
                    att[1 + (trip >> 16), pl.ds(0, 8), pl.ds(0, dh)] = q[0][:8]
                    ln2(jnp.maximum(2 * trip + u - 1, 0), (g - 1) * 16)
                if g == 0:
                    ln1(jnp.minimum(2 * trip + u + 1, n_seg - 1))
                if g == 1 and u == 0:
                    start(ffn_w_cps(trip + 1))
                if g:
                    o[g - 1] = mix(p, v)
                v = proj(2, g)
                p = [probs(qh, kh) for qh, kh in zip(q, k)]
                upto = g + 1 - LAG if g + 1 < n_hg else n_hg - 2
                while done < upto:
                    y = out_proj(o.pop(done), done)
                    acc = y if acc is None else acc + y
                    done += 1
            o[n_hg - 1] = mix(p, v)
            for g in range(done, n_hg):
                acc = acc + out_proj(o.pop(g), g)
            att[0] = acc[M:]
            return acc[:M]

        def seg_body(trip, mem):
            wait(ffn_w_cps(trip))
            for u in range(2):
                mem = seg_step(trip, u, mem)
            return mem

        jax.lax.fori_loop(0, n_trip, seg_body, mem0[...].astype(F32))

        wait(ffn_w_cps(jnp.int32(n_trip)))
        for r in range(0, seg, 16):
            ln2(n_seg - 1, r)

        sb, qm = FFN_TM // seg, FFN_TM // 4

        def h_operand(k, row, n, col=0, width=Dq):
            per_row, per_chunk = WG * dh // Dq, D // 2 // qm
            return (k // (per_row * per_chunk), pl.ds(k // per_row % per_chunk * qm + row, n),
                    pl.ds(k % per_row * Dq + col, width))

        def a_operand(k, cols):
            per_chunk = D // 2 // qm
            return (2 + k // per_chunk, pl.ds(k % per_chunk * qm, qm // 2), cols)

        def ffn_lhs(i, row, half, col):
            rows = pl.ds(pl.multiple_of(row % seg, 16), 16)
            hs = [[h2[i * sb + r * qm // seg + row // seg, rows, pl.ds(c * Dq + col, 128)]
                   .astype(F32)[8 * half:8 * half + 8] for c in range(4)] for r in range(4)]
            for k, a in enumerate(_operands(_strassen_lhs, hs)):
                wqkv[h_operand(k, row + 8 * half, 8, col, 128)] = pltpu.bitcast(a, U32)

        lhs_parts = [(half, col) for half in range(2) for col in range(0, Dq, 128)]

        @pl.loop(0, qm // 16)
        def _(j):
            for half, col in lhs_parts:
                ffn_lhs(0, pl.multiple_of(j * 16, 16), half, col)

        def out_cp(i):
            return pltpu.make_async_copy(x_buf.at[pl.ds(i * sb, sb)], out_hbm.at[pl.ds(i * sb, sb)], sem_out.at[i & 1])

        n_blk = S // FFN_TM

        def ffn_body(i, _):
            @pl.when(i >= 2)
            def _():
                out_cp(i - 2).wait()

            zero, nxt = i >> 16, jnp.minimum(i + 1, n_blk - 1)
            acts = [[] for _ in range(49)]
            for j in range(Fq // 128):
                cols = pl.ds(j * 128, 128)
                gate, up = (_results(lambda k: _dot(pltpu.bitcast(wqkv[h_operand(k, 0, qm)], F32),
                                                    _unpack(w13[t, k, :, cols]))) for t in range(2))
                act = [[_silu(g) * u for g, u in zip(gr, ur)] for gr, ur in zip(gate, up)]
                for k, a in enumerate(_operands(_strassen_lhs, act)):
                    if j < PARKED:
                        wqkv[a_operand(k, cols)] = _pack(a)
                    else:
                        acts[k].append(a.astype(BF16))

            def down_tile(k, n):
                m = _dot(jnp.concatenate([_unpack(wqkv[a_operand(k, pl.ds(0, PARKED * 128))])] + acts[k], axis=1),
                         _unpack(w2[k, :, pl.ds(n * 128, 128)]))
                piece, phase = divmod(k * (Dq // 128) + n, EVERY)
                if 0 <= piece < qm // 16 * len(lhs_parts) and phase == 0:
                    h2[n_seg + zero, pl.ds(0, 16), pl.ds(0, 128)] = m[:16].astype(BF16)
                    ffn_lhs(nxt, piece // len(lhs_parts) * 16, *lhs_parts[piece % len(lhs_parts)])
                return m

            def down(k):
                return jnp.concatenate([down_tile(k, n) for n in range(Dq // 128)], axis=1)

            y = jnp.concatenate([jnp.concatenate(row, axis=1) for row in _results(down)], axis=0)
            xn = x_buf[pl.ds(i * sb, sb)].astype(F32).reshape(FFN_TM, D)
            x_buf[pl.ds(i * sb, sb)] = (xn + mod_rows(5, FFN_TM) * y).reshape(sb, seg, D).astype(BF16)
            out_cp(i).start()
            return 0

        jax.lax.fori_loop(0, n_blk, ffn_body, 0)
        for i in range(max(n_blk - 2, 0), n_blk):
            out_cp(i).wait()

    pl.run_scoped(main_phase,
                  pltpu.VMEM((seg - PRE, D), F32),
                  pltpu.VMEM((2, seg, D), F32),
                  pltpu.VMEM((n_seg + 1, seg, D), BF16),
                  pltpu.VMEM((2, 49, D // 8, F // 4), U32),
                  pltpu.VMEM((49, F // 8, D // 4), U32))


@functools.partial(jax.jit, static_argnames=("A_seg_len",))
def pallas_adaLN_cond__memory_aug_recurrent_mem_tr__glu_gated_swiglu__prompt_kernel(
    A_x, A_mem0, A_Wq, A_Wk, A_Wv, A_Wo, A_seg_len, B_x, B_w1, B_w3, B_w2, c, w_mod,
):
    del B_x
    B, S, D = A_x.shape
    assert B == 1
    M = A_mem0.shape[1]
    _, H, Dh = A_Wq.shape
    F = B_w1.shape[1]
    seg = int(A_seg_len)
    n_seg, n_grp = S // seg, H // WG
    any_spec = pl.BlockSpec(memory_space=pl.ANY)
    out = pl.pallas_call(
        functools.partial(_kernel, n_heads=H, dh=Dh),
        out_shape=jax.ShapeDtypeStruct((n_seg, seg, D), A_x.dtype),
        in_specs=[any_spec] * 11,
        out_specs=any_spec,
        scratch_shapes=[
            pltpu.VMEM((n_seg, seg, D), BF16),
            pltpu.VMEM((M, D), BF16),
            pltpu.VMEM((1, D), BF16),
            pltpu.VMEM((3 * n_grp, D // 2, WG * Dh), U32),
            pltpu.VMEM((H // HG, HG * Dh // 2, D), U32),
            pltpu.VMEM((3 * n_grp, n_seg * PRE, WG * Dh), BF16),
            pltpu.VMEM((6 * D // 128, 8, 128), F32),
            pltpu.VMEM((5, 4, 16, F), BF16),
            pltpu.VMEM((3, 4, 32, D), BF16),
            pltpu.SemaphoreType.DMA((4,)),
            pltpu.SemaphoreType.DMA((6,)),
            pltpu.SemaphoreType.DMA((6,)),
            pltpu.SemaphoreType.DMA((2,)),
            pltpu.SemaphoreType.DMA((6,)),
            pltpu.SemaphoreType.DMA((2,)),
        ],
        compiler_params=pltpu.CompilerParams(vmem_limit_bytes=127 * 1024 * 1024),
    )(
        A_x.reshape(n_seg, seg, D), A_mem0.reshape(M, D),
        A_Wq.reshape(D // 2, 2 * H, Dh), A_Wk.reshape(D // 2, 2 * H, Dh), A_Wv.reshape(D // 2, 2 * H, Dh),
        A_Wo.reshape(H * Dh, D),
        B_w1.reshape(4, D // 4, F), B_w3.reshape(4, D // 4, F), B_w2.reshape(4, F // 4, D), c, w_mod,
    )
    return out.reshape(B, S, D)
```

```python
import functools

import jax
import jax.numpy as jnp
import jax.experimental.pallas as pl
import jax.experimental.pallas.tpu as pltpu

F32 = jnp.float32
BF16 = jnp.bfloat16
U32 = jnp.uint32
LOG2E = 1.4426950408889634

PRE = 8
WG = 8
HG = 4
LAG = 7
FFN_TM = 256
PARKED = 2
CUTS = (0, 14, 28, 35, 42, 49)


def _dot(a, b):
    return jax.lax.dot_general(a, b, (((1,), (0,)), ((), ())), preferred_element_type=F32)


def _dot_nt(a, b):
    return jax.lax.dot_general(a, b, (((1,), (1,)), ((), ())), preferred_element_type=F32)


def _silu(x):
    t = 0.5 * x
    return t * jnp.tanh(t) + t


def _layernorm(x):
    m = jnp.mean(x, axis=-1, keepdims=True)
    d = x - m
    v = jnp.mean(d * d, axis=-1, keepdims=True)
    return d * jax.lax.rsqrt(v + 1e-5)


def _pack(x):
    return pltpu.bitcast(x.astype(BF16), U32)


def _unpack(w):
    return pltpu.bitcast(w, BF16)


def _strassen_lhs(a11, a12, a21, a22):
    return (a11 + a22, a21 + a22, a11, a22, a11 + a12, a21 - a11, a12 - a22)


def _strassen_rhs(b11, b12, b21, b22):
    return (b11 + b22, b11, b12 - b22, b21 - b11, b22, b11 + b12, b21 + b22)


def _strassen_out(m):
    return (m[0] + m[3] - m[4] + m[6], m[2] + m[4], m[1] + m[3], m[0] - m[1] + m[2] + m[5])


def _operands(level, x):
    outer = [level(x[r][c], x[r][c + 2], x[r + 2][c], x[r + 2][c + 2]) for r in range(2) for c in range(2)]
    return [y for i in range(7) for y in level(*[o[i] for o in outer])]


def _results(product):
    inner = [_strassen_out([product(7 * i + j) for j in range(7)]) for i in range(7)]
    outer = [_strassen_out([m[rc] for m in inner]) for rc in range(4)]
    return [[outer[r % 2 * 2 + c % 2][r // 2 * 2 + c // 2] for c in range(4)] for r in range(4)]


def _kernel(x_hbm, mem0_hbm, wq_hbm, wk_hbm, wv_hbm, wo_hbm, w1_hbm, w3_hbm, w2_hbm, c_hbm, wmod_hbm,
            out_hbm,
            x_buf, mem0, c_buf, wqkv, wo, pre, mod, st13, st2,
            sem_x, sem_stage, sem_m, sem_o, sem_ffn, sem_out, *, n_heads, dh):
    n_seg, seg, D = x_buf.shape
    n_trip = n_seg // 2
    S = n_seg * seg
    M = mem0.shape[0]
    L = M + seg
    scale = dh ** -0.5
    F = w1_hbm.shape[2]
    n_grp = n_heads // WG
    w_hbms = (wq_hbm, wk_hbm, wv_hbm)

    x_cp = pltpu.make_async_copy(x_hbm, x_buf, sem_x.at[0])

    Dq, Fq = D // 4, F // 4
    r2 = st2.shape[2]
    n2 = Fq // r2
    assert n_trip * 8 == Dq and n2 * r2 == Fq and n2 <= n_trip

    def ffn_w_cps(i):
        slot, i13, i2 = i & 1, jnp.minimum(i, n_trip - 1), jnp.minimum(i, n2 - 1)
        srcs = [w_hbm.at[:, pl.ds(pl.multiple_of((i13 >> 1) * 16, 16), 16), :] for w_hbm in (w1_hbm, w3_hbm)]
        srcs += [w2_hbm.at[:, pl.ds(pl.multiple_of(i2 * r2, r2), r2), :]]
        dsts = [st13.at[2 * slot], st13.at[2 * slot + 1], st2.at[slot]]
        return [pltpu.make_async_copy(a, b, sem_ffn.at[slot * 3 + n]) for n, (a, b) in enumerate(zip(srcs, dsts))]

    def start(cps):
        for cp in cps:
            cp.start()

    def wait(cps):
        for cp in cps:
            cp.wait()

    def mod_rows(j, rows):
        tile = jnp.concatenate([mod[j * (D // 128) + n] for n in range(D // 128)], axis=1)
        return jnp.concatenate([tile] * (rows // 8), axis=0)

    def ada_ln(x, j):
        return _layernorm(x) * (1.0 + mod_rows(j + 1, x.shape[0])) + mod_rows(j, x.shape[0])

    def load_phase(xp, lnp, hp, stage, ostage, mstage, lstage):
        xp_cps = [pltpu.make_async_copy(x_hbm.at[:, pl.ds(0, PRE), :], xp, sem_x.at[1]),
                  pltpu.make_async_copy(c_hbm, c_buf, sem_x.at[2]),
                  pltpu.make_async_copy(mem0_hbm, mem0, sem_x.at[3])]
        n_mod, _, mod_cols = mstage.shape

        def wmod_cp(j):
            return pltpu.make_async_copy(wmod_hbm.at[:, pl.ds(pl.multiple_of(j * mod_cols, mod_cols), mod_cols)],
                                         mstage.at[j], sem_m.at[j])

        lt = lstage.shape[2] // 128

        def late_tile(c):
            return jnp.minimum(2 * D // 128 + (c - 1) * lt, 6 * D // 128 - lt)

        def late_cp(c):
            return pltpu.make_async_copy(wmod_hbm.at[:, pl.ds(pl.multiple_of(late_tile(c) * 128, 128), lt * 128)],
                                         lstage.at[c & 1], sem_m.at[n_mod + (c & 1)])

        n_wo, wo_rows = wo.shape[0], ostage.shape[1]

        def wo_cp(p):
            return pltpu.make_async_copy(wo_hbm.at[pl.ds(pl.multiple_of(p * wo_rows, wo_rows), wo_rows), :],
                                         ostage.at[p & 1], sem_o.at[p & 1])

        def w_cps(t, g):
            return [pltpu.make_async_copy(w_hbms[t].at[:, pl.ds(pl.multiple_of(p * n_heads + g * WG, WG), WG), :],
                                          stage.at[t, pl.ds(0, D // 2), pl.ds(p * WG, WG), :], sem_stage.at[2 * t + p])
                    for p in range(2)]

        def relayout(t, c, part, n_part):
            per = D // 2 // 8 // n_part
            for b in range(per):
                rows = pl.ds(pl.multiple_of((part * per + b) * 8, 8), 8)
                w = jnp.swapaxes(pltpu.bitcast(stage[t, rows], U32), 0, 1)
                for j in range(WG // 2):
                    even, odd = w[j], w[WG // 2 + j]
                    wqkv[c, rows, pl.ds(2 * j * dh, dh)] = (even & jnp.uint32(0xFFFF)) | (odd << 16)
                    wqkv[c, rows, pl.ds((2 * j + 1) * dh, dh)] = (even >> 16) | (odd & jnp.uint32(0xFFFF0000))

        start(xp_cps)
        start(w_cps(0, 0))
        wmod_cp(0).start()
        ostage[2] = jnp.zeros(ostage.shape[1:], BF16)
        lstage[0] = jnp.zeros(lstage.shape[1:], BF16)
        wait(xp_cps)
        for j in range(1, n_mod):
            wmod_cp(j).start()
        sc = jnp.broadcast_to(_silu(c_buf[...].astype(F32)), (16, D)).astype(BF16)
        nb = 64 // PRE

        @pl.loop(0, n_seg // nb)
        def _(i):
            xs = xp[pl.ds(i * nb, nb)].astype(F32).reshape(nb * PRE, D)
            lnp[pl.ds(pl.multiple_of(i * nb * PRE, nb * PRE), nb * PRE), :] = _layernorm(xs)

        wait(w_cps(0, 0))
        start(w_cps(1, 0))

        @pl.loop(0, 8)
        def _(i):
            relayout(0, 0, i, 8)

        @pl.loop(0, n_mod)
        def _(j):
            wmod_cp(j).wait()
            y = _dot(sc, mstage[j])
            for n in range(mod_cols // 128):
                mod[j * (mod_cols // 128) + n] = y[:8, n * 128:(n + 1) * 128]

        start(w_cps(2, 0))

        hm = n_seg * PRE // 2

        @pl.loop(0, hm // 32)
        def _(i):
            top, bot = (lnp[pl.ds(pl.multiple_of(r * hm + i * 32, 32), 32), :] * (1.0 + mod_rows(1, 32))
                        + mod_rows(0, 32) for r in range(2))
            for k, a in enumerate(_strassen_lhs(top[:, :D // 2], top[:, D // 2:], bot[:, :D // 2], bot[:, D // 2:])):
                hp[k, pl.ds(pl.multiple_of(i * 16, 16), 16), :] = _pack(a)

        n_chunk = 3 * n_grp
        assert (n_chunk - 1) * lt * 128 >= 4 * D

        def pre_body(c, carry):
            g, t_now = carry
            p = c - (n_chunk - n_wo)
            last = c + 1 == n_chunk
            pl.when(jnp.logical_and(p + 1 >= 0, p + 1 < n_wo))(lambda: wo_cp(p + 1).start())
            pl.when(c + 1 < n_chunk)(lambda: late_cp(c + 1).start())
            pl.when(c == n_chunk - 3)(x_cp.start)
            pl.when(last)(lambda: start(ffn_w_cps(jnp.int32(0))))
            for t in range(3):
                @pl.when(t_now == t)
                def _():
                    pl.when(g + 1 < n_grp)(lambda: start(w_cps(t, g + 1)))
                    if t < 2:
                        wait(w_cps(t + 1, g))
                    else:
                        pl.when(g + 1 < n_grp)(lambda: wait(w_cps(0, g + 1)))

            pl.when(p >= 0)(lambda: wo_cp(p).wait())
            pl.when(c > 0)(lambda: late_cp(c).wait())
            t_next = jnp.where(t_now == 2, 0, t_now + 1)
            nxt, slot = jnp.where(last, c, c + 1), jnp.where(last, t_now, t_next)
            sub, n_sub, prev = 0, D // 2 // 8, None
            for n in range(WG // 2):
                cols = [pl.ds((hf * WG // 2 + n) * dh, dh) for hf in range(2)]
                m = {}
                for i, k in enumerate((1, 0, 3, 4, 2, 5, 6)):
                    w = [_unpack(wqkv[c, pl.ds(r * (D // 4), D // 4), cols[hf]]) for r in range(2) for hf in range(2)]
                    rhs = {1: w[0], 4: w[3]}.get(k)
                    if rhs is None:
                        rhs = _strassen_rhs(*[b.astype(F32) for b in w])[k].astype(BF16)
                    m[k] = _dot(_unpack(hp[k]), rhs)
                    first = sub
                    while sub < min(n_sub, (n * 7 + i + 1) * n_sub // (WG // 2 * 7 - 1)):
                        if prev is not None:
                            r0 = 32 + (sub - first) * 80
                            stage[slot, D // 2 + (c >> 16)] = prev[r0:r0 + 2 * WG].astype(BF16)
                        relayout(slot, nxt, sub, n_sub)
                        sub += 1
                    prev = m[k]
                y = _strassen_out(m)
                for r in range(2):
                    for hf in range(2):
                        pre[c, pl.ds(r * hm, hm), cols[hf]] = y[2 * r + hf].astype(BF16)
                if n < lt:
                    mod[late_tile(jnp.maximum(c, 1)) + n] = _dot(sc, lstage[c & 1, :, pl.ds(n * 128, 128)])[:8]
                wr = wo_rows // (WG // 2)
                wo[jnp.maximum(p, 0), pl.ds(n * wr // 2, wr // 2), :] = pltpu.bitcast(
                    ostage[jnp.where(p >= 0, p & 1, 2), pl.ds(n * wr, wr), :], U32)
            return jnp.where(t_now == 2, g + 1, g), t_next

        jax.lax.fori_loop(0, n_chunk, pre_body, (jnp.int32(0), jnp.int32(0)))

    pl.run_scoped(load_phase,
                  pltpu.VMEM((n_seg, PRE, D), BF16),
                  pltpu.VMEM((n_seg * PRE, D), F32),
                  pltpu.VMEM((7, n_seg * PRE // 4, D // 2), U32),
                  pltpu.VMEM((3, D // 2 + 1, 2 * WG, dh), BF16),
                  pltpu.VMEM((3, HG * dh, D), BF16),
                  pltpu.VMEM((4, D, 2 * D // 4), BF16),
                  pltpu.VMEM((2, D, 3 * 128), BF16))

    def main_phase(hn, att, h2, w13, w2):
        x_cp.wait()

        prep = ([(0, 0, cb) for cb in range(Fq // 128)]
                + [(1, rb, cb) for rb in range(r2 // 16) for cb in range(Dq // 128)])
        prep = [p + (range(7 * i, 7 * i + 7),) for p in prep for i in range(7)]

        def ffn_w_prepare(i, part, anchor):
            down, rb, cb, ks = prep[part]
            cols = pl.ds(cb * 128, 128)
            if down:
                st2[2 + (i >> 16), 0, pl.ds(0, 16), pl.ds(0, 128)] = anchor
                w = _operands(_strassen_rhs, [[st2[i & 1, r, pl.ds(rb * 16, 16), pl.ds(c * Dq + cb * 128, 128)]
                                               .astype(F32) for c in range(4)] for r in range(4)])
                rows = pl.ds(pl.multiple_of(jnp.minimum(i, n2 - 1) * (r2 // 2) + rb * 8, 8), 8)
                for k in ks:
                    w2[k, rows, cols] = _pack(w[k])
            else:
                st13[4 + (i >> 16), 0, :, pl.ds(0, 128)] = anchor
                w = _operands(_strassen_rhs, [[st13[(i & 1) * 3, r, :, pl.ds(c * Fq + cb * 128, 128)]
                                               .astype(F32) for c in range(4)] for r in range(4)])
                for k in ks:
                    w13[i & 1, k, pl.ds(pl.multiple_of((i >> 1) * 8, 8), 8), cols] = _pack(w[k])

        def ln1(s):
            hn[...] = ada_ln(x_buf[s, pl.ds(PRE, seg - PRE), :].astype(F32), 0)

        def ln2(s, r):
            rows = pl.ds(r, 8)
            xn = x_buf[s, rows, :].astype(F32) + mod_rows(2, 8) * att[0, rows, :]
            x_buf[s, rows, :] = xn.astype(BF16)
            h2[s, rows, :] = ada_ln(xn, 3).astype(BF16)

        att[0] = jnp.zeros(att.shape[1:], F32)
        ln1(0)
        n_hg = n_heads // HG

        def seg_step(trip, u, mem):
            lhs = jnp.concatenate([mem, hn[...]], axis=0).astype(BF16)
            qi = jax.lax.broadcasted_iota(jnp.int32, (L, L), 0)
            ki = jax.lax.broadcasted_iota(jnp.int32, (L, L), 1)
            mask = (qi < M) | (qi >= ki)
            pr = pl.ds(pl.multiple_of(trip * 2 * PRE, 2 * PRE), 2 * PRE)

            def proj(t, g):
                gi, cols = g * HG // WG, pl.ds(g * HG % WG * dh, HG * dh)
                y = _dot(lhs, _unpack(wqkv[3 * gi + t, :, cols]))
                y = jnp.concatenate([y[:M], pre[3 * gi + t, pr, cols].astype(F32)[u * PRE:(u + 1) * PRE], y[M:]], axis=0)
                return [y[:, h * dh:(h + 1) * dh] for h in range(HG)]

            def probs(q, k):
                sc_ = jnp.where(mask, _dot_nt(q, k.astype(BF16)) * (scale * LOG2E), -1e9 * LOG2E)
                e = jnp.exp2(sc_ - jnp.max(sc_, axis=-1, keepdims=True))
                den = jnp.sum(e, axis=-1, keepdims=True)
                r = pl.reciprocal(den, approx=True)
                return e, r * (2.0 - den * r)

            def mix(p, v):
                return jnp.concatenate([_dot(e, vh.astype(BF16)) * r for (e, r), vh in zip(p, v)], axis=1)

            def out_proj(o, g):
                y = _dot(o, _unpack(wo[g]))
                per = -(-len(prep) // (2 * n_hg))
                first = (u * n_hg + g) * per
                for i in range(first, min(first + per, len(prep))):
                    n = (i - first) * (D // 128) // per
                    ffn_w_prepare(trip, i, y[:16, n * 128:(n + 1) * 128].astype(BF16))
                return y

            o, acc, p, v = {}, None, None, None
            done = 0
            for g in range(n_hg):
                q = proj(0, g)
                k = proj(1, g)
                if 1 <= g <= seg // 8:
                    att[1 + (trip >> 16), pl.ds(0, 8), pl.ds(0, dh)] = q[0][:8]
                    ln2(jnp.maximum(2 * trip + u - 1, 0), (g - 1) * 8)
                if g == 0:
                    ln1(jnp.minimum(2 * trip + u + 1, n_seg - 1))
                if g == 1 and u == 0:
                    start(ffn_w_cps(trip + 1))
                if g:
                    o[g - 1] = mix(p, v)
                v = proj(2, g)
                p = [probs(qh, kh) for qh, kh in zip(q, k)]
                upto = g + 1 - LAG if g + 1 < n_hg else n_hg - 2
                while done < upto:
                    y = out_proj(o.pop(done), done)
                    acc = y if acc is None else acc + y
                    done += 1
            o[n_hg - 1] = mix(p, v)
            for g in range(done, n_hg):
                acc = acc + out_proj(o.pop(g), g)
            att[0] = acc[M:]
            return acc[:M]

        def seg_body(trip, mem):
            wait(ffn_w_cps(trip))
            for u in range(2):
                mem = seg_step(trip, u, mem)
            return mem

        jax.lax.fori_loop(0, n_trip, seg_body, mem0[...].astype(F32))

        wait(ffn_w_cps(jnp.int32(n_trip)))
        for r in range(0, seg, 8):
            ln2(n_seg - 1, r)

        sb, qm = FFN_TM // seg, FFN_TM // 4

        def h_operand(k, row, n, col=0, width=Dq):
            per_row, per_chunk = WG * dh // Dq, D // 2 // qm
            return (k // (per_row * per_chunk), pl.ds(k // per_row % per_chunk * qm + row, n),
                    pl.ds(k % per_row * Dq + col, width))

        def a_operand(k, cols):
            per_chunk = D // 2 // qm
            return (2 + k // per_chunk, pl.ds(k % per_chunk * qm, qm // 2), cols)

        def ffn_lhs(i, row, half, col, ks=range(49)):
            rows = pl.ds(pl.multiple_of(row % seg, 16), 16)
            hs = [[h2[i * sb + r * qm // seg + row // seg, rows, pl.ds(c * Dq + col, 128)]
                   .astype(F32)[8 * half:8 * half + 8] for c in range(4)] for r in range(4)]
            a = _operands(_strassen_lhs, hs)
            for k in ks:
                wqkv[h_operand(k, row + 8 * half, 8, col, 128)] = pltpu.bitcast(a[k], U32)

        lhs_parts = [(half, col) for half in range(2) for col in range(0, Dq, 128)]

        @pl.loop(0, qm // 16)
        def _(j):
            for half, col in lhs_parts:
                ffn_lhs(0, pl.multiple_of(j * 16, 16), half, col)

        def out_cp(i):
            return pltpu.make_async_copy(x_buf.at[pl.ds(i * sb, sb)], out_hbm.at[pl.ds(i * sb, sb)], sem_out.at[i & 1])

        n_blk = S // FFN_TM

        def ffn_body(i, _):
            @pl.when(i >= 2)
            def _():
                out_cp(i - 2).wait()

            zero, nxt = i >> 16, jnp.minimum(i + 1, n_blk - 1)
            acts = [[] for _ in range(49)]
            for j in range(Fq // 128):
                cols = pl.ds(j * 128, 128)
                gate, up = (_results(lambda k: _dot(pltpu.bitcast(wqkv[h_operand(k, 0, qm)], F32),
                                                    _unpack(w13[t, k, :, cols]))) for t in range(2))
                act = [[_silu(g) * u for g, u in zip(gr, ur)] for gr, ur in zip(gate, up)]
                for k, a in enumerate(_operands(_strassen_lhs, act)):
                    if j < PARKED:
                        wqkv[a_operand(k, cols)] = _pack(a)
                    else:
                        acts[k].append(a.astype(BF16))

            def down_tile(k, n):
                m = _dot(jnp.concatenate([_unpack(wqkv[a_operand(k, pl.ds(0, PARKED * 128))])] + acts[k], axis=1),
                         _unpack(w2[k, :, pl.ds(n * 128, 128)]))
                piece, phase = divmod(k * (Dq // 128) + n, len(CUTS) - 1)
                if piece < qm // 16 * len(lhs_parts):
                    h2[n_seg + zero, pl.ds(0, 16), pl.ds(0, 128)] = m[:16].astype(BF16)
                    ffn_lhs(nxt, piece // len(lhs_parts) * 16, *lhs_parts[piece % len(lhs_parts)],
                            range(CUTS[phase], CUTS[phase + 1]))
                return m

            def down(k):
                return jnp.concatenate([down_tile(k, n) for n in range(Dq // 128)], axis=1)

            y = jnp.concatenate([jnp.concatenate(row, axis=1) for row in _results(down)], axis=0)
            xn = x_buf[pl.ds(i * sb, sb)].astype(F32).reshape(FFN_TM, D)
            x_buf[pl.ds(i * sb, sb)] = (xn + mod_rows(5, FFN_TM) * y).reshape(sb, seg, D).astype(BF16)
            out_cp(i).start()
            return 0

        jax.lax.fori_loop(0, n_blk, ffn_body, 0)
        for i in range(max(n_blk - 2, 0), n_blk):
            out_cp(i).wait()

    pl.run_scoped(main_phase,
                  pltpu.VMEM((seg - PRE, D), F32),
                  pltpu.VMEM((2, seg, D), F32),
                  pltpu.VMEM((n_seg + 1, seg, D), BF16),
                  pltpu.VMEM((2, 49, D // 8, F // 4), U32),
                  pltpu.VMEM((49, F // 8, D // 4), U32))


@functools.partial(jax.jit, static_argnames=("A_seg_len",))
def pallas_adaLN_cond__memory_aug_recurrent_mem_tr__glu_gated_swiglu__prompt_kernel(
    A_x, A_mem0, A_Wq, A_Wk, A_Wv, A_Wo, A_seg_len, B_x, B_w1, B_w3, B_w2, c, w_mod,
):
    del B_x
    B, S, D = A_x.shape
    assert B == 1
    M = A_mem0.shape[1]
    _, H, Dh = A_Wq.shape
    F = B_w1.shape[1]
    seg = int(A_seg_len)
    n_seg, n_grp = S // seg, H // WG
    any_spec = pl.BlockSpec(memory_space=pl.ANY)
    out = pl.pallas_call(
        functools.partial(_kernel, n_heads=H, dh=Dh),
        out_shape=jax.ShapeDtypeStruct((n_seg, seg, D), A_x.dtype),
        in_specs=[any_spec] * 11,
        out_specs=any_spec,
        scratch_shapes=[
            pltpu.VMEM((n_seg, seg, D), BF16),
            pltpu.VMEM((M, D), BF16),
            pltpu.VMEM((1, D), BF16),
            pltpu.VMEM((3 * n_grp, D // 2, WG * Dh), U32),
            pltpu.VMEM((H // HG, HG * Dh // 2, D), U32),
            pltpu.VMEM((3 * n_grp, n_seg * PRE, WG * Dh), BF16),
            pltpu.VMEM((6 * D // 128, 8, 128), F32),
            pltpu.VMEM((5, 4, 16, F), BF16),
            pltpu.VMEM((3, 4, 32, D), BF16),
            pltpu.SemaphoreType.DMA((4,)),
            pltpu.SemaphoreType.DMA((6,)),
            pltpu.SemaphoreType.DMA((6,)),
            pltpu.SemaphoreType.DMA((2,)),
            pltpu.SemaphoreType.DMA((6,)),
            pltpu.SemaphoreType.DMA((2,)),
        ],
        compiler_params=pltpu.CompilerParams(vmem_limit_bytes=127 * 1024 * 1024),
    )(
        A_x.reshape(n_seg, seg, D), A_mem0.reshape(M, D),
        A_Wq.reshape(D // 2, 2 * H, Dh), A_Wk.reshape(D // 2, 2 * H, Dh), A_Wv.reshape(D // 2, 2 * H, Dh),
        A_Wo.reshape(H * Dh, D),
        B_w1.reshape(4, D // 4, F), B_w3.reshape(4, D // 4, F), B_w2.reshape(4, F // 4, D), c, w_mod,
    )
    return out.reshape(B, S, D)
```
